```python
import jax
import jax.numpy as jnp

def _softmax(x, axis=-1):
    return jax.nn.softmax(x, axis=axis)

def _gelu(x):
    return jax.nn.gelu(x, approximate=True)

def _silu(x):
    return jax.nn.silu(x)

def _sigmoid(x):
    return jax.nn.sigmoid(x)

def _layernorm(x, axis=-1, eps=1e-05):
    m = jnp.mean(x, axis=axis, keepdims=True)
    v = jnp.var(x, axis=axis, keepdims=True)
    return (x - m) / jnp.sqrt(v + eps)

def _scatter_add(tgt, idx, src, axis=0):
    return tgt.at[idx].add(src)

def _segment_sum(src, seg, n):
    return jax.ops.segment_sum(src, seg, n)

class _Rng:

    def __init__(self, key):
        self._k = key

    def _next(self):
        self._k, sub = jax.random.split(self._k)
        return sub

    def normal(self, shape):
        return jax.random.normal(self._next(), shape, dtype=jnp.bfloat16)

    def randint(self, lo, hi, shape):
        return jax.random.randint(self._next(), shape, lo, hi, dtype=jnp.int32)

    def uniform(self, shape, lo=0.0, hi=1.0):
        return jax.random.uniform(self._next(), shape, jnp.bfloat16, lo, hi)

    def permutation(self, n):
        return jax.random.permutation(self._next(), n)
kernel_name = 'concat_heads__sliding_local_dilated__memory_aug_recurrent_mem_tr__prompt'

def setup_inputs():
    _rng = _Rng(jax.random.key(int.from_bytes(__import__("os").urandom(4), "little")))
    _w = lambda a: (lambda t: t.astype(jnp.bfloat16) if jnp.issubdtype(t.dtype, jnp.floating) else t)(jnp.asarray(a))

    def _A_setup():
        B, S, D = (1, 2048, 640)
        return {'x': _w((lambda *s: _rng.normal(s) * 0.05)(B, S, D)), 'wqkv': _w((lambda *s: _rng.normal(s) * 0.05)(D, 3 * D)), 'wo': _w((lambda *s: _rng.normal(s) * 0.05)(D, D))}
    _A_in = _A_setup()

    def _B_setup():
        B, S, Dm = (1, 2048, 640)
        H, Dh = (32, 192)
        M, seg = (8, 32)
        seg = min(seg, S)
        S = S // seg * seg
        return {'x': _w((lambda *s: _rng.normal(s) * 0.05)(B, S, Dm)), 'mem0': _w((lambda *s: _rng.normal(s) * 0.05)(B, M, Dm)), 'Wq': _w((lambda *s: _rng.normal(s) * 0.05)(Dm, H, Dh) * Dm ** (-0.5)), 'Wk': _w((lambda *s: _rng.normal(s) * 0.05)(Dm, H, Dh) * Dm ** (-0.5)), 'Wv': _w((lambda *s: _rng.normal(s) * 0.05)(Dm, H, Dh) * Dm ** (-0.5)), 'Wo': _w((lambda *s: _rng.normal(s) * 0.05)(H, Dh, Dm) * (H * Dh) ** (-0.5)), 'seg_len': seg}
    _B_in = _B_setup()
    return {'A_x': _A_in['x'], 'A_wqkv': _A_in['wqkv'], 'A_wo': _A_in['wo'], 'B_x': _B_in['x'], 'B_mem0': _B_in['mem0'], 'B_Wq': _B_in['Wq'], 'B_Wk': _B_in['Wk'], 'B_Wv': _B_in['Wv'], 'B_Wo': _B_in['Wo'], 'B_seg_len': _B_in['seg_len']}

def reference(A_x, A_wqkv, A_wo, B_x, B_mem0, B_Wq, B_Wk, B_Wv, B_Wo, B_seg_len):

    def _A_ref(x, wqkv, wo):
        B, S, D = x.shape
        H = 32
        Dh = D // H
        W, dil = (8, 2)
        qkv = (lambda x, *d: x.transpose(*d))((x @ wqkv).reshape(B, S, 3, H, Dh), 2, 0, 3, 1, 4)
        q, k, v = (qkv[0], qkv[1], qkv[2])
        scale = Dh ** (-0.5)
        pos = jnp.arange(S)
        off = jnp.arange(W) * dil
        idx = pos[:, None] - off[None, :]
        mask = idx >= 0
        idx_c = jnp.where(mask, idx, 0).reshape(-1)
        kg = k[:, :, idx_c, :].reshape(B, H, S, W, Dh)
        vg = v[:, :, idx_c, :].reshape(B, H, S, W, Dh)
        logits = jnp.einsum('bhsd,bhswd->bhsw', q, kg) * scale
        logits = jnp.where(mask[None, None, :, :], logits, -1000000000.0)
        attn = _softmax(logits, axis=-1)
        o = jnp.einsum('bhsw,bhswd->bhsd', attn, vg)
        return (lambda x, *d: x.transpose(*d))(o, 0, 2, 1, 3).reshape(B, S, D) @ wo

    def _B_ref(x, mem0, Wq, Wk, Wv, Wo, seg_len):
        B, S, Dm = x.shape
        H, Dh = (Wq.shape[1], Wq.shape[2])
        M = mem0.shape[1]
        scale = Dh ** (-0.5)
        n_seg = S // seg_len
        L = M + seg_len
        idx = jnp.arange(L)
        mask = (idx[:, None] < M) | (idx[:, None] >= idx[None, :])
        mem = mem0
        outs = []
        for s in range(n_seg):
            xs = x[:, s * seg_len:(s + 1) * seg_len, :].copy()
            h = jnp.concatenate([mem, xs], axis=1)
            q = jnp.einsum('btd,dhe->bhte', h, Wq)
            k = jnp.einsum('btd,dhe->bhte', h, Wk)
            v = jnp.einsum('btd,dhe->bhte', h, Wv)
            scores = jnp.einsum('bhqe,bhke->bhqk', q, k) * scale
            scores = jnp.where(mask[None, None], scores, -1000000000.0)
            p = _softmax(scores, axis=-1)
            o = jnp.einsum('bhqk,bhke->bhqe', p, v)
            o = jnp.einsum('bhte,hed->btd', o, Wo)
            mem = o[:, :M, :].copy()
            outs.append(o[:, M:, :])
        return jnp.concatenate(outs, axis=1)
    a = _A_ref(A_x, A_wqkv, A_wo)
    b = _B_ref(B_x, B_mem0, B_Wq, B_Wk, B_Wv, B_Wo, B_seg_len)
    return jnp.concatenate([a, b], axis=-1)
```

```python
import functools

import jax
import jax.numpy as jnp
from jax import lax
from jax.experimental import pallas as pl
from jax.experimental.pallas import tpu as pltpu


F32, BF16, U32 = jnp.float32, jnp.bfloat16, jnp.uint32
NT = (((1,), (1,)), ((), ()))
MASKED = -1000000000.0

S, D = 2048, 640
LT = D // 128

AH, AD, AW, ADIL = 32, 20, 8, 2
HALO = 16
TB = 128
NB = S // TB
RC = 8

H, DH, M, SEG = 32, 192, 8, 32
L = M + SEG
RG = L // 8
NP = H // 2
FT = H * DH // 128
NSEG = S // SEG
GW = 2 * LT
NG = pl.cdiv(FT, GW)

NEAR = 0
ONLY = 0
OMEM = 0
LATE = 1
TAILG = 2
LAG_S, LAG_N, LAG_V = 3, 2, 4


class _Group:
    def __init__(self, n):
        k = n // 2
        self.n = n
        self.side = (range(k), range(k, n))
        self.label = list(range(k)) + list(range(LT - k, LT))
        self.mates = [[b for b in self.side[c < k] if self.label[b] != self.label[c]]
                      for c in range(n)]
        self.plain = [[i for i in range(LT) if i != self.label[c]
                       and i not in [self.label[b] for b in self.mates[c]]] for c in range(n)]
        keys = [(i, c) for c in range(n) for i in range(LT)]
        keys += [("other", c) for c in range(n)]
        keys += [("both", a, b) for a in self.side[0] for b in self.mates[a]]
        self.slot = {key: i for i, key in enumerate(keys)}
        for a in self.side[0]:
            for b in self.mates[a]:
                self.slot["both", b, a] = self.slot["both", a, b]


GROUPS = [_Group(min(GW, FT - g * GW)) for g in range(NG)]
SLOTS = max(GROUPS[0].slot.values()) + 1

IN_PAIRS = {3: 1, 4: 2}


def _out_pairs(g, ph):
    if not OMEM:
        return {3: 1, 4: 2}
    return {3: 0, 4: 1} if (g + ph) % 2 else {2: 2, 3: 0, 4: 1}


def _ds(i, n):
    return pl.ds(i * n if isinstance(i, int) else pl.multiple_of(i * n, n), n)


def _dot(a, b):
    return jnp.dot(a, b, preferred_element_type=F32)


def _share(tasks, k, n):
    return tasks[k * len(tasks) // n:(k + 1) * len(tasks) // n]


def _run(tasks):
    for task in tasks:
        task()


def _rows(parts):
    return parts[0] if len(parts) == 1 else jnp.concatenate(parts, axis=0)


def _split(t):
    return [t[r:r + 8] for r in range(0, t.shape[0], 8)]


class _Sums(dict):
    def add(self, key, t):
        self[key] = self[key] + t if key in self else t

    def sub(self, key, t):
        self[key] = self[key] - t if key in self else -t


def _kernel(ax_hbm, awqkv_hbm, awo_hbm, bx_hbm, mem_hbm, wq_hbm, wk_hbm, wv_hbm, wo_hbm,
            out_hbm,
            ax, awqkv, awo, tmp, wqkv_p, wo_p, q_s, kv_s, oa_s, outa,
            bx, mem, raw, wt, l_own, l_other, l_sum, l_both, l_plain, ahead, o_s, o_old, z_s, outb,
            order0, order1, order2,
            sem_a, sem_x, sem_w, sem_b, sem_o):
    cp = pltpu.make_async_copy

    def rows_copy(src, dst, r0, r1, sem):
        return cp(src.at[pl.ds(r0, r1 - r0), :], dst.at[pl.ds(r0, r1 - r0), :], sem)

    c_wqkv = [cp(awqkv_hbm.at[:, pl.ds(j * D, D)], awqkv.at[j], sem_a.at[j]) for j in range(3)]
    c_awo = cp(awo_hbm, awo, sem_a.at[3])
    x_cuts = (0, 2 * TB, 4 * TB, S)
    c_ax = [rows_copy(ax_hbm, ax, x_cuts[c], x_cuts[c + 1], sem_x.at[c]) for c in range(3)]
    c_mem = cp(mem_hbm, mem, sem_b.at[0])
    c_bx0 = rows_copy(bx_hbm, bx, 0, 8 * SEG, sem_b.at[1])
    c_bx1 = rows_copy(bx_hbm, bx, 8 * SEG, S, sem_b.at[2])
    c_outa = cp(outa, out_hbm.at[:, pl.ds(0, D)], sem_o.at[0])

    def chunk(j, g):
        return 3 * g + j if j < 3 else 3 * NG + g

    def c_w(c):
        j, g = (c % 3, c // 3) if c < 3 * NG else (3, c - 3 * NG)
        n = GROUPS[g].n * 128
        return cp((wq_hbm, wk_hbm, wv_hbm, wo_hbm)[j].at[pl.ds(g * GW * 128, n), :],
                  raw.at[c, pl.ds(0, n), :], sem_w.at[c])

    def w_wait(c):
        cp(raw.at[c], raw.at[c], sem_w.at[c]).wait()

    def c_outb(r0, n):
        return cp(outb.at[pl.ds(r0, n), :], out_hbm.at[pl.ds(r0, n), pl.ds(D, D)], sem_o.at[1])

    def start(copies):
        for c in copies:
            c.start()

    def wait(copies):
        for c in copies:
            c.wait()

    def permute_rows(dst, base):
        for d in range(AD):
            for t in range(LT):
                dst[pl.ds((base + d * AH) // 2, AH // 2), t * 128:(t + 1) * 128] = pltpu.bitcast(
                    tmp[t, pl.ds(d, AH, stride=AD), :].astype(BF16), U32)

    def prep_wqkv(j):
        for t in range(LT):
            tmp[t] = awqkv[j, t * 128:(t + 1) * 128, :].astype(F32).T
        permute_rows(wqkv_p, j * D)

    def prep_wo():
        for t in range(LT):
            tmp[t] = awo[:, t * 128:(t + 1) * 128].astype(F32)
        permute_rows(wo_p, 0)

    def a_proj(i, b, j):
        w = pltpu.bitcast(wqkv_p[j * D // 2:(j + 1) * D // 2, :], BF16)
        r = lax.dot_general(ax[_ds(i, TB), :], w, NT, preferred_element_type=F32)
        for t in range(LT):
            rt = r[:, t * 128:(t + 1) * 128]
            if j == 0:
                q_s[b, t] = rt
                continue
            c = (j - 1) * LT + t
            kv_s[b, c, HALO:HALO + TB, :] = rt
            if isinstance(i, int) and i == 0:
                kv_s[b, c, 0:HALO, :] = jnp.broadcast_to(rt[0:1, :], (HALO, 128))
            else:
                kv_s[b, c, 0:HALO, :] = kv_s[1 - b, c, TB:TB + HALO, :]

    def a_attention(b, first_block=False):
        state = {}

        def window(c, r0, w):
            lo = HALO + r0 - ADIL * w
            return kv_s[b, c, lo:lo + RC, :]

        def logits(r0):
            q = [q_s[b, t, r0:r0 + RC, :] for t in range(LT)]
            state[r0] = []
            for w in range(AW):
                a = q[0] * window(0, r0, w)
                for t in range(1, LT):
                    a = a + q[t] * window(t, r0, w)
                state[r0].append(a + pltpu.roll(a, 2 * AH, 1))

        def fold(r0):
            state[r0] = [a + pltpu.roll(a, AH, 1) for a in state[r0]]

        def mix(r0):
            lg = []
            for w, a in enumerate(state.pop(r0)):
                a = a * (AD ** -0.5)
                if first_block and r0 < ADIL * w:
                    pos = lax.broadcasted_iota(jnp.int32, (RC, 128), 0) + r0
                    a = jnp.where(pos >= ADIL * w, a, MASKED)
                lg.append(a)
            m = functools.reduce(jnp.maximum, lg)
            e = [jnp.exp(a - m) for a in lg]
            inv = 1.0 / functools.reduce(jnp.add, e)
            p = [x * inv for x in e]
            for t in range(LT):
                o = p[0] * window(LT + t, r0, 0)
                for w in range(1, AW):
                    o = o + p[w] * window(LT + t, r0, w)
                oa_s[b, r0:r0 + RC, t * 128:(t + 1) * 128] = o

        n = TB // RC
        return [functools.partial(f, (k - lag) * RC) for k in range(n + 2)
                for lag, f in enumerate((logits, fold, mix)) if 0 <= k - lag < n]

    def a_out(i, b):
        outa[_ds(i, TB), :] = _dot(oa_s[b], pltpu.bitcast(wo_p[...], BF16)).astype(BF16)

    def a_stage(i, b, extra=((), (), ()), first_block=False):
        side = a_attention(1 - b, first_block)
        for j in range(3):
            a_proj(i, b, j)
            _run(_share(side, j, 3))
            _run(extra[j])
        a_out(i - 1, 1 - b)

    def w_prep(c, grp, transposed):
        def transpose(f):
            t = pltpu.bitcast(raw[c, f * 128:(f + 1) * 128, :].T, U32)
            for i in range(LT):
                wt[c, grp.slot[i, f]] = t[i * 64:(i + 1) * 64]

        def combine(r):
            rows = slice(8 * r, 8 * r + 8)

            def tile(i, f):
                if transposed:
                    return pltpu.bitcast(wt[c, grp.slot[i, f], rows], BF16).astype(F32)
                t = pltpu.bitcast(
                    raw[c, f * 128 + 16 * r:f * 128 + 16 * r + 16, i * 128:(i + 1) * 128], U32)
                if i != grp.label[f]:
                    wt[c, grp.slot[i, f], rows] = t
                return pltpu.bitcast(t, BF16).astype(F32)

            def put(key, t):
                wt[c, grp.slot[key], rows] = pltpu.bitcast(t.astype(BF16), U32)

            own = {b: tile(grp.label[b], b) for b in grp.side[1]}
            other = dict(own)
            for a in grp.side[0]:
                own[a] = other[a] = tile(grp.label[a], a)
                for b in grp.mates[a]:
                    ta, tb = tile(grp.label[b], a), tile(grp.label[a], b)
                    put(("both", a, b), ta + tb)
                    own[a], other[a] = own[a] - ta, other[a] + tb
                    own[b], other[b] = own[b] - tb, other[b] + ta
                put((grp.label[a], a), own[a])
                put(("other", a), other[a])
            for b in grp.side[1]:
                put((grp.label[b], b), own[b])
                put(("other", b), other[b])
            if not transposed:
                for f in range(grp.n):
                    for i in grp.plain[f]:
                        tile(i, f)

        return ([functools.partial(transpose, f) for f in range(grp.n * transposed)],
                [functools.partial(combine, r) for r in range(8)])

    full = 3 * (NG - 1)
    if not ONLY:
        AHEAD = 4
        start([c_wqkv[0], c_ax[0], c_wqkv[1]])
        c_wqkv[0].wait()
        c_wqkv[2].start()
        prep_wqkv(0)
        wait([c_ax[0], c_wqkv[1]])
        start([c_awo, c_ax[1]])
        a_proj(0, 0, 0)
        prep_wqkv(1)
        c_wqkv[2].wait()
        c_ax[2].start()
        a_proj(0, 0, 1)
        prep_wqkv(2)
        a_proj(0, 0, 2)
        c_awo.wait()
        c_w(0).start()
        prep_wo()
        a_stage(1, 1, first_block=True)
        start([c_w(c) for c in range(1, AHEAD - 1)])

        full = 3 * (NG - 1)

        def a_step(it, carry):
            for b in range(2):
                c = jnp.where(it == 1, full - 2, 2 * it - 4) + b

                @pl.when(it == 1)
                def _():
                    c_ax[1 + b].wait()
                    if b:
                        start([c_mem, c_bx0, c_w(AHEAD - 1)])

                @pl.when(it > 1)
                def _():
                    for k in range(2, NB // 2):
                        @pl.when(it == k)
                        def _():
                            c_w(2 * k - 4 + b + AHEAD).start()
                    w_wait(c)

                first, second = w_prep(c, GROUPS[0], True)
                a_stage(2 * it + b, b, (first, second[:3], second[3:]))
            return carry

        lax.fori_loop(1, NB // 2, a_step, 0)
        start([c_w(c) for c in range(full + AHEAD, 4 * NG)])
        wait([c_mem, c_bx0])

    NK = 2 * M
    order = (order0, order1, order2)

    def product(parts, c, grp, key):
        return _split(_dot(_rows(parts), pltpu.bitcast(wt[c, grp.slot[key]], BF16)))

    def grp_rows(r):
        return slice(8 * r, 8 * r + 8)

    def memory_operands(ph, known, i, t):
        known[i] = t
        l_plain[ph, i, 0:M] = t
        for k, u in known.items():
            if k != i:
                l_sum[ph, min(i, k), max(i, k), 0:M] = t + u

    def token_operands(s, ph, first=False, last=False):
        def tokens(ds):
            seg = s + ds if isinstance(s, int) else jnp.minimum(s + ds, NSEG - 1)
            return [[None] + _split(bx[_ds(seg, SEG), i * 128:(i + 1) * 128].astype(F32))
                    for i in range(LT)]

        cur = tokens(0)
        mate = {}
        if not first:
            before = tokens(-1)
            mate.update({r1: [t[r0] for t in before] for r0, r1 in IN_PAIRS.items()})
        if not last:
            after, later = tokens(1), tokens(2)
            mate.update({r0: [t[r1] for t in after] for r0, r1 in IN_PAIRS.items()})
        for r in range(1, RG):
            rows = grp_rows(r)
            for i in range(LT):
                l_plain[ph, i, rows] = cur[i][r]
                if r in mate:
                    l_other[ph, i, rows] = cur[i][r] - mate[r][i]
                if not last and r in IN_PAIRS.values():
                    l_own[ph, i, rows] = later[i][r]
                    if first:
                        l_own[1 - ph, i, rows] = after[i][r]
                for k in range(LT):
                    if k > i:
                        l_sum[ph, i, k, rows] = cur[i][r] + cur[k][r]
                    if k != i and not last and r in IN_PAIRS:
                        l_both[ph, i, k, rows] = cur[i][r] + mate[r][k]

    def segment(s, ph, first=False, last=False):
        y = [_Sums() for _ in range(3)]
        st = [dict() for _ in range(NP)]
        near = NEAR and not first and not last
        live = range(1 if last else 0, RG)

        def project(j, g):
            grp, c, f0 = GROUPS[g], chunk(j, g), g * GW
            lab = grp.label
            every = live if j == 0 else range(RG)
            to_next = {} if last else IN_PAIRS
            from_prev = () if first else tuple(IN_PAIRS.values())
            early = [r for r in every if r not in from_prev]
            gift = _Sums()
            left = {a: 1 + len(grp.mates[a]) for a in grp.side[ph]}

            def plain(i, r):
                return l_plain[ph, i, grp_rows(r)]

            def give(a, res):
                for r, t in zip(early, res):
                    if r in to_next:
                        gift.add((a, r), t)
                left[a] -= 1
                if not left[a]:
                    for r0, r1 in to_next.items():
                        ahead[j, f0 + a, 0, grp_rows(r1 - 1)] = gift.pop((a, r0))

            def own(a):
                parts = [plain(lab[a], r) for r in early]
                parts += [l_own[ph, lab[a], grp_rows(r)] for r in to_next.values()]
                res = product(parts, c, grp, (lab[a], a))
                for r, t in zip(early, res):
                    y[j].add((f0 + a, r), t)
                for r in from_prev:
                    y[j].add((f0 + a, r), ahead[j, f0 + a, 1, grp_rows(r - 1)])
                for r, t in zip(to_next.values(), res[len(early):]):
                    ahead[j, f0 + a, 1, grp_rows(r - 1)] = t
                give(a, res)

            def other(b):
                if first:
                    parts = [l_own[1 - ph, lab[b], grp_rows(r)] for r in to_next.values()]
                    for r, t in zip(to_next.values(), product(parts, c, grp, (lab[b], b))):
                        ahead[j, f0 + b, 1, grp_rows(r - 1)] = t
                parts = [l_other[ph, lab[b], grp_rows(r)] if r in to_next or r in from_prev
                         else plain(lab[b], r) for r in every]
                for r, t in zip(every, product(parts, c, grp, ("other", b))):
                    y[j].add((f0 + b, r), t)

            def inherit(b):
                for r in from_prev:
                    y[j].add((f0 + b, r), ahead[j, f0 + b, 0, grp_rows(r - 1)])
                for r0, r1 in to_next.items():
                    y[j].add((f0 + b, r0), ahead[j, f0 + b, 1, grp_rows(r1 - 1)])

            def both(a, b):
                parts = [l_both[ph, lab[a], lab[b], grp_rows(r)] if r in to_next
                         else plain(lab[a], r) for r in early]
                res = product(parts, c, grp, ("both", a, b))
                for r, t in zip(early, res):
                    y[j].add((f0 + b, r), t)
                give(a, res)

            def cross(a, b):
                i, k = sorted((lab[a], lab[b]))
                parts = [l_sum[ph, i, k, grp_rows(r)] for r in every]
                for r, t in zip(every, product(parts, c, grp, (lab[b], a))):
                    y[j].add((f0 + a, r), t)
                    y[j].sub((f0 + b, r), t)

            def single(i, f):
                for r, t in zip(every, product([plain(i, r) for r in every], c, grp, (i, f))):
                    y[j].add((f0 + f, r), t)

            task = functools.partial
            steps = []
            for a, b0 in zip(grp.side[ph], grp.side[1 - ph]):
                step = [((lab[a],), task(own, a)), ((lab[b0],), task(other, b0))]
                step += [((lab[a],), task(both, a, b)) for b in grp.mates[a]]
                step += [((lab[a], lab[b]), task(cross, a, b)) for b in grp.mates[a]]
                step += [((i,), task(single, i, f)) for f in (a, b0) for i in grp.plain[f]]
                steps.append(step)
            got = [((0,), task(inherit, b)) for b in grp.side[1 - ph]]
            if first:
                steps[-1] += got
            else:
                steps[0] = got + steps[0]
            return steps

        def tiles(j, p, groups):
            return [_rows([y[j].pop((3 * p + t, r)) for r in groups]) for t in range(3)]

        def stationary(t):
            low = lax.broadcasted_iota(jnp.int32, (L, 128), 1) < 64
            return (_rows([t[0], t[2]]).astype(BF16),
                    _rows([jnp.where(low, t[1], 0.0), jnp.where(low, 0.0, t[1])]).astype(BF16))

        n = 8 * len(live)
        row = lax.broadcasted_iota(jnp.int32, (n, 2 * L), 0) + (L - n)
        col = lax.broadcasted_iota(jnp.int32, (n, 2 * L), 1)
        head0 = col < L
        visible = (row < M) | (row >= jnp.where(head0, col, col - L))

        def score(p):
            q = tiles(0, p, live)
            outer, shared = stationary(tiles(1, p, range(RG)))
            sc = lax.dot_general(_rows([q[0], q[2]]), outer, NT, preferred_element_type=F32)
            sc = jnp.where(head0, sc[0:n], sc[n:]) + lax.dot_general(
                q[1], shared, NT, preferred_element_type=F32)
            sc = jnp.where(visible, sc * (DH ** -0.5), MASKED)
            m0 = jnp.max(jnp.where(head0, sc, -jnp.inf), axis=1, keepdims=True)
            m1 = jnp.max(jnp.where(head0, -jnp.inf, sc), axis=1, keepdims=True)
            st[p]["s"] = sc - jnp.where(head0, m0, m1)

        def normalize(p):
            e = jnp.exp(st[p]["s"])
            l0 = jnp.sum(jnp.where(head0, e, 0.0), axis=1, keepdims=True)
            l1 = jnp.sum(jnp.where(head0, 0.0, e), axis=1, keepdims=True)
            st[p]["p"] = e / jnp.where(head0, l0, l1)

        def keep(f, r, t):
            o_s[ph, f, grp_rows(r)] = t
            grp = GROUPS[f // GW]
            if not first and f % GW in grp.side[1 - ph]:
                for r0, r1 in _out_pairs(f // GW, 1 - ph).items():
                    if r1 == r:
                        o_old[f, grp_rows(r0)] = t + o_s[1 - ph, f, grp_rows(r0)]

        def pv_near(p):
            v = st[p]["v"] = tiles(2, p, range(RG))
            rest = [jnp.sum(t[NK:NK + 8] + t[NK + 8:NK + 16] + t[NK + 16:L], axis=0, keepdims=True)
                    for t in v]
            pr = st[p]["p"][M:NK]
            low = lax.broadcasted_iota(jnp.int32, (8, 128), 1) < 64
            key = lax.broadcasted_iota(jnp.int32, (8, 2 * L), 1)
            acc = [None] * 3
            for j in range(NK + 1):
                a, b = [jnp.broadcast_to(
                    jnp.sum(jnp.where(key == c, pr, 0.0), axis=1, keepdims=True), (8, 128))
                    for c in (j, L + j)]
                for t, w in enumerate((a, jnp.where(low, a, b), b)):
                    term = w * (v[t][j:j + 1] if j < NK else rest[t])
                    acc[t] = term if j == 0 else acc[t] + term
            for t in range(3):
                keep(3 * p + t, 1, acc[t])
                order[p % 3][8 + 8 * t:16 + 8 * t, :] = acc[t]

        def pv(p):
            pr = st[p]["p"]
            groups = list(live)
            if near:
                zero = pl.multiple_of(lax.shift_right_logical(s, 16) * 8, 8)
                order[p % 3][0:M, 0:2 * L] = pr[0:M]
                pr = _rows([order[p % 3][pl.ds(zero, M), 0:2 * L], pr[NK:L]])
                groups.remove(1)
            outer, shared = stationary(st[p]["v"] if near else tiles(2, p, range(RG)))
            h0 = lax.broadcasted_iota(jnp.int32, pr.shape, 1) < L
            res = _split(_dot(_rows([jnp.where(h0, pr, 0.0), jnp.where(h0, 0.0, pr)]), outer))
            res = (res[:len(groups)], _split(_dot(pr, shared)), res[len(groups):])
            for t in range(3):
                for r, v in zip(groups, res[t]):
                    keep(3 * p + t, r, v)

        z = _Sums()

        def out_project(g):
            grp, c, f0 = GROUPS[g], chunk(3, g), g * GW
            lab = grp.label
            to_next = {} if last else _out_pairs(g, ph)
            from_prev = {} if first else {r1: r0 for r0, r1 in _out_pairs(g, 1 - ph).items()}
            late = [r for r in live if r not in to_next]
            old = () if first else tuple(_out_pairs(g, ph))

            def cur(f, r):
                return o_s[ph, f0 + f, grp_rows(r)]

            def prev(f, r):
                return o_s[1 - ph, f0 + f, grp_rows(from_prev[r])]

            def joined(f, a):
                return [cur(f, r) + prev(a, r) if r in from_prev else cur(f, r) for r in late]

            def own(a):
                parts = joined(a, a) + [o_old[f0 + a, grp_rows(r)] for r in old]
                res = product(parts, c, grp, (lab[a], a))
                for r, t in zip(late, res):
                    z.add((0, lab[a], r), t)
                for r, t in zip(old, res[len(late):]):
                    z.add((2, lab[a], r), t)

            def other(b):
                for r, t in zip(live, product([cur(b, r) for r in live], c, grp, ("other", b))):
                    z.add((0, lab[b], r), t)
                    if r in from_prev:
                        z.sub((1, lab[b], from_prev[r]), t)
                    if r in to_next:
                        z.add((-1, lab[b], to_next[r]), t)
                if last:
                    parts = [o_old[f0 + b, grp_rows(r0)] if r1 in live else prev(b, r1)
                             for r1, r0 in from_prev.items()]
                    for r, t in zip(from_prev.values(), product(parts, c, grp, (lab[b], b))):
                        z.add((1, lab[b], r), t)

            def both(a, b):
                alone = [r for r in from_prev if r not in live]
                parts = joined(b, a) + [prev(a, r) for r in alone]
                for r, t in zip(late + alone, product(parts, c, grp, ("both", a, b))):
                    if r in live:
                        z.add((0, lab[a], r), t)
                    if r in from_prev:
                        z.add((1, lab[b], from_prev[r]), t)

            def cross(a, b):
                parts = [cur(a, r) - cur(b, r) for r in live]
                for r, t in zip(live, product(parts, c, grp, (lab[b], a))):
                    z.add((0, lab[a], r), t)
                    z.add((0, lab[b], r), t)

            def single(i, f):
                for r, t in zip(live, product([cur(f, r) for r in live], c, grp, (i, f))):
                    z.add((0, i, r), t)

            task = functools.partial
            steps = []
            for a, b0 in zip(grp.side[ph], grp.side[1 - ph]):
                step = [((lab[a],), task(own, a)), ((lab[b0],), task(other, b0))]
                step += [((lab[a],), task(both, a, b)) for b in grp.mates[a]]
                step += [((lab[a], lab[b]), task(cross, a, b)) for b in grp.mates[a]]
                step += [((i,), task(single, i, f)) for f in (a, b0) for i in grp.plain[f]]
                steps.append(step)
            return steps

        def postpone(steps, rank):
            flat = [x for step in steps for x in step]
            out = [[x for x in step if rank(x[0]) <= 0] for step in steps]
            return out + [[x for x in flat if rank(x[0]) == k] for k in range(1, LATE + 1)]

        steps, done = [], {}
        for g in range(NG):
            for j in range(3):
                new = project(j, g)
                if not steps and not first:
                    new = postpone(new, lambda t: max(t) - (LT - 1 - LATE))
                steps += new
                done[j, g] = len(steps)
        n_in = len(steps)
        tail = [step for g in range(NG - TAILG, NG) for step in out_project(g)]
        tail = postpone(tail, lambda t: min(t) - (LT - 1 - LATE))
        steps += [step for g in range(NG - TAILG) for step in out_project(g)] + tail
        side = [[] for _ in steps]
        at_s = at_v = 0
        for p in range(NP):
            g = (3 * p + 2) // GW
            at_s = max(at_s + 1, done[1, g] - 1 + LAG_S)
            at_v = max(at_v + (3 if near else 1), done[2, g] - 1 + LAG_V)
            end = n_in - 1 if first else len(steps)
            side[min(at_s, end)].append(functools.partial(score, p))
            side[min(at_s + LAG_N, end)].append(functools.partial(normalize, p))
            if near:
                side[at_v].append(functools.partial(pv_near, p))
            side[min(at_v + (2 if near else 0), end)].append(functools.partial(pv, p))
        if first:
            rest = a_attention(1) + [functools.partial(a_out, NB - 1, 1)]
            for k in range(30):
                side[k] += _share(rest, k, 30)
            side[29].append(lambda: wait([c_w(full + j) for j in range(3)]))
            rest = [t for j in range(3) for part in w_prep(full + j, GROUPS[-1], True) for t in part]
            for k in range(30):
                side[30 + k] += _share(rest, k, 30)

            def prep_out():
                def body(c, carry):
                    w_wait(c)
                    _run(w_prep(c, GROUPS[0], False)[1])
                    return carry
                lax.fori_loop(3 * NG, 4 * NG - 1, body, 0)
                c_w(4 * NG - 1).wait()
                c_bx1.start()
            side[n_in - 1].append(prep_out)
            rest = w_prep(4 * NG - 1, GROUPS[-1], False)[1]
            for k in range(8):
                side[n_in + k] += _share(rest, k, 8)
        if not last:
            side[n_in + 1 if first else n_in - 4].append(functools.partial(token_operands, s + 1, 1 - ph))

        def resume():
            for i in range(LT):
                for r in range(1, RG):
                    z.add((2, i, r), z_s[ph, i, grp_rows(r)])
                    z.add((1, i, r), z_s[1 - ph, i, grp_rows(r)])
                for r in {r1 for g in range(NG) for r1 in _out_pairs(g, 1 - ph).values()}:
                    if r in live:
                        z.sub((0, i, r), z_s[2, i, grp_rows(r)])
        if not first:
            side[n_in - 1].append(resume)

        known = {}
        for k, (step, extra) in enumerate(zip(steps, side)):
            _run(task for _, task in step)
            _run(extra)
            behind = len(steps) - 1 - k
            if not last and behind <= LATE:
                for i in range(LT - behind):
                    if i not in known:
                        memory_operands(1 - ph, known, i, z.pop((0, i, 0)))

        def write(back):
            seg = s - back if isinstance(s, int) else jnp.maximum(s - back, 0)
            for i in range(LT):
                outb[_ds(seg, SEG), i * 128:(i + 1) * 128] = _rows(
                    [z.pop((back, i, r)) for r in range(1, RG)]).astype(BF16)

        if not first:
            write(2)
        if last:
            write(1)
            write(0)
        for (back, i, r), t in z.items():
            z_s[2 if back < 0 else (ph + back) % 2, i, grp_rows(r)] = t

    if ONLY:
        c_bx1.start()
    else:
        known = {}
        for i in range(LT):
            memory_operands(0, known, i, mem[:, i * 128:(i + 1) * 128].astype(F32))
        token_operands(0, 0, first=True)
        segment(0, 0, first=True)
    c_outa.start()

    def b_step(it, carry):
        @pl.when(it == 1)
        def _():
            c_bx1.wait()
        s0 = 1 + 2 * it
        segment(s0, 1)
        segment(s0 + 1, 0)

        @pl.when(it > 0)
        def _():
            c_outb(pl.multiple_of((s0 - 3) * SEG, 2 * SEG), 2 * SEG).start()
        return carry

    lax.fori_loop(0, NSEG // 2 - 1, b_step, 0)
    if not ONLY:
        segment(NSEG - 1, 1, last=True)
    c_outb(S - 4 * SEG, 4 * SEG).start()
    c_outa.wait()
    c_outb(0, S).wait()


def pallas_concat_heads__sliding_local_dilated__memory_aug_recurrent_mem_tr__prompt_kernel(
    A_x, A_wqkv, A_wo, B_x, B_mem0, B_Wq, B_Wk, B_Wv, B_Wo, B_seg_len,
):
    assert B_seg_len == SEG
    assert A_x.shape == B_x.shape == (1, S, D) and B_mem0.shape == (1, M, D)
    assert B_Wq.shape == B_Wk.shape == B_Wv.shape == (D, H, DH) and B_Wo.shape == (H, DH, D)
    vmem, dma = pltpu.VMEM, pltpu.SemaphoreType.DMA
    call = pl.pallas_call(
        _kernel,
        out_shape=jax.ShapeDtypeStruct((S, 2 * D), BF16),
        in_specs=[pl.BlockSpec(memory_space=pl.ANY)] * 9,
        out_specs=pl.BlockSpec(memory_space=pl.ANY),
        scratch_shapes=[
            vmem((S, D), BF16),
            vmem((3, D, D), BF16),
            vmem((D, D), BF16),
            vmem((LT, D, 128), F32),
            vmem((3 * D // 2, D), U32),
            vmem((D // 2, D), U32),
            vmem((2, LT, TB, 128), F32),
            vmem((2, 2 * LT, HALO + TB, 128), F32),
            vmem((2, TB, D), F32),
            vmem((S, D), BF16),
            vmem((S, D), BF16),
            vmem((M, D), BF16),
            vmem((4 * NG, GW * 128, D), BF16),
            vmem((4 * NG, SLOTS, 64, 128), U32),
            vmem((2, LT, L, 128), F32),
            vmem((2, LT, L, 128), F32),
            vmem((2, LT, LT, L, 128), F32),
            vmem((2, LT, LT, L, 128), F32),
            vmem((2, LT, L, 128), F32),
            vmem((3, FT, 2, 16, 128), F32),
            vmem((2, FT, L, 128), F32),
            vmem((FT, L, 128), F32),
            vmem((3, LT, L, 128), F32),
            vmem((S, D), BF16),
            vmem((32, 128), F32), vmem((32, 128), F32), vmem((32, 128), F32),
            dma((4,)), dma((3,)), dma((4 * NG,)), dma((3,)), dma((2,)),
        ],
        compiler_params=pltpu.CompilerParams(vmem_limit_bytes=120 * 1024 * 1024),
        name="sliding_and_memory_attention",
    )

    def by_feature(w):
        return w.transpose(1, 2, 0).reshape(H * DH, D)

    out = call(A_x.reshape(S, D), A_wqkv, A_wo, B_x.reshape(S, D), B_mem0.reshape(M, D),
               by_feature(B_Wq), by_feature(B_Wk), by_feature(B_Wv), B_Wo.reshape(H * DH, D))
    return out.reshape(1, S, 2 * D)
```

```python
import contextlib
import functools
import math

import jax
import jax.numpy as jnp
from jax import lax
from jax.experimental import pallas as pl
from jax.experimental.pallas import tpu as pltpu


F32, BF16, U32 = jnp.float32, jnp.bfloat16, jnp.uint32
NT = (((1,), (1,)), ((), ()))
MASKED = -1000000000.0
LOG2E = math.log2(math.e)

S, D = 2048, 640
LT = D // 128

AH, AD, AW, ADIL = 32, 20, 8, 2
HALO = 16
TB = 128
NB = S // TB

H, DH, M, SEG = 32, 192, 8, 32
L = M + SEG
RG = L // 8
FT = H * DH // 128
NSEG = S // SEG
GW = 2 * LT
NG = pl.cdiv(FT, GW)
RING = 8

ONLY, AONLY, SCOPES = 0, 0, 0
OMEM, IMEM = 5, 1
LATE = 1
LAG_S, LAG_N, LAG_V, LAG_O = 30, 40, 30, 30
GAP_S, GAP_V = 12.5, 20.0
BACK_S, BACK_V, BACK_O = 28, 28, -1
TOK0, TOK1 = 60, 130
PK = 0
P0, P1, P2 = 7, 13, 38
AHEAD = 4
FLAGS = {"XLA_TPU_EVENLY_DISTRIBUTE_CRITICAL_NODES": True} if 1 else {}


def _stream(text):
    return [[("qkvo".index(w[0]), int(w[1])) for w in part.split("+")] for part in text.split(",")]


STREAM0 = _stream("q0,k0,v0,q1,k1,v1,q2,k2,v2,q3,k3,v3,q4,k4,v4,o0+o1,o2,o3,o4")
STREAM = _stream("q0,k0,q1,k1,v0,q2,k2,v1,q3,k3,v2,q4,k4,v3,v4,o0+o1+o2,o3+o4")
PARITY = {jg: k % 2 for k, jg in enumerate(jg for part in STREAM for jg in part)}


def _scope(name):
    return jax.named_scope(name) if SCOPES else contextlib.nullcontext()


class _Group:
    def __init__(self, n):
        k = n // 2
        self.n = n
        self.side = (range(k), range(k, n))
        self.label = list(range(k)) + list(range(LT - k, LT))
        self.mates = [[b for b in self.side[c < k] if self.label[b] != self.label[c]]
                      for c in range(n)]
        self.plain = [[i for i in range(LT) if i != self.label[c]
                       and i not in [self.label[b] for b in self.mates[c]]] for c in range(n)]
        keys = [(i, c) for c in range(n) for i in range(LT)]
        keys += [("other", c) for c in range(n)]
        keys += [("both", a, b) for a in self.side[0] for b in self.mates[a]]
        self.slot = {key: i for i, key in enumerate(keys)}
        for a in self.side[0]:
            for b in self.mates[a]:
                self.slot["both", b, a] = self.slot["both", a, b]


GROUPS = [_Group(min(GW, FT - g * GW)) for g in range(NG)]
SLOTS = max(GROUPS[0].slot.values()) + 1


def _pairs(j, g, ph):
    if (g >= OMEM) if j == 3 else (3 * g + j < IMEM):
        return {3: 1, 4: 2}
    if j < 3:
        return {0: 1, 4: 2} if (PARITY[j, g] + ph) % 2 else {0: 1, 3: 3, 4: 2}
    return {2: 2, 3: 0, 4: 1} if (PARITY[j, g] + ph) % 2 else {3: 0, 4: 1}


IN_PAIRS = sorted({p for j in range(3) for g in range(NG) for ph in range(2)
                   for p in _pairs(j, g, ph).items()})


def _ds(i, n):
    return pl.ds(i * n if isinstance(i, int) else pl.multiple_of(i * n, n), n)


def _dot(a, b):
    return jnp.dot(a, b, preferred_element_type=F32)


def _inverse(x):
    r = pl.reciprocal(x, approx=True)
    return r * (2.0 - x * r)


def _rows(parts):
    return parts[0] if len(parts) == 1 else jnp.concatenate(parts, axis=0)


def _group(r):
    return slice(8 * r, 8 * r + 8)


class _Sums:
    def __init__(self):
        self.sums = {}

    def add(self, key, t, minus=False):
        if key not in self.sums:
            self.sums[key] = t, minus
            return
        u, neg = self.sums[key]
        self.sums[key] = (u + t, neg) if neg == minus else (t - u if neg else u - t, False)

    def pop(self, key):
        t, neg = self.sums.pop(key)
        return -t if neg else t


class _Plan:
    def __init__(self, zero, main):
        self.zero = zero
        self.tasks = [(k - 1e-6, 0, task) for k, task in enumerate(main)]
        self.results = []

    def spread(self, tasks, k0, k1):
        step = (k1 - k0) / max(len(tasks), 1)
        self.tasks += [(k0 + n * step, step, task) for n, task in enumerate(tasks)]

    def run(self):
        for self.at, self.span, task in sorted(self.tasks, key=lambda x: x[0]):
            task(self)

    def result(self, t):
        self.results.append([t[r:r + 8] for r in range(0, t.shape[0], 8)])
        return self.results[-1]

    def paced(self, t, part=0.0, back=0):
        if self.zero is None or not 0 <= back < len(self.results):
            return t
        now = self.results[-1 - back]
        now = now[min(int((self.at % 1 + part * self.span) * len(now)), len(now) - 1)]
        return jnp.where(self.zero > 0, now if t.dtype == F32 else pltpu.bitcast(now, t.dtype), t)


def _task(fn, *args):
    return lambda plan: fn(plan, *args)


def _kernel(ax_hbm, awqkv_hbm, awo_hbm, bx_hbm, mem_hbm, wq_hbm, wk_hbm, wv_hbm, wo_hbm,
            out_hbm,
            ax, awqkv, awo, tmp, wqkv_p, wo_p, xw, qkv_s, oa_s, outa,
            bx, mem, raw, wt0, wt1, l_plain, l_sum, l_own, l_other, l_both, l_mate, scale,
            ahead, o_old, z_s, outb,
            sem_a, sem_x, sem_w, sem_b, sem_o, *more):
    y_s, o_s = more[:3 * NG], (more[3 * NG:4 * NG], more[4 * NG:])

    cp = pltpu.make_async_copy

    def rows_copy(src, dst, r0, r1, sem):
        return cp(src.at[pl.ds(r0, r1 - r0), :], dst.at[pl.ds(r0, r1 - r0), :], sem)

    c_wqkv = [cp(awqkv_hbm.at[:, pl.ds(j * D, D)], awqkv.at[j], sem_a.at[j]) for j in range(3)]
    c_awo = cp(awo_hbm, awo, sem_a.at[3])
    x_cuts = (0, 2 * TB, 6 * TB, S)
    c_ax = [rows_copy(ax_hbm, ax, x_cuts[c], x_cuts[c + 1], sem_x.at[c]) for c in range(3)]
    c_mem = rows_copy(mem_hbm, mem, 0, M, sem_b.at[0])
    c_bx0 = rows_copy(bx_hbm, bx, 0, 6 * SEG, sem_b.at[1])
    c_bx1 = rows_copy(bx_hbm, bx, 6 * SEG, S, sem_b.at[2])
    c_outa = cp(outa, out_hbm.at[:, pl.ds(0, D)], sem_o.at[0])

    def chunk(j, g):
        return 3 * g + j if j < 3 else 3 * NG + g

    def c_w(c):
        j, g = (c % 3, c // 3) if c < 3 * NG else (3, c - 3 * NG)
        n = GROUPS[g].n * 128
        return cp((wq_hbm, wk_hbm, wv_hbm, wo_hbm)[j].at[pl.ds(g * GW * 128, n), :],
                  raw.at[c % RING, pl.ds(0, n), :], sem_w.at[c])

    def c_outb(r0, n):
        return cp(outb.at[pl.ds(r0, n), :], out_hbm.at[pl.ds(r0, n), pl.ds(D, D)], sem_o.at[1])

    def start(copies):
        for c in copies:
            c.start()

    def wait(copies):
        with _scope("wait"):
            for c in copies:
                c.wait()

    def permute_rows(dst, base):
        for d in range(AD):
            for t in range(LT):
                dst[pl.ds((base + d * AH) // 2, AH // 2), t * 128:(t + 1) * 128] = pltpu.bitcast(
                    tmp[t, pl.ds(d, AH, stride=AD), :].astype(BF16), U32)

    def prep_wqkv(j):
        for t in range(LT):
            tmp[t] = awqkv[j, t * 128:(t + 1) * 128, :].astype(F32).T
        permute_rows(wqkv_p, j * D)

    def prep_wo():
        for t in range(LT):
            tmp[t] = awo[:, t * 128:(t + 1) * 128].astype(F32)
        permute_rows(wo_p, 0)

    def a_proj(i, b, j):
        def tile(plan, t):
            c = j * LT + t
            x = ax[_ds(i, TB), :] if isinstance(i, int) else pltpu.bitcast(xw[b], BF16)
            w = pltpu.bitcast(wqkv_p[c * 64:(c + 1) * 64, :], BF16)
            r = lax.dot_general(x, w, NT, preferred_element_type=F32)
            plan.result(r)
            qkv_s[b, c, HALO:HALO + TB, :] = r
            if j and isinstance(i, int) and i == 0:
                qkv_s[b, c, 0:HALO, :] = jnp.broadcast_to(r[0:1, :], (HALO, 128))
            elif j:
                qkv_s[b, c, 0:HALO, :] = qkv_s[1 - b, c, TB:TB + HALO, :]
        return [_task(tile, t) for t in range(LT)]

    def a_attention(b, first_block=False):
        state = {}

        def window(c, r0, w):
            lo = HALO + r0 - ADIL * w
            return qkv_s[b, c, lo:lo + 8, :]

        def logits(plan, r0):
            q = [plan.paced(window(t, r0, 0), t / LT) for t in range(LT)]
            state[r0] = []
            for w in range(AW):
                a = q[0] * window(LT, r0, w)
                for t in range(1, LT):
                    a = a + q[t] * window(LT + t, r0, w)
                state[r0].append(a + pltpu.roll(a, 2 * AH, 1))

        def fold(plan, r0):
            state[r0] = [a + pltpu.roll(a, AH, 1) for a in state[r0]]

        def weigh(plan, r0):
            lg = []
            for w, a in enumerate(state[r0]):
                if first_block and r0 < ADIL * w:
                    pos = lax.broadcasted_iota(jnp.int32, (8, 128), 0) + r0
                    a = jnp.where(pos >= ADIL * w, a, MASKED * AD ** 0.5)
                lg.append(a)
            m = functools.reduce(jnp.maximum, lg)
            state[r0] = [jnp.exp2((a - m) * (AD ** -0.5 * LOG2E)) for a in lg]

        def mix(plan, r0):
            e = [plan.paced(x, w / AW) for w, x in enumerate(state.pop(r0))]
            inv = _inverse(functools.reduce(jnp.add, e))
            for t in range(LT):
                o = e[0] * window(2 * LT + t, r0, 0)
                for w in range(1, AW):
                    o = o + e[w] * window(2 * LT + t, r0, w)
                oa_s[b, r0:r0 + 8, t * 128:(t + 1) * 128] = o * inv

        n = TB // 8
        return [_task(f, (k - lag) * 8) for k in range(n + 2)
                for lag, f in ((2, weigh), (0, logits), (1, fold), (2, mix)) if 0 <= k - lag < n]

    def a_out(i, b):
        def tile(plan, t):
            r = _dot(oa_s[b], pltpu.bitcast(wo_p[:, t * 128:(t + 1) * 128], BF16))
            plan.result(r)
            outa[_ds(i, TB), t * 128:(t + 1) * 128] = r.astype(BF16)
        return [_task(tile, t) for t in range(LT)]

    def tiles_of(c, odd=None, words=True):
        ref = (wt0, wt1)[c % 2 if odd is None else odd]
        return (ref.bitcast(U32) if PK and words else ref).at[c // 2]

    def w_transpose(c, grp, odd=None):
        def two(plan, i, f):
            t = pltpu.bitcast(raw[c % RING, f * 128:(f + 2) * 128, i * 128:(i + 1) * 128].T, U32)
            for k in range(2):
                tiles_of(c, odd)[grp.slot[i, f + k]] = t[:, k * 128:(k + 1) * 128]
        return [_task(two, i, f) for f in range(0, grp.n, 2) for i in range(LT)]

    def w_combine(c, grp, transposed=True, odd=None, zero=0):
        own, other = {}, {}

        def edge(plan, r, a, b):
            def tile(i, f, part=0.0):
                if transposed:
                    t = tiles_of(c + zero, odd)[grp.slot[i, f], _group(r)]
                else:
                    t = pltpu.bitcast(raw[c % RING, _ds(8 * f + r, 16), i * 128:(i + 1) * 128], U32)
                t = plan.paced(t, part)
                if not transposed and i != grp.label[f]:
                    tiles_of(c, odd)[grp.slot[i, f], _group(r)] = t
                return pltpu.bitcast(t, BF16).astype(F32)

            def put(key, t):
                if PK:
                    tiles_of(c + zero, odd, False)[grp.slot[key], _ds(r, 16)] = t.astype(BF16)
                else:
                    tiles_of(c + zero, odd)[grp.slot[key], _group(r)] = pltpu.bitcast(t.astype(BF16), U32)

            for f in (a, b):
                if f not in own:
                    own[f] = other[f] = tile(grp.label[f], f)
            ta, tb = tile(grp.label[b], a), tile(grp.label[a], b, 0.5)
            put(("both", a, b), ta + tb)
            own[a], other[a] = own[a] - ta, other[a] + tb
            own[b], other[b] = own[b] - tb, other[b] + ta
            for f, mate in ((a, b), (b, a)):
                if mate == grp.mates[f][-1]:
                    put((grp.label[f], f), own.pop(f))
                    put(("other", f), other.pop(f))
                    for i in grp.plain[f] * (not transposed):
                        tile(i, f)

        return [_task(edge, r, a, b) for r in range(8) for a in grp.side[0] for b in grp.mates[a]]

    full = 3 * (NG - 1)

    def a_step(it, carry):
        c = jnp.where(it == 1, RING - 2, 2 * it - 4)

        @pl.when(it == 2)
        def _():
            c_ax[2].wait()

        @pl.when(it > 1)
        def _():
            for k in range(2, NB // 2):
                @pl.when(it == k)
                def _():
                    start([c_w(2 * k - 4 + b + AHEAD) for b in range(2)])
            wait([cp(raw.at[(c + b) % RING], raw.at[(c + b) % RING], sem_w.at[c + b])
                  for b in range(2)])

        zero = lax.shift_right_logical(it, 16)
        plan = _Plan(zero, a_out(jnp.where(it == 1, 1, 2 * it - 3), 1) + a_out(2 * it - 2, 0) + [
            t for b in range(2) for j in range(3) for t in a_proj(2 * it + b, b, j)])
        for b in range(2):
            before = jnp.where(c + b == 0, full - 1, c + b - 1)
            plan.spread(w_combine(before, GROUPS[0], True, 1 - b), P0 * b, P0 * (b + 1))
            plan.spread(w_transpose(c + b, GROUPS[0], b), P0 * b, P0 * (b + 1))
        plan.spread(a_attention(1), P1, 24.99)
        plan.spread(a_attention(0), 24.99, P2)
        plan.run()
        for b in range(2):
            xw[b] = pltpu.bitcast(ax[_ds(jnp.minimum(2 * it + 2 + b, NB - 1), TB), :], U32)
        return zero

    if not ONLY:
        start([c_wqkv[0], c_ax[0], c_wqkv[1]])
        c_wqkv[0].wait()
        c_wqkv[2].start()
        prep_wqkv(0)
        wait([c_ax[0], c_wqkv[1]])
        start([c_ax[1], c_awo])
        _Plan(None, a_proj(0, 0, 0) + a_proj(1, 1, 0)).run()
        prep_wqkv(1)
        c_wqkv[2].wait()
        _Plan(None, a_proj(0, 0, 1) + a_proj(1, 1, 1)).run()
        prep_wqkv(2)
        wait([c_ax[1], c_awo])
        start([c_ax[2], c_w(0)])
        _Plan(None, a_proj(0, 0, 2) + a_proj(1, 1, 2) + a_attention(0, True)).run()
        prep_wo()
        for b in range(2):
            xw[b] = pltpu.bitcast(ax[_ds(2 + b, TB), :], U32)
        start([c_w(c) for c in range(1, AHEAD)] + [c_mem, c_bx0])
        with _scope("a_loop"):
            nil = lax.fori_loop(1, NB // 2, a_step, 0)
        start([c_w(c) for c in range(full + AHEAD, 4 * NG)])
        wait([c_mem, c_bx0] + [c_w(full + j) for j in range(3)])
        plan = _Plan(nil, a_out(NB - 3, 1) + a_out(NB - 2, 0))
        plan.spread(w_combine(full - 1, GROUPS[0]), 0, 9)
        plan.spread([t for j in (0, 2) for t in w_transpose(full + j, GROUPS[-1])], 0, 9)
        plan.run()

    def binade(tiles):
        top = jnp.max(functools.reduce(jnp.maximum, map(jnp.abs, tiles)), axis=1, keepdims=True)
        top = jnp.clip(jnp.broadcast_to(top, (8, 128)), 2.0 ** -60, 2.0 ** 60)
        return pltpu.bitcast(top, jnp.int32) & 0x7F800000

    def memory_operands(ph, known, i, t):
        known[i] = t
        l_plain[ph, i, 0:M] = t
        for k, u in known.items():
            if k != i:
                l_sum[ph, min(i, k), max(i, k), 0:M] = t + u

    def memory_pair(plan, ph):
        n = IN_PAIRS.index((0, 1))
        cur = [l_plain[ph, i, 0:M] for i in range(LT)]
        shift = binade(cur) - pltpu.bitcast(l_mate[ph, LT], jnp.int32)
        down, up = [pltpu.bitcast(x, F32) for x in (0x3F800000 + shift, 0x3F800000 - shift)]
        scale[ph, 0], scale[ph, 1] = down, up
        for k in range(LT):
            mate = l_mate[ph, k] * down
            l_other[ph, 0, n, k] = cur[k] - mate
            l_other[1 - ph, 1, n, k] = l_mate[ph, k] - cur[k] * up
            for i in range(LT):
                if i != k:
                    l_both[ph, n, i, k] = cur[i] + mate

    def token_operands(s, ph, first=False):
        def tokens(plan, ds, r):
            seg = s + ds if isinstance(s, int) else jnp.minimum(s + ds, NSEG - 1)
            rows = _ds(2 * seg + (r - 1) // 2, 16)
            return [pltpu.bitcast(plan.paced(pltpu.bitcast(bx[rows, i * 128:(i + 1) * 128], U32)),
                                  BF16).astype(F32)[_group((r - 1) % 2)] for i in range(LT)]

        state = {}

        def current(plan, r, i):
            if i == 0:
                state[0] = tokens(plan, 0, r)
            t = l_plain[ph, i, _group(r)] = plan.paced(state[0][i])
            for k in range(i + 1, LT):
                l_sum[ph, i, k, _group(r)] = t + state[0][k]

        def later(plan, r):
            for i, t in enumerate(tokens(plan, 2, r)):
                l_own[ph, i, _group(r)] = t
            for i, t in enumerate(tokens(plan, 1, r) * first):
                l_own[1 - ph, i, _group(r)] = t

        def after(plan, n, k):
            r0, r1 = IN_PAIRS[n]
            if k == 0:
                state[1] = tokens(plan, 1, r1)
            mate = plan.paced(state[1][k])
            if r0 == 0:
                l_mate[ph, k] = mate
                if k == 0:
                    l_mate[ph, LT] = pltpu.bitcast(binade(state[1]), F32)
                return
            l_other[ph, 0, n, k] = state[0][k] - mate
            for i in range(LT):
                if i != k:
                    l_both[ph, n, i, k] = state[0][i] + mate

        def before(plan, n):
            for i, t in enumerate(tokens(plan, -1, IN_PAIRS[n][0])):
                l_other[ph, 1, n, i] = state[0][i] - t

        tasks = [_task(later, r) for r in sorted({r1 for _, r1 in IN_PAIRS})]
        for r in range(RG):
            tasks += [_task(current, r, i) for i in range(LT * (r > 0))]
            for n, (r0, r1) in enumerate(IN_PAIRS):
                tasks += [_task(after, n, k) for k in range(LT * (r0 == r))]
                tasks += [_task(before, n)] * (r1 == r and r0 > 0 and not first)
        return tasks

    def segment(s, ph, zero, first=False, last=False):
        live = range(1 if last else 0, RG)
        pieces = {}

        def product(plan, parts, j, g, key):
            w = tiles_of(chunk(j, g))[GROUPS[g].slot[key]]
            return plan.result(_dot(_rows(parts), pltpu.bitcast(w, BF16)))

        def project(j, g):
            grp, f0 = GROUPS[g], g * GW
            lab = grp.label
            every = live if j == 0 else range(RG)
            to_next = {} if last else _pairs(j, g, ph)
            from_prev = {} if first else {r1: r0 for r0, r1 in _pairs(j, g, 1 - ph).items()}
            future = () if last else tuple(_pairs(j, g, 1 - ph).values())
            early = [r for r in every if r not in from_prev]
            y, gift, places = _Sums(), _Sums(), []
            owed = {a: 1 + len(grp.mates[a]) for a in grp.side[ph]}
            left = {f: LT + len(grp.mates[f]) * (f not in owed) for f in range(grp.n)}

            def plain(i, r):
                return l_plain[ph, i, _group(r)]

            def take(f, rows, res, minus=False):
                for r, t in zip(rows, res):
                    y.add((f, r), t, minus)
                left[f] -= 1
                if not left[f] or minus:
                    signs = {}
                    for r in every:
                        if (f, r) in y.sums:
                            t, signs[r] = y.sums.pop((f, r))
                            y_s[chunk(j, g)][0, len(places), _group(r)] = t
                    pieces.setdefault((j, f0 + f), []).append((len(places), signs))
                    places.append(f)

            def give(a, res):
                for r, t in zip(early, res):
                    if r in to_next:
                        gift.add((a, r), t)
                owed[a] -= 1
                for r0, r1 in to_next.items() if not owed[a] else ():
                    t = gift.pop((a, r0))
                    ahead[j, f0 + a, 0, _group(r1 - 1)] = t if r0 else t * scale[ph, 1]

            def own(plan, a):
                parts = [plain(lab[a], r) for r in early]
                parts += [l_own[ph, lab[a], _group(r)] for r in future]
                res = product(plan, parts, j, g, (lab[a], a))
                for r in from_prev:
                    y.add((a, r), ahead[j, f0 + a, 1, _group(r - 1)])
                for r, t in zip(future, res[len(early):]):
                    ahead[j, f0 + a, 1, _group(r - 1)] = t
                take(a, early, res)
                give(a, res)

            def opening(plan, b):
                parts = [l_own[1 - ph, lab[b], _group(r)] for r in to_next.values()]
                for r, t in zip(to_next.values(), product(plan, parts, j, g, (lab[b], b))):
                    ahead[j, f0 + b, 1, _group(r - 1)] = t

            def other(plan, b):
                parts = [l_other[ph, 0, IN_PAIRS.index((r, to_next[r])), lab[b]] if r in to_next else
                         l_other[ph, 1, IN_PAIRS.index((from_prev[r], r)), lab[b]] if r in from_prev
                         else plain(lab[b], r) for r in every]
                res = product(plan, parts, j, g, ("other", b))
                for r in from_prev:
                    y.add((b, r), ahead[j, f0 + b, 0, _group(r - 1)])
                for r0, r1 in to_next.items():
                    t = ahead[j, f0 + b, 1, _group(r1 - 1)]
                    y.add((b, r0), t if r0 else plan.paced(t, 0, 1) * scale[ph, 0])
                take(b, every, res)

            def both(plan, a, b):
                parts = [l_both[ph, IN_PAIRS.index((r, to_next[r])), lab[a], lab[b]]
                         if r in to_next else plain(lab[a], r) for r in early]
                res = product(plan, parts, j, g, ("both", a, b))
                take(b, early, res)
                give(a, res)

            def cross(plan, a, b):
                i, k = sorted((lab[a], lab[b]))
                res = product(plan, [l_sum[ph, i, k, _group(r)] for r in every], j, g, (lab[b], a))
                take(a, every, res)
                take(b, every, res, True)

            def single(plan, i, f):
                take(f, every, product(plan, [plain(i, r) for r in every], j, g, (i, f)))

            passes = []
            others = list(grp.side[1 - ph])
            for a, b0 in zip(grp.side[ph], others[grp.n == GW:] + others):
                passes += [((), _task(opening, b0))] * first
                passes += [((lab[a],), _task(own, a)), ((lab[b0],), _task(other, b0))]
                passes += [((i,), _task(single, i, f)) for f in (a, b0) for i in grp.plain[f]]
                passes += [((lab[a],), _task(both, a, b)) for b in grp.mates[a]]
                passes += [((lab[a], lab[b]), _task(cross, a, b)) for b in grp.mates[a]]
            return passes

        n = 8 * len(live)
        key = lax.broadcasted_iota(jnp.int32, (L, 2 * n), 0)
        col = lax.broadcasted_iota(jnp.int32, (L, 2 * n), 1)
        head0 = col < n
        query = jnp.where(head0, col, col - n) + (L - n)
        visible = (query < M) | (query >= key)
        scores, probs = _Sums(), {}

        def tile(plan, j, f, back):
            t = _Sums()
            for place, signs in pieces[j, f]:
                for r, minus in signs.items():
                    u = y_s[chunk(j, f // GW)][zero, place, _group(r)]
                    t.add(r, u if r in t.sums else plan.paced(u, 0, back - r), minus)
            return _rows([t.pop(r) for r in sorted(t.sums)])

        def by_head(t, f, short=False):
            low = lax.broadcasted_iota(jnp.int32, t.shape, 1) < 64
            if f % 3 == 1:
                return _rows([jnp.where(low, t, 0.0), jnp.where(low, 0.0, t)]).astype(BF16)
            if f % 3 == 0 and short:
                return t.astype(BF16)
            return _rows([t, jnp.zeros_like(t)][::1 - f % 3]).astype(BF16)

        def score(plan, f):
            q = by_head(tile(plan, 0, f, BACK_S + 6 * (BACK_S > 0)), f)
            scores.add(f // 3, lax.dot_general(tile(plan, 1, f, BACK_S), q, NT,
                                               preferred_element_type=F32))
            if f % 3 == 2:
                sc = jnp.where(visible, scores.pop(f // 3), MASKED * DH ** 0.5)
                e = jnp.exp2((sc - jnp.max(sc, axis=0, keepdims=True)) * (DH ** -0.5 * LOG2E))
                p = e * _inverse(jnp.sum(e, axis=0, keepdims=True))
                probs[f // 3] = _rows([jnp.where(head0, p, 0.0), jnp.where(head0, 0.0, p)]).T

        def mix(plan, f):
            p = probs[f // 3]
            p = (p[0:n, 0:L], p[0:n] + p[n:], p[n:])[f % 3]
            res = _dot(p, by_head(tile(plan, 2, f, BACK_V), f, True))
            g = f // GW
            for k, r in enumerate(live):
                o_s[ph][g][0, f % GW, _group(r)] = res[_group(k)]
                for r0, r1 in _pairs(3, g, 1 - ph).items():
                    if r1 == r and not first and f % GW in GROUPS[g].side[1 - ph]:
                        o_old[f, _group(r0)] = (res[_group(k)]
                                                + o_s[1 - ph][g][zero, f % GW, _group(r0)])

        z = _Sums()

        def out_passes(g, passes):
            grp, f0 = GROUPS[g], g * GW
            lab = grp.label
            to_next = {} if last else _pairs(3, g, ph)
            from_prev = {} if first else {r1: r0 for r0, r1 in _pairs(3, g, 1 - ph).items()}
            late = [r for r in live if r not in to_next]
            old = () if first else tuple(_pairs(3, g, ph))

            def cur(f, r):
                return o_s[ph][g][zero, f, _group(r)]

            def prev(f, r):
                return o_s[1 - ph][g][zero, f, _group(from_prev[r])]

            def joined(plan, f, a):
                return [plan.paced(cur(f, r), 0, BACK_O - r) + prev(a, r) if r in from_prev
                        else cur(f, r) for r in late]

            def own(plan, a):
                parts = joined(plan, a, a) + [o_old[f0 + a, _group(r)] for r in old]
                to = [((0, lab[a], r),) for r in late] + [((2, lab[a], r),) for r in old]
                return zip(to, product(plan, parts, 3, g, (lab[a], a)))

            def other(plan, b):
                to = [((0, lab[b], r),) + ((1, lab[b], from_prev.get(r), True),) * (r in from_prev)
                      + ((-1, lab[b], to_next.get(r)),) * (r in to_next) for r in live]
                return zip(to, product(plan, [cur(b, r) for r in live], 3, g, ("other", b)))

            def closing(plan, b):
                parts = [o_old[f0 + b, _group(r0)] if r1 in live else prev(b, r1)
                         for r1, r0 in from_prev.items()]
                to = [((1, lab[b], r),) for r in from_prev.values()]
                return zip(to, product(plan, parts, 3, g, (lab[b], b)))

            def both(plan, a, b):
                alone = [r for r in from_prev if r not in live]
                to = [((0, lab[a], r),) * (r in live)
                      + ((1, lab[b], from_prev.get(r)),) * (r in from_prev) for r in late + alone]
                parts = joined(plan, b, a) + [prev(a, r) for r in alone]
                return zip(to, product(plan, parts, 3, g, ("both", a, b)))

            def cross(plan, a, b):
                i, k = sorted((lab[a], lab[b]))
                parts = [plan.paced(cur(a, r), 0, BACK_O - r) - cur(b, r) for r in live]
                return zip([((0, i, r), (0, k, r)) for r in live],
                           product(plan, parts, 3, g, (lab[b], a)))

            def single(plan, i, f):
                parts = [cur(f, r) for r in live]
                return zip([((0, i, r),) for r in live], product(plan, parts, 3, g, (i, f)))

            def add(i, k, kind, *task):
                passes.setdefault((min(i, k), max(i, k), kind, i), []).append(_task(*task))

            for a, b in zip(grp.side[ph], grp.side[1 - ph]):
                add(lab[a], lab[a], 0, own, a)
                add(lab[b], lab[b], 0, other, b)
                if last:
                    add(lab[b], lab[b], 0, closing, b)
                for f in (a, b):
                    for i in grp.plain[f]:
                        add(i, i, 0, single, i, f)
                for b in grp.mates[a]:
                    add(lab[a], lab[b], 1, both, a, b)
                    add(min(lab[a], lab[b]), max(lab[a], lab[b]), 2, cross, a, b)

        def out_project(groups):
            passes, part = {}, _Sums()
            for g in groups:
                out_passes(g, passes)

            def run(plan, task, flush):
                for to, t in task(plan):
                    part.add(to, t)
                for to in list(part.sums) * flush:
                    t = part.pop(to)
                    for key in to:
                        z.add(key[:3], t, len(key) > 3)

            return [((lo, hi) if kind == 2 else (i,), _task(run, task, task is tasks[-1]))
                    for (lo, hi, kind, i), tasks in sorted(passes.items(), key=lambda x: x[0])
                    for task in tasks]

        main, begin, done = [], {}, {}
        parts = STREAM0 if first else STREAM
        for part in parts:
            new = out_project([g for _, g in part]) if part[0][0] == 3 else project(*part[0])
            if part is parts[0] and not first:
                new.sort(key=lambda x: max(max(x[0]), LT - 1 - LATE))
            if part is parts[-1]:
                new.sort(key=lambda x: max(min(x[0]), LT - 1 - LATE))
            begin.update({jg: len(main) for jg in part})
            main += new
            done.update({jg: len(main) for jg in part})
        plan = _Plan(zero, [task for _, task in main])

        ready = {}
        for stage, gap, windows in (
                (score, GAP_S, lambda f: (max(done[j, f // GW] for j in range(2)) + LAG_S,
                                          begin[3, f // 3 * 3 // GW] - LAG_O - LAG_N)),
                (mix, GAP_V, lambda f: (max(done[2, f // GW] + LAG_V, ready[f // 3] + LAG_N),
                                        begin[3, f // GW] - LAG_O))):
            at = -gap
            for f in range(FT):
                step = min([gap] + [(windows(k)[1] - at) / (k - f + 1) for k in range(f, FT)])
                at = max(at + max(step, 0.01), windows(f)[0])
                assert at < begin[3, f // GW] - 1
                plan.spread([_task(stage, f)], at, at)
                if stage is score:
                    ready[f // 3] = at

        if first:
            def arrive(plan, c):
                wait([c_w(c)])

            def combine(j, g, k0, k1):
                c = chunk(j, g)
                plan.spread(w_combine(c, GROUPS[g], j < 3, c % 2), k0, k1)

            plan.spread(a_attention(1), 0, 200)
            plan.spread(a_out(NB - 1, 1), 240, 240.5)
            plan.spread(w_transpose(full + 1, GROUPS[-1]), 200, 300)
            for k, j in enumerate((0, 2, 1)):
                combine(j, NG - 1, 200 + 110 * k, 310 + 110 * k)
            ends = [530, (530 + begin[3, 0] - 10) // 2, begin[3, 0] - 10]
            ends += [begin[3, g] - 0.5 for g in range(2, NG)]
            for g in range(NG):
                plan.spread([_task(arrive, chunk(3, g))], ends[g], ends[g])
                combine(3, g, ends[g], ends[g + 1])
        if not last:
            k0 = begin[3, 0] if first else TOK0
            plan.spread(token_operands(s + 1, 1 - ph), k0, k0 + TOK1 - TOK0)
            plan.spread([_task(memory_pair, ph)] * ((0, 1) in IN_PAIRS), 1, 1)
            known = {}
            for i in range(LT):
                at = max(k for k, (tiles, _) in enumerate(main) if i in tiles)
                plan.spread([lambda _, i=i: memory_operands(1 - ph, known, i, z.pop((0, i, 0)))],
                            at, at)
        for i in range(LT * (not first)):
            for r in range(1, RG):
                z.add((2, i, r), z_s[ph, i, _group(r)])
                z.add((1, i, r), z_s[1 - ph, i, _group(r)])
            for r in sorted({r1 for g in range(NG) for r1 in _pairs(3, g, 1 - ph).values()}):
                if r in live:
                    z.add((0, i, r), z_s[2, i, _group(r)], True)
        plan.run()

        for back in (2, 1, 0) if last else (2,) * (not first):
            seg = s - back if isinstance(s, int) else jnp.maximum(s - back, 0)
            for i in range(LT):
                outb[_ds(seg, SEG), i * 128:(i + 1) * 128] = _rows(
                    [z.pop((back, i, r)) for r in range(1, RG)]).astype(BF16)
        for back, i, r in list(z.sums):
            z_s[2 if back < 0 else (ph + back) % 2, i, _group(r)] = z.pop((back, i, r))

    if AONLY:
        c_outa.start()
        wait([c_outa] + [c_w(c) for c in range(full + 3, 4 * NG)])
        outb[0:128, 0:128] = pltpu.bitcast(tiles_of(nil, 0)[nil] + tiles_of(nil, 1)[nil], BF16)
        c_outb(0, S).start()
        c_outb(0, S).wait()
        return
    if not ONLY:
        _Plan(None, token_operands(0, 0, first=True)).run()
        known = {}
        for i in range(LT):
            memory_operands(0, known, i, mem[0:M, i * 128:(i + 1) * 128].astype(F32))
        segment(0, 0, nil, first=True)
    start([c_bx1, c_outa])

    def b_step(it, carry):
        @pl.when(it == 1)
        def _():
            c_bx1.wait()
        zero = lax.shift_right_logical(it, 16)
        segment(1 + 2 * it, 1, zero)
        segment(2 + 2 * it, 0, zero)

        @pl.when(it > 0)
        def _():
            c_outb(pl.multiple_of((it - 1) * 2 * SEG, 2 * SEG), 2 * SEG).start()
        return zero

    with _scope("b_loop"):
        nil = lax.fori_loop(0, NSEG // 2 - 1, b_step, 0)
    if not ONLY:
        segment(NSEG - 1, 1, nil, last=True)
    c_outb(S - 4 * SEG, 4 * SEG).start()
    wait([c_outa, c_outb(0, S)])


def pallas_concat_heads__sliding_local_dilated__memory_aug_recurrent_mem_tr__prompt_kernel(
    A_x, A_wqkv, A_wo, B_x, B_mem0, B_Wq, B_Wk, B_Wv, B_Wo, B_seg_len,
):
    assert B_seg_len == SEG
    assert A_x.shape == B_x.shape == (1, S, D) and B_mem0.shape == (1, M, D)
    assert B_Wq.shape == B_Wk.shape == B_Wv.shape == (D, H, DH) and B_Wo.shape == (H, DH, D)
    dma = pltpu.SemaphoreType.DMA

    def vmem(dtype, *shape):
        assert math.prod(shape) * jnp.dtype(dtype).itemsize % 16384 == 0, shape
        return pltpu.VMEM(shape, dtype)

    call = pl.pallas_call(
        _kernel,
        out_shape=jax.ShapeDtypeStruct((S, 2 * D), BF16),
        in_specs=[pl.BlockSpec(memory_space=pl.ANY)] * 9,
        out_specs=pl.BlockSpec(memory_space=pl.ANY),
        scratch_shapes=[
            vmem(BF16, S, D),
            vmem(BF16, 3, D, D),
            vmem(BF16, D, D),
            vmem(F32, LT, D, 128),
            vmem(U32, 3 * D // 2, D),
            vmem(U32, D // 2, D),
            vmem(U32, 2, TB // 2, D),
            vmem(F32, 2, 3 * LT, HALO + TB, 128),
            vmem(F32, 2, TB, D),
            vmem(BF16, S, D),
            vmem(BF16, S, D),
            vmem(BF16, 64, D),
            vmem(BF16, RING, GW * 128, D),
            *[vmem(BF16, 2 * NG, SLOTS, 128, 128) if PK else vmem(U32, 2 * NG, SLOTS, 64, 128)] * 2,
            vmem(F32, 2, LT + 1, L, 128),
            vmem(F32, 2, LT - 1, LT, L, 128),
            vmem(F32, 2, LT + 1, L, 128),
            vmem(F32, 2, 2, 4, LT, 8, 128),
            vmem(F32, 2, 4, LT, LT, 8, 128),
            vmem(F32, 2, LT + 1, 8, 128),
            vmem(F32, 2, 2, 8, 128),
            vmem(F32, 3, FT, 2, 24, 128),
            vmem(F32, FT, L, 128),
            vmem(F32, 4, LT, L, 128),
            vmem(BF16, S, D),
            dma((4,)), dma((3,)), dma((4 * NG,)), dma((3,)), dma((2,)),
            *[vmem(F32, 1, 28, L, 128)] * (3 * NG),
            *[vmem(F32, 1, 12, L, 128)] * (2 * NG),
        ],
        compiler_params=pltpu.CompilerParams(vmem_limit_bytes=120 * 1024 * 1024, flags=FLAGS),
        name="sliding_and_memory_attention",
    )

    def by_feature(w):
        return w.transpose(1, 2, 0).reshape(H * DH, D)

    out = call(A_x.reshape(S, D), A_wqkv, A_wo, B_x.reshape(S, D), B_mem0.reshape(M, D),
               by_feature(B_Wq), by_feature(B_Wk), by_feature(B_Wv), B_Wo.reshape(H * DH, D))
    return out.reshape(1, S, 2 * D)
```

```python
import contextlib
import functools
import math

import jax
import jax.numpy as jnp
from jax import lax
from jax.experimental import pallas as pl
from jax.experimental.pallas import tpu as pltpu


F32, BF16, U32 = jnp.float32, jnp.bfloat16, jnp.uint32
NT = (((1,), (1,)), ((), ()))
MASKED = -1000000000.0
LOG2E = math.log2(math.e)

S, D = 2048, 640
LT = D // 128

AH, AD, AW, ADIL = 32, 20, 8, 2
HALO = 16
TB = 128
NB = S // TB

H, DH, M, SEG = 32, 192, 8, 32
L = M + SEG
RG = L // 8
FT = H * DH // 128
NSEG = S // SEG
GW = 2 * LT
NG = pl.cdiv(FT, GW)
RING = 8

ONLY, AONLY, SCOPES = 0, 0, 0
OMEM, IMEM = 5, 1
LATE = 1
LAG_S, LAG_N, LAG_V, LAG_O = 36, 68, 34, 26
GAP_S, GAP_V = 10.0, 10.0
BACK_S, BACK_V, BACK_O = 28, 28, -1
TOK0, TOK1 = 800, 900
STEP = "gdc"
DS, OMIX = 1, 4
GSPAN = 10
EP, HP, NZ = 1, 0, 3
JIT = {(k // (2 * FT), k // FT % 2, k % FT): ord(c) - ord("e") for k, c in enumerate("")}
DYN, ALT, BACK_P = 1, 4, 24
FOLD0, FOLD1 = 30, 130
P0, P1, P2 = 8.0, 15.5, 39
S0, S1 = 9, 9
EARLY = 1
R0, R1 = 13, 23
FLAGS = {"XLA_TPU_EVENLY_DISTRIBUTE_CRITICAL_NODES": True} if 1 else {}


def _stream(text):
    return [[("qkvo".index(w[0]), int(w[1])) for w in part.split("+")] for part in text.split(",")]


STREAM0 = _stream("q0,k0,v0,q1,k1,v1,q2,k2,v2,q3,k3,v3,q4,k4,v4,o0+o1,o2+o3+o4")
Q = [int(k) for k in "0,360,640".split(",")]
PRIO = 1
W1, HEAD = 2, 0
STREAM = _stream("q0,k0+v0,q1+k1,v1+q2,k2+v2,q3+k3,q4+k4,v3+v4,o0+o1+o2,o3+o4")
PARITY = {jg: k % 2 for k, jg in enumerate(jg for part in STREAM for jg in part)}


def _scope(name):
    return jax.named_scope(name) if SCOPES else contextlib.nullcontext()


class _Group:
    def __init__(self, n):
        k = n // 2
        self.n = n
        self.side = (range(k), range(k, n))
        self.label = list(range(k)) + list(range(LT - k, LT))
        self.mates = [[b for b in self.side[c < k] if self.label[b] != self.label[c]]
                      for c in range(n)]
        self.plain = [[i for i in range(LT) if i != self.label[c]
                       and i not in [self.label[b] for b in self.mates[c]]] for c in range(n)]
        keys = [(i, c) for c in range(n) for i in range(LT)]
        keys += [("other", c) for c in range(n)]
        keys += [("both", a, b) for a in self.side[0] for b in self.mates[a]]
        self.slot = {key: i for i, key in enumerate(keys)}
        for a in self.side[0]:
            for b in self.mates[a]:
                self.slot["both", b, a] = self.slot["both", a, b]


GROUPS = [_Group(min(GW, FT - g * GW)) for g in range(NG)]
SLOTS = max(GROUPS[0].slot.values()) + 1


def _pairs(j, g, ph):
    if (g >= OMEM) if j == 3 else (3 * g + j < IMEM):
        return {3: 1, 4: 2}
    if j < 3:
        return {0: 1, 4: 2} if (PARITY[j, g] + ph) % 2 else {0: 1, 3: 3, 4: 2}
    return {2: 2, 3: 0, 4: 1} if (PARITY[j, g] + ph) % 2 else {3: 0, 4: 1}


IN_PAIRS = sorted({p for j in range(3) for g in range(NG) for ph in range(2)
                   for p in _pairs(j, g, ph).items()})


def _out_passes(groups, ph, first=False, last=False):
    passes = {}
    live = range(1 if last else 0, RG)
    for g in groups:
        grp = GROUPS[g]
        lab = grp.label
        to_next = {} if last else _pairs(3, g, ph)
        from_prev = {} if first else {r1: r0 for r0, r1 in _pairs(3, g, 1 - ph).items()}
        late = [r for r in live if r not in to_next]

        def add(i, k, kind, key, rows):
            passes.setdefault((min(i, k), max(i, k), kind, i), []).append((g, key, rows))

        def mate(key, r):
            return ((1, *key, from_prev[r]),) if r in from_prev else ()

        for a, b in zip(grp.side[ph], grp.side[1 - ph]):
            i, k = lab[a], lab[b]
            add(i, i, 0, (i, a), [(((0, a, r),) + mate([a], r), ((0, i, r),)) for r in late]
                + [(((2, a, r),), ((2, i, r),)) for r in _pairs(3, g, ph) if not first])
            add(k, k, 0, ("other", b), [
                (((0, b, r),), ((0, k, r),) + tuple((*x, True) for x in mate([k], r))
                 + ((-1, k, to_next.get(r)),) * (r in to_next)) for r in live])
            if last:
                add(k, k, 0, (k, b), [(((3 if r1 else 1, b, r0),), ((1, k, r0),))
                                     for r1, r0 in from_prev.items()])
            for f in (a, b):
                for k in grp.plain[f]:
                    add(k, k, 0, (k, f), [(((0, f, r),), ((0, k, r),)) for r in live])
            for b in grp.mates[a]:
                k = lab[b]
                add(i, k, 1, ("both", a, b), [
                    (((0, b, r),) * (r in live) + mate([a], r),
                     ((0, i, r),) * (r in live) + mate([k], r))
                    for r in sorted({*late, *from_prev})])
                add(min(i, k), max(i, k), 2, (k, a), [
                    (((0, a, r), (0, b, r, True)), ((0, min(i, k), r), (0, max(i, k), r)))
                    for r in live])
    return sorted(passes.items())


def _parts(ph):
    keys = [(part[0][1], kind, to) for part in STREAM if part[0][0] == 3
            for kind, passes in _out_passes([g for _, g in part], ph)
            for _, _, rows in passes for _, to in rows]
    if ph == 0:
        keys += [(None, None, ((back, i, r),)) for i in range(LT)
                 for back, rows in ((0, range(1, RG)), (-1, _carried(ph))) for r in rows]
    return {key: n for n, key in enumerate(dict.fromkeys(keys))}


def _carried(ph):
    return sorted({r for g in range(NG) for r in _pairs(3, g, ph).values()})


PARTS = _parts(0), _parts(1)


def _ds(i, n):
    return pl.ds(i * n if isinstance(i, int) else pl.multiple_of(i * n, n), n)


def _dot(a, b):
    return jnp.dot(a, b, preferred_element_type=F32)


def _inverse(x):
    r = pl.reciprocal(x, approx=True)
    return r * (2.0 - x * r)


def _rows(parts):
    return parts[0] if len(parts) == 1 else jnp.concatenate(parts, axis=0)


def _group(r):
    return slice(8 * r, 8 * r + 8)


class _Sums:
    def __init__(self):
        self.sums = {}

    def add(self, key, t, minus=False):
        if key not in self.sums:
            self.sums[key] = t, minus
            return
        u, neg = self.sums[key]
        self.sums[key] = (u + t, neg) if neg == minus else (t - u if neg else u - t, False)

    def pop(self, key):
        t, neg = self.sums.pop(key)
        return -t if neg else t


class _Plan:
    def __init__(self, zero, main):
        self.zero = zero
        self.tasks = [(k - 1e-6, 0, task) for k, task in enumerate(main)]
        self.results = []

    def spread(self, tasks, k0, k1):
        step = (k1 - k0) / max(len(tasks), 1)
        self.tasks += [(k0 + n * step, step, task) for n, task in enumerate(tasks)]

    def run(self):
        for self.at, self.span, task in sorted(self.tasks, key=lambda x: x[0]):
            task(self)

    def result(self, t):
        self.results.append([t[r:r + 8] for r in range(0, t.shape[0], 8)])
        return self.results[-1]

    def paced(self, t, part=0.0, back=0):
        if self.zero is None or not 0 <= back < len(self.results):
            return t
        now = self.results[-1 - back]
        now = now[min(int((self.at % 1 + part * self.span) * len(now)), len(now) - 1)]
        return jnp.where(self.zero > 0, now if t.dtype == F32 else pltpu.bitcast(now, t.dtype), t)


def _task(fn, *args):
    return lambda plan: fn(plan, *args)


def _kernel(ax_hbm, awqkv_hbm, awo_hbm, bx_hbm, mem_hbm, wq_hbm, wk_hbm, wv_hbm, wo_hbm,
            out_hbm,
            ax, awqkv, awo, tmp, aw, xw, qkv_s, oa_s, outa,
            bx, mem, raw, wt, l_tok, l_mem, ahead, y_s, p_s, qkv, o_s, o_old, z_part, z_s, outb,
            sem_a, sem_x, sem_w, sem_b, sem_o):

    cp = pltpu.make_async_copy

    def rows_copy(src, dst, r0, r1, sem):
        return cp(src.at[pl.ds(r0, r1 - r0), :], dst.at[pl.ds(r0, r1 - r0), :], sem)

    c_wqkv = [cp(awqkv_hbm.at[:, pl.ds(j * D, D)], awqkv.at[j], sem_a.at[j]) for j in range(3)]
    c_awo = cp(awo_hbm, awo, sem_a.at[3])
    x_cuts = (0, 2 * TB, 3 * TB, 11 * TB, S, 7 * TB)
    c_ax = [rows_copy(ax_hbm, ax, x_cuts[c], x_cuts[c + 1], sem_x.at[c]) for c in range(4)]
    c_ax[2] = rows_copy(ax_hbm, ax, 7 * TB, 11 * TB, sem_x.at[2])
    c_ax.append(rows_copy(ax_hbm, ax, 3 * TB, 7 * TB, sem_x.at[4]))
    c_mem = rows_copy(mem_hbm, mem, 0, M, sem_b.at[0])
    c_bx0 = rows_copy(bx_hbm, bx, 0, 6 * SEG, sem_b.at[1])
    c_bx1 = rows_copy(bx_hbm, bx, 6 * SEG, S, sem_b.at[2])
    c_outa = cp(outa, out_hbm.at[:, pl.ds(0, D)], sem_o.at[0])

    def chunk(j, g):
        return 3 * g + j if j < 3 else 3 * NG + g

    def c_w(c):
        j, g = (c % 3, c // 3) if c < 3 * NG else (3, c - 3 * NG)
        n = GROUPS[g].n * 128
        return cp((wq_hbm, wk_hbm, wv_hbm, wo_hbm)[j].at[pl.ds(g * GW * 128, n), :],
                  raw.at[c % RING, pl.ds(0, n), :], sem_w.at[c])

    def c_outb(r0, n):
        return cp(outb.at[pl.ds(r0, n), :], out_hbm.at[pl.ds(r0, n), pl.ds(D, D)], sem_o.at[1])

    def start(copies, priority=1):
        for c in copies:
            c.start(priority=priority)

    def wait(copies):
        with _scope("wait"):
            for c in copies:
                c.wait()

    def a_weights(j):
        def fill(plan, t):
            tmp[j % 2, t] = (awo[:, t * 128:(t + 1) * 128].astype(F32) if j == 3 else
                             awqkv[j, t * 128:(t + 1) * 128, :].astype(F32).T)

        def move(plan, t, d):
            rows = [plan.paced(tmp[j % 2, t, pl.ds(d + h * AD, 8, stride=AD), :], h / AH)
                    for h in range(0, AH, 8)]
            aw[_ds(j * AD + d, AH // 2), t * 128:(t + 1) * 128] = pltpu.bitcast(
                _rows(rows).astype(BF16), U32)

        return [task for t in range(LT)
                for task in [_task(fill, t)] + [_task(move, t, d) for d in range(AD)]]

    def a_proj(i, b, j):
        def tile(plan, t):
            c = j * LT + t
            x = pltpu.bitcast(xw[plan.zero + b], BF16)
            w = pltpu.bitcast(aw[c * 64:(c + 1) * 64, :], BF16)
            r = lax.dot_general(x, w, NT, preferred_element_type=F32)
            plan.result(r)
            qkv_s[b, c, HALO:HALO + TB, :] = r
            if j and isinstance(i, int) and i == 0:
                qkv_s[b, c, 0:HALO, :] = jnp.broadcast_to(r[0:1, :], (HALO, 128))
            elif j:
                qkv_s[b, c, 0:HALO, :] = qkv_s[1 - b, c, TB:TB + HALO, :]
        return [_task(tile, t) for t in range(LT)]

    def a_attention(b, first_block=False):
        state = {}

        def window(c, r0, w):
            lo = HALO + r0 - ADIL * w
            return qkv_s[b, c, lo:lo + 8, :]

        def logits(plan, r0):
            q = [plan.paced(window(t, r0, 0), t / LT) for t in range(LT)]
            state[r0] = []
            for w in range(AW):
                a = q[0] * window(LT, r0, w)
                for t in range(1, LT):
                    a = a + q[t] * window(LT + t, r0, w)
                state[r0].append(a + pltpu.roll(a, 2 * AH, 1))

        def fold(plan, r0):
            state[r0] = [a + pltpu.roll(a, AH, 1) for a in state[r0]]

        def weigh(plan, r0):
            lg = []
            for w, a in enumerate(state[r0]):
                if first_block and r0 < ADIL * w:
                    pos = lax.broadcasted_iota(jnp.int32, (8, 128), 0) + r0
                    a = jnp.where(pos >= ADIL * w, a, MASKED * AD ** 0.5)
                lg.append(a)
            m = functools.reduce(jnp.maximum, lg)
            state[r0] = [jnp.exp2((a - m) * (AD ** -0.5 * LOG2E)) for a in lg]

        def mix(plan, r0):
            e = [plan.paced(x, w / AW) for w, x in enumerate(state.pop(r0))]
            inv = _inverse(functools.reduce(jnp.add, e))
            for t in range(LT):
                o = e[0] * window(2 * LT + t, r0, 0)
                for w in range(1, AW):
                    o = o + e[w] * window(2 * LT + t, r0, w)
                oa_s[b][0, r0:r0 + 8, t * 128:(t + 1) * 128] = o * inv

        n = TB // 8
        return [_task(f, (k - lag) * 8) for k in range(n + 2)
                for lag, f in ((2, weigh), (0, logits), (1, fold), (2, mix)) if 0 <= k - lag < n]

    def a_out(i, b):
        def tile(plan, t):
            r = _dot(oa_s[b][plan.zero], pltpu.bitcast(aw[3 * D // 2:, t * 128:(t + 1) * 128], BF16))
            plan.result(r)
            outa[_ds(i, TB), t * 128:(t + 1) * 128] = r.astype(BF16)
        return [_task(tile, t) for t in range(LT)]

    def tiles_of(c, odd=None, zero=0):
        if isinstance(c, int) and c >= full:
            return wt[2 + c - full].at[zero]
        return wt[c % 2 if odd is None else odd].at[c // 2 + zero]

    def w_transpose(c, grp, odd=None):
        def two(plan, i, f):
            t = pltpu.bitcast(raw[c % RING, f * 128:(f + 2) * 128, i * 128:(i + 1) * 128].T, U32)
            for k in range(2):
                tiles_of(c, odd)[grp.slot[i, f + k]] = t[:, k * 128:(k + 1) * 128]
        return [_task(two, i, f) for f in range(0, grp.n, 2) for i in range(LT)]

    def w_combine(c, grp, transposed=True, odd=None):
        own, other = {}, {}

        def edge(plan, r, a, b):
            def tile(i, f, part=0.0):
                if transposed:
                    t = tiles_of(c, odd, plan.zero)[grp.slot[i, f], _group(r)]
                else:
                    t = pltpu.bitcast(raw[c % RING, _ds(8 * f + r, 16), i * 128:(i + 1) * 128], U32)
                t = plan.paced(t, part)
                if not transposed and i != grp.label[f]:
                    tiles_of(c, odd, plan.zero)[grp.slot[i, f], _group(r)] = t
                return pltpu.bitcast(t, BF16).astype(F32)

            def put(key, t):
                tiles_of(c, odd, plan.zero)[grp.slot[key], _group(r)] = pltpu.bitcast(
                    t.astype(BF16), U32)

            for f in (a, b):
                if f not in own:
                    own[f] = other[f] = tile(grp.label[f], f)
            ta, tb = tile(grp.label[b], a), tile(grp.label[a], b, 0.5)
            put(("both", a, b), ta + tb)
            own[a], other[a] = own[a] - ta, other[a] + tb
            own[b], other[b] = own[b] - tb, other[b] + ta
            for f, mate in ((a, b), (b, a)):
                if mate == grp.mates[f][-1]:
                    put((grp.label[f], f), own.pop(f))
                    put(("other", f), other.pop(f))
                    for i in grp.plain[f] * (not transposed):
                        tile(i, f)

        return [_task(edge, r, a, b) for r in range(8) for a in grp.side[0] for b in grp.mates[a]]

    full = 3 * (NG - 1)

    def stage_x(i, b):
        xw[b] = pltpu.bitcast(ax[_ds(i, TB), :], U32)

    def qkv_of(i, b):
        return [t for j in range(3) for t in a_proj(i, b, j)]

    def a_step(it, carry):
        for k in range(full // 2):
            @pl.when(it == k)
            def _():
                wait([c_w(c) for c in (2 * k - 1, 2 * k) if c >= 0]
                     + [c_ax[2 + k // 2] for _ in range(k in (1, 3))])
                start([c_w(2 * k + 2), c_w(2 * k + 3)])
                start({0: [c_ax[2]], 2: [c_ax[3]], 4: [c_mem, c_bx0]}.get(k, []), 0)
        c = 2 * it
        plan = _Plan(nil, a_out(c, 0) + a_out(c + 1, 1) + qkv_of(c + 3, 1) + qkv_of(c + 4, 0))
        for b in range(2):
            new, before = [jnp.where(k < 0, k + RING, k) for k in (c + b - 1, c + b - 2)]
            plan.spread(w_combine(before, GROUPS[0], True, b), P0 * b, P0 * (b + 1))
            plan.spread(w_transpose(new, GROUPS[0], 1 - b), P0 * b, P0 * (b + 1))
        plan.spread(a_attention(0), P1, 24.99)
        plan.spread(a_attention(1), 24.99, P2)
        plan.run()
        for b in range(2):
            stage_x(jnp.minimum(c + 6 - b, NB - 1), b)
        return carry

    def clear(k, carry):
        z_part[0][0, _ds(k, 20)] = jnp.zeros((20, 8, 128), F32)
        return lax.shift_right_logical(k, 16)

    def binade(tiles):
        top = jnp.max(functools.reduce(jnp.maximum, map(jnp.abs, tiles)), axis=1, keepdims=True)
        top = jnp.clip(jnp.broadcast_to(top, (8, 128)), 2.0 ** -60, 2.0 ** 60)
        return pltpu.bitcast(top, jnp.int32) & 0x7F800000

    slots = ({}, {})

    def put(ph, key, t, memory=False):
        (l_tok, l_mem)[memory][ph][0, slots[memory].setdefault(key, len(slots[memory]))] = t

    def get(ph, key, zero, memory=False):
        return (l_tok, l_mem)[memory][ph][zero, slots[memory].setdefault(key, len(slots[memory]))]

    def memory_operands(ph, known, i, t):
        known[i] = t
        put(ph, ("plain", i, 0), t, True)
        for k, u in known.items():
            if k != i:
                put(ph, ("sum", min(i, k), max(i, k), 0), t + u, True)

    def memory_pair(plan, ph):
        n = IN_PAIRS.index((0, 1))
        cur = [get(ph, ("plain", i, 0), 0, True) for i in range(LT)]
        shift = binade(cur) - pltpu.bitcast(get(ph, "binade", plan.zero), jnp.int32)
        down, up = [pltpu.bitcast(x, F32) for x in (0x3F800000 + shift, 0x3F800000 - shift)]
        put(ph, "down", down, True)
        put(ph, "up", up, True)
        for k in range(LT):
            mate = get(ph, ("mate", k), plan.zero)
            put(1 - ph, ("back", n, k), mate - cur[k] * up)
            mate = mate * down
            put(ph, ("both", n, k, k), cur[k] - mate, True)
            for i in range(LT):
                if i != k:
                    put(ph, ("both", n, i, k), cur[i] + mate, True)

    def token_operands(x, s, ph, first=False):
        def tokens(plan, ds, r):
            rows = _ds(2 * (s + ds) + (r - 1) // 2, 16)
            return [pltpu.bitcast(plan.paced(pltpu.bitcast(x[rows, i * 128:(i + 1) * 128], U32)),
                                  BF16).astype(F32)[_group((r - 1) % 2)] for i in range(LT)]

        state = {}

        def current(plan, r, i):
            if i == 0:
                state[0] = tokens(plan, 0, r)
            t = plan.paced(state[0][i])
            put(ph, ("plain", i, r), t)
            for k in range(i + 1, LT):
                put(ph, ("sum", i, k, r), t + state[0][k])

        def later(plan, r):
            for i, t in enumerate(tokens(plan, 2, r)):
                put(ph, ("later", i, r), t)
            for i, t in enumerate(tokens(plan, 1, r) * first):
                put(ph, ("next", i, r), t)

        def after(plan, n, k):
            r0, r1 = IN_PAIRS[n]
            if k == 0:
                state[1] = tokens(plan, 1, r1)
            mate = plan.paced(state[1][k])
            if r0 == 0:
                put(ph, ("mate", k), mate)
                if k == 0:
                    put(ph, "binade", pltpu.bitcast(binade(state[1]), F32))
                return
            put(ph, ("both", n, k, k), state[0][k] - mate)
            for i in range(LT):
                if i != k:
                    put(ph, ("both", n, i, k), state[0][i] + mate)

        def before(plan, n):
            for i, t in enumerate(tokens(plan, -1, IN_PAIRS[n][0])):
                put(ph, ("back", n, i), state[0][i] - t)

        tasks = [_task(later, r) for r in sorted({r1 for _, r1 in IN_PAIRS})]
        for r in range(RG):
            tasks += [_task(current, r, i) for i in range(LT * (r > 0))]
            for n, (r0, r1) in enumerate(IN_PAIRS):
                tasks += [_task(after, n, k) for k in range(LT * (r0 == r))]
                tasks += [_task(before, n)] * (r1 == r and r0 > 0 and not first)
        return tasks

    def segment(s, ph, zero, first=False, last=False):
        live = range(1 if last else 0, RG)
        pieces = {}

        zeros, uses = [zero >> k for k in range(NZ)], {}

        def fresh(key):
            uses[key] = uses.get(key, 0) + 1
            return zeros[uses[key] % NZ]

        def product(plan, parts, j, g, key):
            w = tiles_of(chunk(j, g))[GROUPS[g].slot[key]]
            return plan.result(_dot(_rows(parts), pltpu.bitcast(w, BF16)))

        def project(j, g):
            grp, f0 = GROUPS[g], g * GW
            lab = grp.label
            every = live if j == 0 else range(RG)
            to_next = {} if last else _pairs(j, g, ph)
            from_prev = {} if first else {r1: r0 for r0, r1 in _pairs(j, g, 1 - ph).items()}
            future = () if last else tuple(_pairs(j, g, 1 - ph).values())
            early = [r for r in every if r not in from_prev]
            y, gift, places, crossed = _Sums(), _Sums(), [], {}
            owed = {a: 1 + len(grp.mates[a]) for a in grp.side[ph]}
            left = {f: LT + len(grp.mates[f]) * (f not in owed) for f in range(grp.n)}

            def operand(key, r):
                at_once = r == 0 and chunk(j, g) == 0
                return get(ph, key, 0 if at_once or not DYN else fresh(key), r == 0)

            def plain(i, r):
                return operand(("plain", i, r), r)

            def mixed(i, k, r):
                return operand(("both", IN_PAIRS.index((r, to_next[r])), i, k), r)

            def take(f, rows, res, minus=False, now=False):
                for r, t in zip(rows, res):
                    y.add((f, r), t, minus)
                left[f] -= 1
                crossed[f] = crossed.get(f, 0) + minus
                if not left[f] or minus and crossed[f] % DS == 0 or now:
                    signs = {}
                    for r in every:
                        if (f, r) in y.sums:
                            t, signs[r] = y.sums.pop((f, r))
                            y_s[chunk(j, g)][0, len(places), _group(r)] = t
                    pieces.setdefault((j, f0 + f), []).append((len(places), signs))
                    places.append(f)

            def give(a, res):
                for r, t in zip(early, res):
                    if r in to_next:
                        gift.add((a, r), t)
                owed[a] -= 1
                for r0, r1 in to_next.items() if not owed[a] else ():
                    t = gift.pop((a, r0))
                    ahead[ph][0, j, f0 + a, 0, _group(r1 - 1)] = t if r0 else t * operand("up", 0)

            def own(plan, a):
                parts = [plain(lab[a], r) for r in early]
                parts += [operand(("later", lab[a], r), r) for r in future]
                res = product(plan, parts, j, g, (lab[a], a))
                for r in from_prev:
                    y.add((a, r), ahead[ph][0, j, f0 + a, 1, _group(r - 1)])
                for r, t in zip(future, res[len(early):]):
                    ahead[ph][0, j, f0 + a, 1, _group(r - 1)] = t
                take(a, early, res)
                give(a, res)

            def opening(plan, b):
                parts = [operand(("next", lab[b], r), r) for r in to_next.values()]
                for r, t in zip(to_next.values(), product(plan, parts, j, g, (lab[b], b))):
                    ahead[1 - ph][0, j, f0 + b, 1, _group(r - 1)] = t

            def other(plan, b):
                parts = [mixed(lab[b], lab[b], r) if r in to_next else
                         operand(("back", IN_PAIRS.index((from_prev[r], r)), lab[b]), r) if r in from_prev
                         else plain(lab[b], r) for r in every]
                res = product(plan, parts, j, g, ("other", b))
                for r in from_prev:
                    y.add((b, r), ahead[1 - ph][0 if first else zero, j, f0 + b, 0, _group(r - 1)])
                for r0, r1 in to_next.items():
                    t = ahead[1 - ph][0 if first else zero, j, f0 + b, 1, _group(r1 - 1)]
                    y.add((b, r0), t if r0 else plan.paced(t, 0, 1) * operand("down", 0))
                take(b, every, res, False, HP)

            def both(plan, a, b):
                parts = [mixed(lab[a], lab[b], r)
                         if r in to_next else plain(lab[a], r) for r in early]
                res = product(plan, parts, j, g, ("both", a, b))
                take(b, early, res, False, EP and not first)
                give(a, res)

            def cross(plan, a, b):
                i, k = sorted((lab[a], lab[b]))
                res = product(plan, [operand(("sum", i, k, r), r) for r in every], j, g, (lab[b], a))
                take(a, every, res)
                take(b, every, res, True)

            def single(plan, i, f):
                take(f, every, product(plan, [plain(i, r) for r in every], j, g, (i, f)))

            passes = []
            others = list(grp.side[1 - ph])
            for a, b0 in zip(grp.side[ph], others[grp.n == GW:] + others):
                passes += [((), _task(opening, b0), RG)] * first
                kinds = {
                    "g": [((lab[a],), _task(own, a), RG), ((lab[b0],), _task(other, b0), RG)]
                    + [((i,), _task(single, i, f), RG) for f in (a, b0) for i in grp.plain[f]],
                    "d": [((lab[a],), _task(both, a, b), len(early)) for b in grp.mates[a]],
                    "c": [((lab[a], lab[b]), _task(cross, a, b), RG) for b in grp.mates[a]]}
                passes += [x for kind in STEP for x in kinds[kind]]
            return passes

        n = 8 * len(live)
        key = lax.broadcasted_iota(jnp.int32, (L, 2 * n), 0)
        col = lax.broadcasted_iota(jnp.int32, (L, 2 * n), 1)
        head0 = col < n
        query = jnp.where(head0, col, col - n) + (L - n)
        visible = (query < M) | (query >= key)
        scores = _Sums()

        def gather(j, f):
            rows = []

            def add_up(plan, r):
                t = _Sums()
                for place, signs in pieces[j, f]:
                    if r in signs:
                        u = y_s[chunk(j, f // GW)][zero, place, _group(r)]
                        t.add(r, u if t.sums else plan.paced(u), signs[r])
                rows.append(t.pop(r))
                if r < RG - 1:
                    return
                t = _rows(rows)
                low = lax.broadcasted_iota(jnp.int32, t.shape, 1) < 64
                if j == 1:
                    pass
                elif f % 3 == 1:
                    t = _rows([jnp.where(low, t, 0.0), jnp.where(low, 0.0, t)]).astype(BF16)
                elif f % 3 == 0:
                    t = _rows([t, jnp.zeros((48 - t.shape[0], 128), F32)]).astype(BF16)
                else:
                    t = _rows([jnp.zeros((t.shape[0] % 16, 128), F32), t][t.shape[0] % 16 == 0:]).astype(BF16)
                t = pltpu.bitcast(t, U32)
                qkv[j != 2][f][0, j % 2, 0:t.shape[0]] = t

            return [_task(add_up, r) for r in (range(RG) if j else live)]

        def by_head(j, f):
            rows = L if j else n
            words = qkv[j != 2][f][zero, 0, 0:(24, rows, pl.cdiv(rows, 16) * 8)[f % 3]]
            if f % 3 == 2 or f % 3 == 0 and not j:
                words = _rows([words, jnp.zeros((rows - words.shape[0], 128), U32)][::1 - f % 3])
            return pltpu.bitcast(words, BF16)

        def score(plan, f):
            k = pltpu.bitcast(qkv[1][f][zero, 1, 0:L], F32)
            scores.add(f // 3, lax.dot_general(k, by_head(0, f), NT, preferred_element_type=F32))
            if f % 3 == 2:
                sc = jnp.where(visible, scores.pop(f // 3), MASKED * DH ** 0.5)
                e = jnp.exp2((sc - jnp.max(sc, axis=0, keepdims=True)) * (DH ** -0.5 * LOG2E))
                p = e * _inverse(jnp.sum(e, axis=0, keepdims=True))
                p = _rows([jnp.where(head0, p, 0.0), jnp.where(head0, 0.0, p)]).T
                p = jnp.concatenate([p, jnp.zeros((2 * n, 128 - 2 * L), F32)], axis=1)
                p_s[f // 3][0, 0:3 * n] = _rows([p[0:n], p[0:n] + p[n:], p[n:]])

        def mix(plan, f):
            v = by_head(2, f)
            res = _dot(p_s[f // 3][zero, f % 3 * n:(f % 3 + 1) * n, 0:v.shape[0]], v)
            g = f // GW
            for k, r in enumerate(live):
                o_s[ph][g][0, f % GW, _group(r)] = res[_group(k)]
                for r0, r1 in _pairs(3, g, 1 - ph).items():
                    if r1 == r and not first and f % GW in GROUPS[g].side[1 - ph]:
                        o_old[1 - ph][0, f, _group(r0)] = (res[_group(k)]
                                                + o_s[1 - ph][g][zero, f % GW, _group(r0)])

        z = _Sums()

        def out_project(groups):
            def operand(g, terms):
                t = _Sums()
                for back, f, r, *minus in terms:
                    if back < 2:
                        u = o_s[(ph + back) % 2][g][fresh((back, g, f, r)), f, _group(r)]
                    else:
                        u = o_old[(ph + back) % 2][zero if back == 2 else 0, g * GW + f, _group(r)]
                    t.add(0, u, *minus)
                return t.pop(0)

            def run(plan, kind, part, left, g, key, rows):
                res = product(plan, [operand(g, terms) for terms, _ in rows], 3, g, key)
                for (_, to), t in zip(rows, res):
                    part.add(to, t)
                left.pop()
                for to in sorted(part.sums) * (not left):
                    t = part.pop(to)
                    for key in to:
                        if last or first or key[0] == key[2] == 0:
                            z.add(key[:3], t, len(key) > 3)
                        else:
                            z_part[ph][0, PARTS[ph][groups[0], kind, to]] = t

            tasks = []
            for kind, passes in _out_passes(groups, ph, first, last):
                part, left = _Sums(), list(passes)
                tasks += [(kind[:2] if kind[2] == 2 else kind[3:],
                           _task(run, kind, part, left, *x), len(x[2])) for x in passes]
            if OMIX:
                short = [x for x in tasks if x[2] < 4]
                long = [x for x in tasks if x[2] >= 4]
                order = [((k // OMIX + 0.5) / len(xs), n, k, x) for n, xs in enumerate((long, short))
                         for k, x in enumerate(xs)]
                tasks = [x[3] for x in sorted(order, key=lambda x: x[:3])]
            return tasks

        main, begin, done = [], {}, {}
        parts = STREAM0 if first else STREAM
        for part in parts:
            if part[0][0] == 3:
                new = out_project([g for _, g in part])
            else:
                new = [project(*jg) for jg in part]
                new = [x for k in range(0, len(new[0]), GW) for passes in new for x in passes[k:k + GW]]
            if part is parts[0] and not first:
                new.sort(key=lambda x: max(max(x[0]), LT - 1 - LATE))
            if part is parts[-1]:
                new.sort(key=lambda x: max(min(x[0]), LT - 1 - LATE))
            begin.update({jg: len(main) for jg in part})
            main += new
            done.update({jg: len(main) for jg in part})
        extra = []

        ready = {}
        for stage, gap, windows in (
                (score, GAP_S, lambda f: (max(done[j, f // GW] for j in range(2)) + LAG_S,
                                          begin[3, f // 3 * 3 // GW] - LAG_O - LAG_N)),
                (mix, GAP_V, lambda f: (max(done[2, f // GW] + LAG_V, ready[f // 3] + LAG_N),
                                        begin[3, f // GW] - LAG_O))):
            at = -gap
            for f in range(FT):
                step = min([gap] + [(windows(k)[1] - at) / (k - f + 1) for k in range(f, FT)])
                at = max(at + max(step, 0.01), windows(f)[0])
                assert at < begin[3, f // GW] - 1
                extra.append((at + JIT.get((ph, stage is mix, f), 0), stage, f))
                if stage is score:
                    ready[f // 3] = at

        if first:
            k = begin[3, NG - 1]
            main[k:k] = [((), task) for task in a_out(NB - 1, 1)]
        plan = _Plan(zero, [x[1] for x in main])
        for at, stage, f in extra:
            plan.spread([_task(stage, f)], at, at)
            js = (0, 1) if stage is score else (2,)
            k0 = max(at - BACK_S - GSPAN, max(done[j, f // GW] for j in js) - 1)
            plan.spread([t for j in js for t in gather(j, f)], k0, max(at - BACK_S, k0))

        if first:
            def arrive(plan, groups):
                wait([c_w(chunk(3, g)) for g in groups])
                start([c_w(chunk(3, g + 3)) for g in groups if EARLY <= g < NG - 3])

            def sums(j, groups):
                return [t for g in groups for t in w_combine(chunk(j, g), GROUPS[g], j < 3)]

            k = begin[3, NG - 1]
            plan.spread([t for j in (1, 2) for t in w_transpose(full + j, GROUPS[-1])], 0, 0)
            plan.spread([t for j in range(3) for t in sums(j, [NG - 1])], 0, Q[1] - 8)
            for groups, k0, k1 in (((0, 1), Q[1], Q[2] - 8), ((2, 3), Q[2], k - 8), ((4,), k - 1, k + 4)):
                plan.spread([_task(arrive, groups)], k0, k0)
                plan.spread(sums(3, groups), k0, k1)
        if not last:
            k0 = begin[3, NG - 2] + 5 if first else TOK0
            x = bx if first else bx.at[pl.ds(pl.multiple_of((s - 2 + ph) * SEG, 2 * SEG), 6 * SEG)]
            plan.spread(token_operands(x, 1 if first else 3 - ph, 1 - ph), k0, k0 + TOK1 - TOK0)
            plan.spread([_task(memory_pair, ph)] * ((0, 1) in IN_PAIRS), 1, 1)
            known = {}
            for i in range(LT):
                at = max(k for k, (tiles, *_) in enumerate(main) if i in tiles)
                plan.spread([lambda _, i=i: memory_operands(1 - ph, known, i, z.pop((0, i, 0)))],
                            at, at)
        if not first:
            plan.spread(settle(s - 1, 1 - ph), FOLD0, FOLD1)

        def resume(plan):
            for i in range(LT):
                for r in range(1, RG * last):
                    for back in range(2):
                        z.add((back + 1, i, r), z_s[1 - ph][zero, back, i, _group(r)])
                for r in _carried(1 - ph):
                    if (r > 0) == last:
                        z.add((0, i, r), z_s[1 - ph][zero, 2, i, _group(r)], True)

        plan.spread([resume] * (not first), begin[3, 0] - 1, begin[3, 0])
        plan.run()
        for back in (2, 1, 0) * last:
            for i in range(LT):
                outb[_ds(s - back, SEG), i * 128:(i + 1) * 128] = _rows(
                    [z.pop((back, i, r)) for r in range(1, RG)]).astype(BF16)
        for (g, _, to), place in PARTS[ph].items():
            if g is None:
                z_part[ph][0, place] = z.pop(to[0]) if first else jnp.zeros((8, 128), F32)

    def settle(s, ph):
        layout, done = {}, []
        for (_, _, to), place in PARTS[ph].items():
            for key in to:
                layout.setdefault(key[:3], []).append((place, len(key) > 3))

        def add_up(plan, back, i, r):
            t = _Sums()
            if back > 0 or back == 0 and r in _carried(1 - ph):
                t.add(0, plan.paced(z_s[1 - ph][plan.zero, (back - 1) % 3, i, _group(r)]), back == 0)
            for place, minus in layout.get((back, i, r), ()):
                u = z_part[ph][plan.zero, place]
                t.add(0, u if t.sums else plan.paced(u), minus)
            if back < 2:
                z_s[ph][0, back % 3, i, _group(r)] = t.pop(0)
                return
            done.append(t.pop(0))
            if r % 2 == 0:
                seg = s - 2 if isinstance(s, int) else jnp.maximum(s - 2, 0)
                outb[_ds(2 * seg + r // 2 - 1, 16), i * 128:(i + 1) * 128] = _rows(
                    done[-2:]).astype(BF16)

        return [_task(add_up, back, i, r) for i in range(LT) for back in (0, -1, 1, 2)
                for r in range(RG) if (r > 0 if back >= 0 else (back, i, r) in layout)]

    if not ONLY:
        start([c_wqkv[0], c_ax[0], c_wqkv[1]])
        nil = lax.fori_loop(0, z_part[0].shape[1] // 20, clear, 0)
        z_s[1][...] = jnp.zeros(z_s[1].shape, F32)
        bx[S:, :] = jnp.zeros((2 * SEG, D), BF16)
        wait([c_wqkv[0]])
        start([c_wqkv[2]])
        _Plan(nil, a_weights(0)).run()
        wait([c_ax[0]])
        start([c_ax[1]])
        for b in range(2):
            stage_x(b, b)
        _Plan(nil, a_proj(0, 0, 0)).run()
        for j, copies in ((1, [c_awo]), (2, [c_ax[4]])):
            wait([c_wqkv[j]])
            start(copies)
            plan = _Plan(nil, a_proj(1, 1, j - 1) + a_proj(0, 0, j))
            plan.spread(a_weights(j), 0, W1)
            plan.run()
        wait([c_ax[1], c_awo])
        start([c_w(0), c_w(1)])
        stage_x(2, 0)
        plan = _Plan(nil, a_proj(1, 1, 2) + qkv_of(2, 0))
        plan.spread(a_attention(0, True), 0, 4.99)
        plan.spread(a_attention(1), S0, 18.5)
        plan.spread(a_weights(3), S1, 18.5)
        plan.run()
        wait([c_ax[4]])
        for b in range(2):
            stage_x(4 - b, b)
        with _scope("a_loop"):
            lax.fori_loop(0, full // 2, a_step, 0)
        wait([c_mem, c_bx0] + [c_w(full + j) for j in (-1, 0)])
        start([c_w(full + 2), c_w(full + 3)])
        plan = _Plan(nil, a_out(NB - 4, 0) + a_out(NB - 3, 1) + qkv_of(NB - 1, 1) + a_out(NB - 2, 0))
        for b in range(2):
            plan.spread(w_combine(full - 2 + b, GROUPS[0], True, b), P0 * b, P0 * (b + 1))
            plan.spread(w_transpose(full - 1 + b, GROUPS[-b]), P0 * b, P0 * (b + 1))
        plan.spread(a_attention(0), R0, R1)
        plan.spread(a_attention(1), 23.99, 29)
        plan.spread(token_operands(bx, 0, 0, first=True), 16, 28)
        plan.run()
        wait([c_w(full + j) for j in (1, 2)])
        start([c_w(full + 4), c_w(full + 5)] + [c_w(full + 6) for _ in range(EARLY)])

    if not ONLY:
        known = {}
        for i in range(LT):
            memory_operands(0, known, i, mem[0:M, i * 128:(i + 1) * 128].astype(F32))
        segment(0, 0, nil, first=True)
    start([c_bx1, c_outa])
    if ONLY:
        def touch(i, c):
            for w in wt:
                w[0, i] = jnp.zeros(w.shape[2:], w.dtype)
            return c
        lax.fori_loop(0, 2, touch, 0)

    def b_step(it, carry):
        @pl.when(it == 1)
        def _():
            c_bx1.wait()
        zero = lax.shift_right_logical(it, 16)
        if HEAD:
            outb[0:16, 0:128] = _rows([z_part[0][zero, zero] + l_mem[1][zero, zero], l_tok[1][zero, zero] + ahead[0][zero, zero, zero, zero, 0:8] + ahead[1][zero, zero, zero, zero, 0:8]]).astype(BF16)
        else:
            segment(1 + 2 * it, 1, zero)
            segment(2 + 2 * it, 0, zero)

        @pl.when(it > 0)
        def _():
            c_outb(pl.multiple_of((it - 1) * 2 * SEG, 2 * SEG), 2 * SEG).start()
        return zero

    with _scope("b_loop"):
        nil = lax.fori_loop(0, NSEG // 2 - 1, b_step, 0)
    if not ONLY and not HEAD:
        segment(NSEG - 1, 1, nil, last=True)
    c_outb(S - 4 * SEG, 4 * SEG).start()
    wait([c_outa, c_outb(0, S)])


def pallas_concat_heads__sliding_local_dilated__memory_aug_recurrent_mem_tr__prompt_kernel(
    A_x, A_wqkv, A_wo, B_x, B_mem0, B_Wq, B_Wk, B_Wv, B_Wo, B_seg_len,
):
    assert B_seg_len == SEG
    assert A_x.shape == B_x.shape == (1, S, D) and B_mem0.shape == (1, M, D)
    assert B_Wq.shape == B_Wk.shape == B_Wv.shape == (D, H, DH) and B_Wo.shape == (H, DH, D)
    dma = pltpu.SemaphoreType.DMA

    def vmem(dtype, *shape):
        assert math.prod(shape) * jnp.dtype(dtype).itemsize % 16384 == 0, shape
        return pltpu.VMEM(shape, dtype)

    call = pl.pallas_call(
        _kernel,
        out_shape=jax.ShapeDtypeStruct((S, 2 * D), BF16),
        in_specs=[pl.BlockSpec(memory_space=pl.ANY)] * 9,
        out_specs=pl.BlockSpec(memory_space=pl.ANY),
        scratch_shapes=[
            vmem(BF16, S, D),
            vmem(BF16, 3, D, D),
            vmem(BF16, D, D),
            vmem(F32, 2, LT, D, 128),
            vmem(U32, 2 * D, D),
            vmem(U32, 2, TB // 2, D),
            vmem(F32, 2, 3 * LT, HALO + TB, 128),
            [vmem(F32, 1, TB, D)] * 2,
            vmem(BF16, S, D),
            vmem(BF16, S + 2 * SEG, D),
            vmem(BF16, 64, D),
            vmem(BF16, RING, GW * 128, D),
            [vmem(U32, 6, SLOTS, 64, 128)] * 2 + [vmem(U32, 1, SLOTS, 64, 128)] * 8,
            [vmem(F32, 1, 200, 8, 128)] * 2,
            [vmem(F32, 1, 44, 8, 128)] * 2,
            [vmem(F32, 1, 3, FT, 2, 24, 128)] * 2,
            [vmem(F32, 1, 48, L, 128)] * (3 * NG),
            [vmem(F32, 1, 128, 128)] * (FT // 3),
            [[vmem(U32, 1, 2, 48, 128)] * FT] * 2,
            [[vmem(F32, 1, 12, L, 128)] * NG] * 2,
            [vmem(F32, 1, FT, L, 128)] * 2,
            [vmem(F32, 1, 420, 8, 128)] * 2,
            [vmem(F32, 1, 4, LT, L, 128)] * 2,
            vmem(BF16, S, D),
            dma((4,)), dma((5,)), dma((4 * NG,)), dma((3,)), dma((2,)),
        ],
        compiler_params=pltpu.CompilerParams(vmem_limit_bytes=126 * 1024 * 1024, flags=FLAGS),
        name="sliding_and_memory_attention",
    )

    def by_feature(w):
        return w.transpose(1, 2, 0).reshape(H * DH, D)

    out = call(A_x.reshape(S, D), A_wqkv, A_wo, B_x.reshape(S, D), B_mem0.reshape(M, D),
               by_feature(B_Wq), by_feature(B_Wk), by_feature(B_Wv), B_Wo.reshape(H * DH, D))
    return out.reshape(1, S, 2 * D)
```

```python
import functools
import math

import jax
import jax.numpy as jnp
from jax import lax
from jax.experimental import pallas as pl
from jax.experimental.pallas import tpu as pltpu

F32, BF16, U32 = jnp.float32, jnp.bfloat16, jnp.uint32
NT = (((1,), (1,)), ((), ()))
MASKED = -1000000000.0
LOG2E = math.log2(math.e)

S, D = 2048, 640
LT = D // 128

AH, AD, AW, ADIL = 32, 20, 8, 2
HALO = 16
TB = 128
NB = S // TB

H, DH, M, SEG = 32, 192, 8, 32
L = M + SEG
FT = H * DH // 128
NSEG = S // SEG
GW = 2 * LT
NG = pl.cdiv(FT, GW)
FULL = 3 * (NG - 1)
RING = 8


def _stream(text):
    return [[("qkvo".index(w[0]), int(w[1])) for w in part.split("+")] for part in text.split(",")]


FIRST = _stream("q0,k0,v0,q1,k1,v1,q2,k2,v2,q3,k3,v3,q4,k4,v4,o0+o1+o2,o3,o4")
STREAM = _stream("q0,k0+v0,q1+k1,v1+q2,k2+v2,q3+k3,q4+k4,v3+v4,o0+o1+o2,o3+o4")
ORDER = (
    "10000000000010000000100000000000010000000010000000000000100000100000000000100000000001000000"
    "00000100000000000001000000000100000000010000000000010300000010000000000030010000300001000300"
    "00001000003000001000000030000000100300000000103000000103000000000014030004000000001000000401"
    "04000000000001040000000000100400000010400000000100400000001430003000000000031000000000010000"
    "00300000100003001000000300003100000000030000010000014000003000000310040000000104000000000104"
    "00000040000000010040000100000004000000010040000100000400000100303000000000030100000100030000"
    "00000100300000000130000000003000010040000000013000000103400000000001040430000000100000000041"
    "00004000000000014000000000104000000001004000000104000000000104003030000000000134000000000010"
    "30000000013000000000003001000000001000300001030000000000010030000001400030400000000010040000"
    "00100400000000100000004000010040000000300100301140024012055520135000010103021401000125535105"
    "00002001100310200205155501030000300112002100455515102000000012410110400125555100000011204001"
    "01042255150500001001010420400011225000000411000012000402022002020222000000022202000202020200"
    "0202002020010010110000010100011000001010010100010",
    "02200022020002200202002020220020202000020220020000222020000101100100000202200102011000020120"
    "00220000111000010220002000210110000202100022000001100011002002220000011000110200002020210010"
    "30102021000022300011000011000023020231201000002101002033002021001000101302022000021300001301"
    "02100030220210140001310024020202000011014001300020202243000101034101000202002324000101001134"
    "00000223204023000114010100000222023400010101030002010242002000110401000201024002200100110400"
    "10024200200012010104010000202240001201010140002002020200001101000100002302020120010130002213"
    "00002200101013030002210200002003011100001000022300012030140001002400220030001001134000002020"
    "42003000101014300300202020240000101301140000022204302030001104100000202024203000011403100002"
    "02302024000010101003002020230003201010101030002020220000001230022002003110020002001203022002"
    "01032000010240031240202010240400000120420012400200214400002020012402401004020200400202002141"
    "02400204014000020201014240202010000020201020001010201000001020101000002010000210100002001020"
    "10000020101000201000102000102010102010201020",
    "00202020202020202000202020202020202000202020200000111010000002220200001110100000222020000011"
    "10100000222020000011101000002220200000111010000002220200001010101000002022200100101000100200"
    "20202010101300021030032200201000011130002200002102000310310102000020220000113010031000223020"
    "02000113100202104003202010101014040020200203200010101314000202304202000101010430001202020432"
    "00000111400310020202040302010011401030000222030001200114000020102420200001010114000200024022"
    "00100110400010242020200000111040010202024000010201010001020002020201000301010132002002020100"
    "01330012010002020201010300023102100200020300101103100200242002000013401000140002023000200014"
    "01013040000202030200010410030000210240302000013101410040020202030201001140030100400202032001"
    "01014300100000020230201031001000103002202000101003101000301020101000301020102000101320100001"
    "30102010001420012340010101440200000120410102401040210004001001024011400142000010402010012040"
    "14102400010001400100124010410202000001020101000201000202000102020100020200010200010102000001"
    "02020100002102000120010200000210020102200002",
    "02002020202022002000222022000220200000000020220020220000120200011002010020020200001111000002"
    "22000020100100101200002012020000101201002002020000111100000022002200001011001000220022000010"
    "31100100032022200000310110100020023202000031011010000220022030001301011000020220020003130101"
    "02100034020202000431101001000420220020030131010010040432020202000431101001000342222000000140"
    "13010100042302020210003401101000032022020000141001010020020420210004010101200202400020001100"
    "10100240200202040011001010040420202201000010210100002012020003100101020002020203001031100100"
    "02032022000013010110000202302020003110100100020340200200004010310100004032200200003101004100"
    "00020320204000430102101000032020420004311010010004320202200000401013100003202402021000000104"
    "10200320020210000113000200300322020010010031012000320020202002010003200000021020012300201020"
    "04300210003420200000410221000040042122000042001042020004004102020100000422002100042000402410"
    "20021001200040020412200000400412200004200002010200121022000000010001201000010201100000000200"
    "10000100020120000010021200000010010000210010020000110022111002000002",
)
UN = len(ORDER) - 2
RANK = {jg: k for k, jg in enumerate(jg for part in STREAM for jg in part)}


class _Group:
    def __init__(self, n):
        k = n // 2
        self.n = n
        self.side = (range(k), range(k, n))
        self.label = list(range(k)) + list(range(LT - k, LT))
        self.mates = [[b for b in self.side[c < k] if self.label[b] != self.label[c]]
                      for c in range(n)]
        self.plain = [[i for i in range(LT) if i != self.label[c]
                       and i not in [self.label[b] for b in self.mates[c]]] for c in range(n)]
        keys = [(i, c) for c in range(n) for i in range(LT)]
        keys += [("other", c) for c in range(n)]
        keys += [("both", a, b) for a in self.side[0] for b in self.mates[a]]
        self.slot = {key: i for i, key in enumerate(keys)}
        for a in self.side[0]:
            for b in self.mates[a]:
                self.slot["both", b, a] = self.slot["both", a, b]


GROUPS = [_Group(min(GW, FT - g * GW)) for g in range(NG)]
SLOTS = max(GROUPS[0].slot.values()) + 1


def _kind(j, g, ph):
    return 2 if RANK[j, g] < 1 else (RANK[j, g] + ph + (j == 3)) % 2


MATES = ((16, 0, 8), (None, 0, 8), (8, 0, None))


def _out_passes(groups, ph, first=False, last=False):
    passes = {}
    r0 = M * last
    for g in groups:
        grp = GROUPS[g]
        lab = grp.label
        n = 16 + 8 * _kind(3, g, ph)
        now = L if last else n

        def add(i, k, order, what, a, b, *to):
            to = tuple(x for x in to if not (first and x[0] > 0 or last and x[0] < 0))
            passes.setdefault((min(i, k), max(i, k), order, i), []).append((what, g, a, b, to))

        for a, b in zip(grp.side[ph], grp.side[1 - ph]):
            i, k = lab[a], lab[b]
            add(i, i, 0, "own", a, a, (0, i, r0, 0, now - r0, False),
                (2, i, n, now - r0, L - n, False))
            add(k, k, 0, "other", b, b, (0, k, r0, 0, L - r0, False),
                (1, k, L - n + r0, 0, n - r0, True), (-1, k, 0, n, L - n, True))
            if last:
                add(k, k, 0, "closing", b, b, (1, k, L - n, 0, n, False))
            for f in (a, b):
                for k in grp.plain[f]:
                    add(k, k, 0, "plain", f, f, (0, k, r0, 0, L - r0, False))
            for b in grp.mates[a]:
                k = lab[b]
                add(i, k, 1, "both", a, b, (0, i, r0, r0, now - r0, False),
                    (1, k, L - n, 0, n, False))
                add(min(i, k), max(i, k), 2, "cross", a, b,
                    *[(0, t, r0, 0, L - r0, False) for t in sorted((i, k))])
    return sorted(passes.items())


def _parts(ph):
    keys = [(part[0][1], x[-1]) for part in STREAM if part[0][0] == 3
            for _, passes in _out_passes([g for _, g in part], ph) for x in passes]
    if ph == 0:
        keys += [(None, (to,)) for i in range(LT)
                 for to in ((0, i, M, 0, SEG, False), (-1, i, 0, 0, 24, False))]
    return {key: n for n, key in enumerate(dict.fromkeys(keys))}


PARTS = _parts(0), _parts(1)


def _ds(i, n):
    return pl.ds(i * n if isinstance(i, int) else pl.multiple_of(i * n, n), n)


def _dot(a, b):
    return jnp.dot(a, b, preferred_element_type=F32)


def _inverse(x):
    r = pl.reciprocal(x, approx=True)
    return r * (2.0 - x * r)


def _rows(*parts):
    return parts[0] if len(parts) == 1 else lax.concatenate(parts, 0)


def _words(t):
    return pltpu.bitcast(t.astype(BF16), U32)


class _Sums(dict):
    def add(self, key, t, minus=False):
        if key in self:
            u, neg = self[key]
            t, minus = (t + u, neg) if neg == minus else (t - u if neg else u - t, False)
        self[key] = t, minus

    def add_rows(self, key, r0, t, minus=False):
        for r in range(0, t.shape[0], 8):
            self.add((*key, r0 + r), t[r:r + 8], minus)

    def take(self, key):
        t, neg = self.pop(key)
        return -t if neg else t


class _Plan:
    def __init__(self, zero, main):
        self.zero, self.never = zero, zero > 0
        self.tasks = [(k - 1e-6, 0, task) for k, task in enumerate(main)]
        self.latest = {}

    def spread(self, tasks, k0, k1=None):
        step = 0 if k1 is None else (k1 - k0) / len(tasks)
        self.tasks += [(k0 + n * step, step, task) for n, task in enumerate(tasks)]

    def run(self):
        for self.at, self.span, task in sorted(self.tasks, key=lambda x: x[0]):
            task(self)

    def result(self, t):
        self.latest.update({rows: (t, {}) for rows in range(8, t.shape[0] + 1, 8)})
        return t

    def paced(self, t, part=0.0):
        if t.shape[0] not in self.latest:
            return t
        now, cuts = self.latest[t.shape[0]]
        r = min(int((self.at % 1 + part * self.span) * now.shape[0]) // 8 * 8,
                now.shape[0] - t.shape[0])
        if (r, t.dtype) not in cuts:
            now = now[r:r + t.shape[0]]
            cuts[r, t.dtype] = now if t.dtype == F32 else pltpu.bitcast(now, t.dtype)
        return lax.select(self.never, cuts[r, t.dtype], t)


def _task(fn, *args):
    return lambda plan: fn(plan, *args)


def _kernel(ax_hbm, awqkv_hbm, awo_hbm, bx_hbm, mem_hbm, wq_hbm, wk_hbm, wv_hbm, wo_hbm,
            out_hbm,
            ax, awqkv, awo, tmp, aw, xw, qkv_s, oa_s, outa,
            bx, mem, raw, wt, l_tok, l_mem, ahead, y_s, qk_s, v_s, p_s, o_s, o_old, z_part, z_s,
            outb, sem_a, sem_x, sem_w, sem_b, sem_o):
    cp = pltpu.make_async_copy

    def rows_copy(src, dst, r0, r1, sem):
        return cp(src.at[pl.ds(r0, r1 - r0), :], dst.at[pl.ds(r0, r1 - r0), :], sem)

    c_wqkv = [cp(awqkv_hbm.at[:, pl.ds(j * D, D)], awqkv.at[j], sem_a.at[j]) for j in range(3)]
    c_awo = cp(awo_hbm, awo, sem_a.at[3])
    cuts = (0, 2, 3, 7, 11, NB)
    c_ax = [rows_copy(ax_hbm, ax, cuts[c] * TB, cuts[c + 1] * TB, sem_x.at[c]) for c in range(5)]
    c_mem = rows_copy(mem_hbm, mem, 0, M, sem_b.at[0])
    c_bx0 = rows_copy(bx_hbm, bx, 0, (4 + UN) * SEG, sem_b.at[1])
    c_bx1 = rows_copy(bx_hbm, bx, (4 + UN) * SEG, S, sem_b.at[2])
    c_outa = cp(outa, out_hbm.at[:, pl.ds(0, D)], sem_o.at[0])

    def chunk(j, g):
        return 3 * g + j if j < 3 else 3 * NG + g

    def c_w(c):
        j, g = (c % 3, c // 3) if c < 3 * NG else (3, c - 3 * NG)
        n = GROUPS[g].n * 128
        return cp((wq_hbm, wk_hbm, wv_hbm, wo_hbm)[j].at[pl.ds(g * GW * 128, n), :],
                  raw.at[c % RING, pl.ds(0, n), :], sem_w.at[c])

    def c_outb(r0, n):
        return cp(outb.at[pl.ds(r0, n), :], out_hbm.at[pl.ds(r0, n), pl.ds(D, D)], sem_o.at[1])

    def start(copies, priority=1):
        for c in copies:
            c.start(priority=priority)

    def wait(copies):
        for c in copies:
            c.wait()

    def a_weights(j):
        def fill(plan, t):
            tmp[j % 2, t] = (awo[:, t * 128:(t + 1) * 128].astype(F32) if j == 3 else
                             awqkv[j, t * 128:(t + 1) * 128, :].astype(F32).T)

        def move(plan, t, d):
            aw[_ds(j * AD + d, AH // 2), t * 128:(t + 1) * 128] = _words(
                plan.paced(tmp[j % 2, t, pl.ds(d, AH, stride=AD), :]))

        return [task for t in range(LT)
                for task in [_task(fill, t)] + [_task(move, t, d) for d in range(AD)]]

    def a_input(i, b):
        xw[b] = _words(ax[_ds(i, TB), :])

    def a_proj(b, js=range(3), first_block=False):
        def tile(plan, c):
            x = pltpu.bitcast(xw[plan.zero + b], BF16)
            w = pltpu.bitcast(aw[c * 64:(c + 1) * 64, :], BF16)
            r = plan.result(lax.dot_general(x, w, NT, preferred_element_type=F32))
            qkv_s[b, c, HALO:HALO + TB, :] = r
            if c >= LT:
                qkv_s[b, c, 0:HALO, :] = (jnp.broadcast_to(r[0:1, :], (HALO, 128)) if first_block
                                          else qkv_s[1 - b, c, TB:TB + HALO, :])
        return [_task(tile, j * LT + t) for j in js for t in range(LT)]

    def a_attention(b, first_block=False, to=None):
        state = {}

        def window(j, r0, w):
            lo = HALO + r0 - ADIL * w
            return qkv_s[b, j * LT:(j + 1) * LT, lo:lo + 8, :]

        def logits(plan, r0):
            q = jnp.stack([plan.paced(qkv_s[b, t, HALO + r0:HALO + r0 + 8, :], t / LT)
                           for t in range(LT)])
            a = _rows(*[jnp.sum(q * window(1, r0, w), axis=0) for w in range(AW)])
            state[r0] = a + pltpu.roll(a, 2 * AH, 1)

        def fold(plan, r0):
            state[r0] = state[r0] + pltpu.roll(state[r0], AH, 1)

        def weigh(plan, r0):
            a = state[r0].reshape(AW, 8, 128)
            if first_block and r0 < HALO:
                w, pos = [lax.broadcasted_iota(jnp.int32, a.shape, axis) for axis in range(2)]
                a = jnp.where(pos + r0 >= ADIL * w, a, MASKED * AD ** 0.5)
            state[r0] = jnp.exp2((a - jnp.max(a, axis=0)) * (AD ** -0.5 * LOG2E))

        def mix(plan, r0):
            e = state.pop(r0)
            e = [plan.paced(e[w], w / AW) for w in range(AW)]
            o = functools.reduce(jnp.add, (e[w] * window(2, r0, w) for w in range(AW)))
            oa_s[to or b][0, :, r0:r0 + 8, :] = o * _inverse(functools.reduce(jnp.add, e))

        n = TB // 8
        return [_task(f, (k - lag) * 8) for k in range(n + 2)
                for lag, f in ((2, weigh), (0, logits), (1, fold), (2, mix)) if 0 <= k - lag < n]

    def a_out(i, b, depth=LT):
        sums = _Sums()

        def tile(plan, t, k0):
            o = lax.concatenate([oa_s[b][plan.zero, k] for k in range(k0, k0 + depth)], 1)
            n = 48 if depth > 1 else TB
            sums.add(t, _rows(*[_dot(o[r:r + n], pltpu.bitcast(aw[pl.ds(
                pl.multiple_of((plan.zero >> r // n + 3 * b) * 32 + 3 * D // 2 + k0 * 64, 32), depth * 64),
                t * 128:(t + 1) * 128], BF16)) for r in range(0, TB, n)]))
            if k0 + depth == LT:
                outa[_ds(i, TB), t * 128:(t + 1) * 128] = plan.result(sums.take(t)).astype(BF16)
        return [_task(tile, t, k0) for t in range(LT) for k0 in range(0, LT, depth)]

    def tiles_of(c, odd=None, zero=0):
        if isinstance(c, int) and c >= FULL:
            return wt[2 + c - FULL].at[zero]
        return wt[c % 2 if odd is None else odd].at[c // 2 + zero]

    def w_transpose(c, grp, odd=None):
        src, dst = raw.at[c % RING], tiles_of(c, odd)

        def two(plan, i, f):
            t = _words(src[f * 128:(f + 2) * 128, i * 128:(i + 1) * 128].T)
            for k in range(2):
                dst[grp.slot[i, f + k]] = t[:, k * 128:(k + 1) * 128]
        return [_task(two, i, f) for f in range(0, grp.n, 2) for i in range(LT)]

    def w_combine(c, grp, odd=None, transposed=True):
        w, own, other = tiles_of(c, odd, nil), {}, {}

        def edge(plan, r, a, b):
            def tile(i, f, part=0.0):
                if transposed:
                    t = plan.paced(w[grp.slot[i, f], _ds(r, 8)], part)
                else:
                    t = _words(raw[c % RING, _ds(8 * f + r, 16), i * 128:(i + 1) * 128])
                    t = plan.paced(t, part)
                    if i != grp.label[f]:
                        w[grp.slot[i, f], _ds(r, 8)] = t
                return pltpu.bitcast(t, BF16).astype(F32)

            for f in (a, b):
                if f not in own:
                    own[f] = other[f] = tile(grp.label[f], f)
            ta, tb = tile(grp.label[b], a), tile(grp.label[a], b, 0.5)
            w[grp.slot["both", a, b], _ds(r, 8)] = _words(ta + tb)
            own[a], other[a] = own[a] - ta, other[a] + tb
            own[b], other[b] = own[b] - tb, other[b] + ta
            for f, mate in ((a, b), (b, a)):
                if mate == grp.mates[f][-1]:
                    w[grp.slot[grp.label[f], f], _ds(r, 8)] = _words(own.pop(f))
                    w[grp.slot["other", f], _ds(r, 8)] = _words(other.pop(f))
                    for i in grp.plain[f] * (not transposed):
                        tile(i, f)

        return [_task(edge, r, a, b) for r in range(8) for a in grp.side[0] for b in grp.mates[a]]

    places = {}, {}

    def place(memory, *key):
        return places[memory].setdefault(key, len(places[memory]))

    def binade(tiles):
        top = jnp.max(functools.reduce(jnp.maximum, map(jnp.abs, tiles)), axis=1, keepdims=True)
        top = jnp.clip(jnp.broadcast_to(top, (8, 128)), 2.0 ** -60, 2.0 ** 60)
        return pltpu.bitcast(top, jnp.int32) & 0x7F800000

    def memory_operands(ph, known, i, t):
        known[i] = l_mem[ph][0, place(1, "plain", i)] = t
        for k, u in known.items():
            if k != i:
                l_mem[ph][0, place(1, "cross", min(i, k), max(i, k))] = t + u

    def memory_pair(plan, ph):
        cur = [l_mem[ph][0, place(1, "plain", i)] for i in range(LT)]
        shift = binade(cur) - pltpu.bitcast(
            l_tok[ph][plan.zero, place(0, "mate", 0), 8:16], jnp.int32)
        down, up = [pltpu.bitcast(x, F32) for x in (0x3F800000 + shift, 0x3F800000 - shift)]
        l_mem[ph][0, place(1, "down")], l_mem[ph][0, place(1, "up")] = down, up
        for k in range(LT):
            mate = l_tok[ph][plan.zero, place(0, "mate", k), 0:8]
            for kind in range(2):
                l_tok[1 - ph][0, place(0, "other", kind, k), 8:16] = mate - cur[k] * up
            mate = mate * down
            for i in range(LT):
                l_mem[ph][0, place(1, "both", i, k)] = cur[i] - mate if i == k else cur[i] + mate

    def token_operands(x, s, ph):
        def tokens(plan, ds, i):
            t = _words(x[_ds(max(s + ds, 0), SEG), i * 128:(i + 1) * 128])
            return pltpu.bitcast(plan.paced(t), BF16).astype(F32)

        def one(plan, i, kind):
            before, cur, after, later = [tokens(plan, ds, i) for ds in range(-1, 3)]
            third = (after[16:24], before[16:24], after[8:16])[kind]
            at = place(0, "other", kind, i)
            l_tok[ph][0, at, 0:8] = cur[0:8] - before[24:32]
            l_tok[ph][0, at, 16:32] = cur[16:32] - _rows(third, after[0:8])
            if kind < 2:
                l_tok[ph][0, place(0, "own", kind, i), 0:SEG] = _rows(later[:16 + 8 * kind],
                                                              cur[16 + 8 * kind:])
                return
            l_tok[ph][0, at, 8:16] = cur[8:16] - before[16:24]
            l_tok[ph][0, place(0, "plain", i), 0:SEG] = cur
            l_tok[ph][0, place(0, "mate", i), 0:8] = after[8:16]
            if s == 0:
                l_tok[ph][0, place(0, "next", i), 0:SEG] = after

        def two(plan, i, k):
            cur, after = tokens(plan, 0, i), tokens(plan, 1, k)
            if i < k:
                l_tok[ph][0, place(0, "cross", i, k), 0:SEG] = cur + tokens(plan, 0, k)
            fourth = cur[24:32] + after[0:8]
            l_tok[ph][0, place(0, "both", i, k), 0:SEG] = _rows(cur[16:24] + after[8:16], fourth,
                                                         cur[16:24] + after[16:24], fourth)

        def magnitude(plan):
            l_tok[ph][0, place(0, "mate", 0), 8:16] = pltpu.bitcast(
                binade([tokens(plan, 1, i)[8:16] for i in range(LT)]), F32)

        return [magnitude] + [task for i in range(LT) for task in
                              [_task(one, i, kind) for kind in range(3)]
                              + [_task(two, i, k) for k in range(LT) if k != i]]

    def segment(s, ph, operands, first=False, last=False):
        zero = nil if isinstance(s, int) else s >> 16
        zeros, uses = [zero >> k for k in range(3)], {}

        def again(*key):
            uses[key] = uses.get(key, 0) + 1
            return zeros[uses[key] % len(zeros)]

        def product(plan, parts, j, g, key):
            w = tiles_of(chunk(j, g))[GROUPS[g].slot[key]]
            return plan.result(_dot(_rows(*parts), pltpu.bitcast(w, BF16)))

        pieces = {}

        def project(j, g):
            grp, f0, kind = GROUPS[g], g * GW, _kind(j, g, ph)
            lab = grp.label
            late = 16 + 8 * (kind == 1)
            lo, end = 0 if first else late, SEG if last and j == 0 else L
            y, gift, kept = _Sums(), _Sums(), []
            left = {a: LT for a in grp.side[ph]}
            owed = {a: 1 + len(grp.mates[a]) for a in grp.side[ph]}

            def tok(r0, r1, *key):
                return [l_tok[ph][again(*key), place(0, *key), r0:r1]]

            def memory(*key):
                at = again(1, *key) if kind < 2 else 0
                return [l_mem[ph][at, place(1, *key)]] * (end == L)

            def keep(f, r0, t, minus=False):
                y_s[chunk(j, g)][0, len(kept), r0:end] = t
                pieces.setdefault((j, f0 + f), []).append((len(kept), r0, minus))
                kept.append(f)

            def add(a, t):
                y.add(a, t)
                left[a] -= 1
                if not left[a]:
                    keep(a, 0, y.take(a))

            def give(a, t):
                if last:
                    return
                gift.add(a, t)
                owed[a] -= 1
                if not owed[a]:
                    t = gift.take(a)
                    for r, mate in zip((16, 24, 32), MATES[kind]):
                        if mate is not None:
                            u = t[r - lo:r - lo + 8]
                            ahead[ph][0, j, f0 + a, 0, mate:mate + 8] = (
                                u if r < SEG else u * memory("up")[0])

            def own(plan, a):
                parts = tok(0, late if first else SEG, "own", kind % 2, lab[a]) * (not last)
                parts += tok(lo, SEG, "plain", lab[a]) if first or last else []
                t = product(plan, parts + memory("plain", lab[a]), j, g, (lab[a], a))
                old = [] if first else [ahead[ph][0, j, f0 + a, 1, 0:late]]
                if not last:
                    ahead[ph][0, j, f0 + a, 1, 0:late] = t[:late]
                    t = t[late:]
                add(a, _rows(*old, t))
                give(a, t)

            def opening(plan, b):
                n = 16 + 8 * (kind == 0)
                ahead[1 - ph][0, j, f0 + b, 1, 0:n] = product(
                    plan, tok(0, n, "next", lab[b]), j, g, (lab[b], b))

            def other(plan, b):
                k = lab[b]
                parts = tok(0, late, "plain", k) if first else []
                parts += tok(late - lo, late if last else SEG, "other", kind, k)
                parts += tok(late, SEG, "plain", k) if last else []
                parts += memory("plain", k) if last or kind == 2 else memory("both", k, k)
                at = 0 if first else zero
                got = [] if first else [ahead[1 - ph][at, j, f0 + b, 0, 0:late]]
                for r, mate in zip((16, 24, 32), MATES[kind] * (not last)):
                    if mate is not None:
                        u = ahead[1 - ph][at, j, f0 + b, 1, mate:mate + 8]
                        got.append(u if r < SEG else plan.paced(u) * memory("down")[0])
                t, got = product(plan, parts, j, g, ("other", b)), _rows(*got)
                r0, r1 = late - lo, late - lo + got.shape[0]
                t = _rows(*[t[:r0] for _ in range(r0 > 0)], t[r0:r1] + got,
                          *[t[r1:] for _ in range(r1 < end)])
                y.add(b, t)

            def both(plan, a, b):
                i, k = lab[a], lab[b]
                parts = tok(0, late, "plain", i) if first else []
                parts += tok(late, SEG, "plain", i) if last else tok(
                    *((0, 16) if kind == 2 else (late, SEG)), "both", i, k)
                parts += memory("plain", i) if last or kind == 2 else memory("both", i, k)
                t = product(plan, parts, j, g, ("both", a, b))
                give(a, t)
                if first:
                    y.add(b, t)
                elif b in y:
                    u = y.take(b)
                    keep(b, 0, _rows(u[:lo], u[lo:] + t))
                else:
                    keep(b, lo, t)

            def cross(plan, a, b):
                key = "cross", *sorted((lab[a], lab[b]))
                t = product(plan, tok(0, SEG, *key) + memory(*key), j, g, (lab[b], a))
                add(a, t)
                y.add(b, t, True)
                keep(b, 0, *y.pop(b))

            def plain(plan, i, f):
                t = product(plan, tok(0, SEG, "plain", i) + memory("plain", i), j, g, (i, f))
                (add if f in left else y.add)(f, t)

            passes = []
            others = list(grp.side[1 - ph])
            for a, b0 in zip(grp.side[ph], others[grp.n == GW:] + others):
                passes += [((), _task(opening, b0), 1, 16 + 8 * (kind == 0))] * first
                passes += [((lab[a],), _task(own, a), 0, end + late * (first - last)),
                           ((lab[b0],), _task(other, b0), 0, end)]
                passes += [((i,), _task(plain, i, f), 0, end)
                           for f in (a, b0) for i in grp.plain[f]]
                passes += [((lab[a],), _task(both, a, b), (2 - kind % 2) * (not first), end - lo)
                           for b in grp.mates[a]]
                passes += [((lab[a], lab[b]), _task(cross, a, b), 0, end) for b in grp.mates[a]]
            return passes

        n = SEG if last else L
        row, col = [lax.broadcasted_iota(jnp.int32, (L, 2 * n), axis) for axis in range(2)]
        head0 = col < n
        query = jnp.where(head0, col, col - n) + (L - n)
        visible = (query < M) | (row >= SEG) | (query >= row + M)
        scores = _Sums()

        def gather(j, f):
            sums, end = _Sums(), L if j else n

            def add_up(plan, part):
                todo = pieces[j, f]
                for k, (at, r0, minus) in enumerate(todo[part::2]):
                    u = y_s[chunk(j, f // GW)][zero, at, r0:end]
                    sums.add(r0, u if k else plan.paced(u), minus)
                if part < 2 - 1:
                    return
                t = sums.take(0)
                for r0 in list(sums):
                    t = _rows(t[:r0], t[r0:] + sums.take(r0))
                if j == 1:
                    qk_s[f][0, 1, 0:L] = pltpu.bitcast(t, U32)
                    return
                if j == 0 and not last:
                    t = _rows(t[SEG:], t[:SEG])
                pad = [jnp.zeros((8, 128), F32)] * (end % 16 // 8)
                if f % 3 == 1:
                    low = lax.broadcasted_iota(jnp.int32, t.shape, 1) < 64
                    t = _words(_rows(jnp.where(low, t, 0.0), jnp.where(low, 0.0, t)))
                else:
                    t = _words(_rows(*[t, *pad][::1 - f % 3]))
                (v_s if j else qk_s)[f][0, 0, 0:t.shape[0]] = t

            return [_task(add_up, part) for part in range(2)]

        def by_head(ref, f, rows, short=False):
            t = ref[f][zero, 0, 0:rows if f % 3 == 1 else pl.cdiv(rows, 16) * 8]
            if f % 3 == 2 or f % 3 == 0 and not short:
                t = _rows(*[t, jnp.zeros((rows - t.shape[0], 128), U32)][::1 - f % 3])
            return pltpu.bitcast(t, BF16)

        def score(plan, f):
            k = pltpu.bitcast(qk_s[f][zero, 1, 0:L], F32)
            scores.add(f // 3, lax.dot_general(k, by_head(qk_s, f, n), NT,
                                               preferred_element_type=F32))
            if f % 3 == 2:
                sc = jnp.where(visible, scores.take(f // 3), MASKED * DH ** 0.5)
                e = jnp.exp2((sc - jnp.max(sc, axis=0, keepdims=True)) * (DH ** -0.5 * LOG2E))
                p = e * _inverse(jnp.sum(e, axis=0, keepdims=True))
                p = _rows(jnp.where(head0, p, 0.0), jnp.where(head0, 0.0, p)).T
                p_s[f // 3][0, 0:3 * n, 0:2 * L] = _rows(p[:n], p[:n] + p[n:], p[n:])

        def mix(plan, f):
            v = by_head(v_s, f, L, True)
            o = _dot(p_s[f // 3][zero, _ds(f % 3, n), 0:v.shape[0]], v)
            if last:
                o = _rows(jnp.zeros((M, 128), F32), o)
            g = f // GW
            o_s[ph][g][0, f % GW] = o
            if not first and f % GW in GROUPS[g].side[1 - ph]:
                k = 16 + 8 * _kind(3, g, ph)
                o_old[1 - ph][0, f, 0:k] = o[:k] + o_s[1 - ph][g][zero, f % GW, L - k:]

        z = _Sums()

        def out_project(groups):
            def run(plan, part, left, what, g, a, b, to):
                k, r0, i = 16 + 8 * _kind(3, g, ph), L - n, to[0][1]

                def cur(f, r0, r1=L):
                    return o_s[ph][g][again(g, f), f, r0:r1]

                def joined(r0):
                    t = cur(b, r0, k)
                    if not first:
                        t = t + o_s[1 - ph][g][again(1, g, a), a, L - k + r0:]
                    return [t, cur(b, k)] if last else [t]

                if what == "own":
                    old = [] if first else [o_old[ph][zero, g * GW + a, 0:L - k]]
                    t = product(plan, joined(r0) + old, 3, g, (i, a))
                elif what == "closing":
                    t = product(plan, [o_old[1 - ph][0, g * GW + b, 0:k]], 3, g, (i, b))
                elif what == "both":
                    t = product(plan, joined(0), 3, g, (what, a, b))
                elif what == "cross":
                    t = product(plan, [cur(a, r0) - cur(b, r0)], 3, g, (GROUPS[g].label[b], a))
                else:
                    t = product(plan, [cur(b, r0)], 3, g, (what if what == "other" else i, b))
                part.add(to, t)
                left.remove(to)
                if to in left:
                    return
                t = part.take(to)
                for back, i, dst, src, rows, minus in to:
                    if first or last:
                        z.add_rows((back, i), dst, t[src:src + rows], minus)
                    elif back == 0:
                        z.add((0, i, 0), t[:M])
                if not first and not last:
                    r0 = M * all(x[0] % 2 == 0 for x in to)
                    z_part[ph][0, PARTS[ph][groups[0], to], r0:t.shape[0]] = t[r0:]

            tasks = [], []
            for (lo, hi, order, i), passes in _out_passes(groups, ph, first, last):
                part, left = _Sums(), [x[-1] for x in passes]
                tasks[order == 1].extend(
                    ((lo, hi) if order == 2 else (i,), _task(run, part, left, *x),
                     (order == 1) * (1 + _kind(3, x[1], ph)), max(t[3] + t[4] for t in x[-1]))
                    for x in passes)
            order = [((k // 4 + 0.5) / len(xs), short, k) for short, xs in enumerate(tasks)
                     for k in range(len(xs))]
            return [tasks[short][k] for _, short, k in sorted(order)]

        main, begin, done = [], {}, {}
        parts = FIRST if first else STREAM
        for part in parts:
            if part[0][0] == 3:
                new = out_project([g for _, g in part])
            else:
                new = [project(*jg) for jg in part]
                new = [x for k in range(0, len(new[0]), GW) for xs in new for x in xs[k:k + GW]]
            if part is parts[0] and not first:
                new.sort(key=lambda x: max(x[0]) == LT - 1)
            if part is parts[-1]:
                new.sort(key=lambda x: min(x[0]) == LT - 1)
            begin.update({jg: len(main) for jg in part})
            main += new
            done.update({jg: len(main) for jg in part})

        lag_s, lag_n, lag_v, lag_o = 36, 68, 34, 26
        ready, extra = {}, []
        for stage, js in ((score, (0, 1)), (mix, (2,))):
            at = -GW
            for f in range(FT):
                due = [begin[3, k // GW] if stage is mix else begin[3, k // 3 * 3 // GW] - lag_n
                       for k in range(f, FT)]
                step = min([GW] + [(x - lag_o - at) / k for k, x in enumerate(due, 1)])
                whole = max(done[j, f // GW] for j in js)
                at = max(at + max(step, 0.01), whole + lag_s if stage is score else
                         max(whole + lag_v, ready[f // 3] + lag_n))
                assert at < begin[3, f // GW] - 1
                if stage is score:
                    ready[f // 3] = at
                extra.append((at, stage, js, f, whole))
        queues = [[x for x in main if x[2] == q] for q in range(3)] + [extra[:FT], extra[FT:]]
        queues.append([((), task) for task in a_out(NB - 1, 2, 1) * first])
        main, extra = [], []
        for q in map(int, ORDER[0 if first else -1 if last else 2 - ph]):
            x = queues[q].pop(0)
            if q < 3:
                main.append(x)
            else:
                extra.append((len(main) - 1 + len(extra) * 1e-4, *x[1:]))
        plan = _Plan(zero, [x[1] for x in main])
        for at, stage, *rest in extra:
            if not rest:
                plan.spread([stage], at)
                continue
            js, f, whole = rest
            k0 = max(at - 38, whole - 1)
            plan.spread([t for j in js for t in gather(j, f)], k0, max(at - 28, k0))
            plan.spread([_task(stage, f)], at)

        if first:
            def arrive(plan, groups):
                wait([c_w(chunk(3, g)) for g in groups])
                start([c_w(chunk(3, g + 3)) for g in groups if g + 3 < NG])

            plan.spread([t for j in (1, 2) for t in w_transpose(FULL + j, GROUPS[-1])], 0)
            ends = 340, 640, 770, 880, begin[3, 4]
            plan.spread([t for j in range(3) for t in w_combine(FULL + j, GROUPS[-1])], 0, ends[0] - 8)
            for groups, k0, k1 in zip(((0, 1), (2,), (3,), (4,)), ends, ends[1:]):
                plan.spread([_task(arrive, groups)], k0)
                plan.spread([t for g in groups
                             for t in w_combine(chunk(3, g), GROUPS[g], None, False)], k0, k1 - 8)
        else:
            def resume(plan):
                for i in range(LT):
                    if not last:
                        z.add((0, i, 0), z_s[1 - ph][zero, 2, i, 0:M])
                        continue
                    for back in range(3):
                        z.add_rows((back, i), M, z_s[1 - ph][zero, (back - 1) % 3, i,
                                                            M:L if back else 24])

            plan.spread(settle(s - 1, 1 - ph), 30, 130)
            plan.spread([resume], begin[3, 0] - 1)
        if not last:
            k0 = 945 if first else 800
            plan.spread(operands, k0, k0 + 100)
            plan.spread([_task(memory_pair, ph)], 0)
            known = {}
            for i in range(LT):
                plan.spread([lambda _, i=i: memory_operands(1 - ph, known, i, z.take((0, i, 0)))],
                            max(k for k, (tiles, *_) in enumerate(main) if i in tiles))
        plan.run()
        for back in (2, 1, 0) * last:
            for i in range(LT):
                outb[_ds(s - back, SEG), i * 128:(i + 1) * 128] = _rows(
                    *[z.take((back, i, r)) for r in range(M, L, 8)]).astype(BF16)
        for (g, ((back, i, r0, _, rows, _), *_)), at in PARTS[ph].items():
            if g is None:
                z_part[ph][0, at, 0:rows] = _rows(
                    *[z.take((back, i, r)) for r in range(r0, r0 + rows, 8)]
                ) if first else jnp.zeros((rows, 128), F32)

    def settle(s, ph):
        found, sums = {}, _Sums()
        for (_, to), at in PARTS[ph].items():
            for back, i, dst, src, rows, minus in to:
                skip = M * (back == dst == 0)
                found.setdefault((i, back), []).append(
                    (at, dst + skip, src + skip, rows - skip, minus))

        def add(plan, some):
            for k, (at, dst, src, rows, minus) in enumerate(some):
                u = z_part[ph][plan.zero, at, src:src + rows]
                sums.add((dst, rows), u if k else plan.paced(u), minus)

        def finish(plan, i, back):
            t = _Sums()
            if back >= 0:
                t.add_rows((), M, z_s[1 - ph][plan.zero, (back - 1) % 3, i, M:L if back else 24])
            for dst, rows in list(sums):
                t.add_rows((), dst, *sums.pop((dst, rows)))
            r0 = min(t)[0]
            t = _rows(*[t.take(r) for r in sorted(t)])
            if back < 2:
                z_s[ph][0, back % 3, i, r0:r0 + t.shape[0]] = t
            else:
                seg = max(s - 2, 0) if isinstance(s, int) else jnp.maximum(s - 2, 0)
                outb[_ds(seg, SEG), i * 128:(i + 1) * 128] = t.astype(BF16)

        return [task for key, xs in sorted(found.items()) for task in
                [_task(add, xs[k:k + 4]) for k in range(0, len(xs), 4)] + [_task(finish, *key)]]

    def clear(k, carry):
        z_part[0][0, _ds(k, 4)] = jnp.zeros((4, L, 128), F32)
        return lax.shift_right_logical(k, 16)

    def with_weights(plan, first, groups):
        for b, grp in enumerate(groups):
            new, before = [k if isinstance(k, int) else jnp.where(k < 0, k + RING, k)
                           for k in (first + b, first + b - 1)]
            p0 = 7.5
            plan.spread(w_combine(before, GROUPS[0], b), p0 * b, p0 * (b + 1))
            plan.spread(w_transpose(new, grp, 1 - b), p0 * b, p0 * (b + 1))

    def a_step(it, carry):
        for k in range(FULL // 2):
            @pl.when(it == k)
            def _():
                wait([c_w(c) for c in (2 * k - 1, 2 * k) if c >= 0]
                     + {1: [c_ax[3]], 3: [c_ax[4]]}.get(k, []))
                start([c_w(2 * k + 2), c_w(2 * k + 3)])
                start({0: [c_ax[3]], 2: [c_ax[4]], 4: [c_mem, c_bx0]}.get(k, []), 0)
        plan = _Plan(nil, a_out(2 * it, 0) + a_out(2 * it + 1, 1) + a_proj(1) + a_proj(0))
        with_weights(plan, 2 * it - 1, [GROUPS[0]] * 2)
        plan.spread(a_attention(0), 15.5, 24.99)
        plan.spread(a_attention(1), 24.99, 38.5)
        plan.run()
        for b in range(2):
            a_input(jnp.minimum(2 * it + 6 - b, NB - 1), b)
        return carry

    def b_step(it, carry):
        @pl.when(it == 1)
        def _():
            c_bx1.wait()
        x = bx.at[pl.ds(pl.multiple_of(it * UN * SEG, UN * SEG), (4 + UN) * SEG)]
        for u in range(1, UN + 1):
            segment(it * UN + u, u % 2, token_operands(x, u + 1, 1 - u % 2))

        @pl.when(it > 1)
        def _():
            c_outb(pl.multiple_of((it - 2) * UN * SEG, UN * SEG), UN * SEG).start()
        return carry

    start([c_wqkv[0], c_ax[0], c_wqkv[1]])
    nil = lax.fori_loop(0, z_part[0].shape[1] // 4, clear, 0)
    z_s[1][...] = jnp.zeros(z_s[1].shape, F32)
    bx[S:, :] = jnp.zeros((2 * SEG, D), BF16)
    wait([c_wqkv[0]])
    start([c_wqkv[2]])
    _Plan(nil, a_weights(0)).run()
    wait([c_ax[0]])
    start([c_ax[1]])
    for b in range(2):
        a_input(b, b)
    _Plan(nil, a_proj(0, [0])).run()
    for j, copy in ((1, c_awo), (2, c_ax[2])):
        wait([c_wqkv[j]])
        start([copy])
        plan = _Plan(nil, a_proj(1, [j - 1]) + a_proj(0, [j], True))
        plan.spread(a_weights(j), 0, 2)
        plan.run()
    wait([c_ax[1], c_awo])
    start([c_w(0), c_w(1)])
    a_input(2, 0)
    plan = _Plan(nil, a_proj(1, [2]) + a_proj(0))
    plan.spread(a_attention(0, True), 0, 4.99)
    plan.spread(a_attention(1), 9, 18.5)
    plan.spread(a_weights(3), 9, 18.5)
    plan.run()
    wait([c_ax[2]])
    for b in range(2):
        a_input(4 - b, b)
    lax.fori_loop(0, FULL // 2, a_step, 0)
    wait([c_mem, c_bx0, c_w(FULL - 1), c_w(FULL), c_w(FULL + 1)])
    start([c_w(FULL + 2), c_w(FULL + 3), c_w(FULL + 4)])
    plan = _Plan(nil, a_out(NB - 4, 0) + a_proj(1) + a_out(NB - 3, 1) + a_out(NB - 2, 0))
    with_weights(plan, FULL - 1, [GROUPS[0], GROUPS[-1]])
    plan.spread(a_attention(0), 14, 21.0)
    plan.spread(a_attention(1, to=2), 21.0, 29)
    plan.spread(token_operands(bx, 0, 0), 16, 28)
    plan.run()
    wait([c_w(FULL + 2)])
    start([c_w(FULL + 5)])
    known = {}
    for i in range(LT):
        memory_operands(0, known, i, mem[0:M, i * 128:(i + 1) * 128].astype(F32))
    segment(0, 0, token_operands(bx, 1, 1), first=True)
    start([c_bx1, c_outa])
    steps = (NSEG - 2) // UN
    lax.fori_loop(0, steps, b_step, 0)
    c_outb((steps - 2) * UN * SEG, (2 * UN - 2) * SEG).start()
    for s in range(steps * UN + 1, NSEG - 1):
        segment(s, s % 2, token_operands(bx, s + 1, 1 - s % 2))
    segment(NSEG - 1, 1, None, last=True)
    c_outb((steps * UN - 2) * SEG, S - (steps * UN - 2) * SEG).start()
    wait([c_outa, c_outb(0, S)])


def pallas_concat_heads__sliding_local_dilated__memory_aug_recurrent_mem_tr__prompt_kernel(
    A_x, A_wqkv, A_wo, B_x, B_mem0, B_Wq, B_Wk, B_Wv, B_Wo, B_seg_len,
):
    assert B_seg_len == SEG
    assert A_x.shape == B_x.shape == (1, S, D) and B_mem0.shape == (1, M, D)
    assert B_Wq.shape == B_Wk.shape == B_Wv.shape == (D, H, DH) and B_Wo.shape == (H, DH, D)
    dma = pltpu.SemaphoreType.DMA

    def vmem(dtype, *shape):
        assert math.prod(shape) * jnp.dtype(dtype).itemsize % 16384 == 0, shape
        return pltpu.VMEM(shape, dtype)

    call = pl.pallas_call(
        _kernel,
        out_shape=jax.ShapeDtypeStruct((S, 2 * D), BF16),
        in_specs=[pl.BlockSpec(memory_space=pl.ANY)] * 9,
        out_specs=pl.BlockSpec(memory_space=pl.ANY),
        scratch_shapes=[
            vmem(BF16, S, D),
            vmem(BF16, 3, D, D),
            vmem(BF16, D, D),
            vmem(F32, 2, LT, D, 128),
            vmem(U32, 2 * D, D),
            vmem(U32, 2, TB // 2, D),
            vmem(F32, 2, 3 * LT, HALO + TB, 128),
            [vmem(F32, 1, LT, TB, 128)] * 3,
            vmem(BF16, S, D),
            vmem(BF16, S + 2 * SEG, D),
            vmem(BF16, 64, D),
            vmem(BF16, RING, GW * 128, D),
            [vmem(U32, n, SLOTS, 64, 128) for n in [FULL // 2] * 2 + [1] * 8],
            [vmem(F32, 1, 72, 40, 128)] * 2,
            [vmem(F32, 1, 44, M, 128)] * 2,
            [vmem(F32, 1, 3, FT, 2, 24, 128)] * 2,
            [vmem(F32, 1, 52, L, 128)] * (3 * NG),
            [vmem(U32, 1, 2, 48, 128)] * FT,
            [vmem(U32, 1, 1, 64, 128)] * FT,
            [vmem(F32, 1, 128, 128)] * (FT // 3),
            [[vmem(F32, 1, 12, L, 128)] * NG] * 2,
            [vmem(F32, 1, FT, 24, 128)] * 2,
            [vmem(F32, 1, pl.cdiv(len(PARTS[0]), 4) * 4, L, 128)] * 2,
            [vmem(F32, 1, 4, LT, L, 128)] * 2,
            vmem(BF16, S, D),
            dma((4,)), dma((5,)), dma((4 * NG,)), dma((3,)), dma((2,)),
        ],
        compiler_params=pltpu.CompilerParams(
            vmem_limit_bytes=126 * 1024 * 1024,
            flags={"XLA_TPU_EVENLY_DISTRIBUTE_CRITICAL_NODES": True}),
        name="sliding_and_memory_attention",
    )

    def by_feature(w):
        return w.transpose(1, 2, 0).reshape(H * DH, D)

    out = call(A_x.reshape(S, D), A_wqkv, A_wo, B_x.reshape(S, D), B_mem0.reshape(M, D),
               by_feature(B_Wq), by_feature(B_Wk), by_feature(B_Wv), B_Wo.reshape(H * DH, D))
    return out.reshape(1, S, 2 * D)
```

```python
import functools
import math

import jax
import jax.numpy as jnp
from jax import lax
from jax.experimental import pallas as pl
from jax.experimental.pallas import tpu as pltpu

F32, BF16, U32 = jnp.float32, jnp.bfloat16, jnp.uint32
NT = (((1,), (1,)), ((), ()))
MASKED = -1000000000.0
LOG2E = math.log2(math.e)

S, D = 2048, 640
LT = D // 128

AH, AD, AW, ADIL = 32, 20, 8, 2
HALO = 16
TB = 128
NB = S // TB

H, DH, M, SEG = 32, 192, 8, 32
L = M + SEG
FT = H * DH // 128
NSEG = S // SEG
GW = 2 * LT
NG = pl.cdiv(FT, GW)
FULL = 3 * (NG - 1)
RING = 8


def _stream(text):
    return [[("qkvo".index(w[0]), int(w[1])) for w in part.split("+")] for part in text.split(",")]


FIRST = _stream("v0,v1,q0,k0,q1,k1,q2,k2,v2,q3,k3,v3,q4,k4,v4,o0+o1+o2,o3,o4")
STREAM = _stream("q0,k0+v0,q1+k1,v1+q2,k2+v2,q3+k3,q4+k4,v3+v4,o0+o1+o2,o3+o4")
ORDER = (
    "10000000000010000001000000000000100000000001000000000001000000010000000000100000000000010000"
    "00010000000000000001000000100000000000000100000100000000000000010000000000100000000100000001"
    "00000000000100000000000100000000000010000001000000000001000000000001000000000103003000000000"
    "03010000000010030000001000000003000010030000000100003000000000103000001000030000031040000400"
    "00000100000000134000043000000000010400000103000430000001040000030000000001034000003014000000"
    "00000300100400000001030000030010404000000100000000001340000300004000000134000000001004000003"
    "00000010040030003104000000000003010040000000010300000100403000400000100430000000000010000004"
    "00001004000000014000000001004000000104000000000104000000000103000040000003000143000000000100"
    "30000000013000000000300001000000001000300000300100000000000301000000014004300000000010000000"
    "40104000000000100000400000010040000003000100301140042012055520135000010100321401002100553515"
    "00002000211013001020355551000000001032114100255501500020101001040200021551541500002010102400"
    "01120555140500001001004024020101250100010004100204120200000222200020200200020020020202200202"
    "0020000212000101010000000101011000010110000101000",
    "20200020200202202002002020220020202000020220200000222020000101101000000202202001011010000002"
    "22200000011110000020202200000111100000020220200001111000000022220000001110100002022020000011"
    "10103000202300122000001100102023002020001110130002022030032000011110000020202230003110100010"
    "00023020202010141001300300222402000101014300100202020240300101301014000202002402300101001140"
    "30000223024002001130011400002022023400010101010300200242020000101011400000222024000010114000"
    "10202020240001001104010000220240001201010140000202200200001110100300020202200001110030102003"
    "02002010320010001120300022200100310000103100220000200110401300002032402000001010341000000220"
    "40230000101041300000220202430001001140103000022230240030010104001002400220300001200114003000"
    "22023400200001101030002032020200013001101000020202320000020102030102030201020002020102300231"
    "00200200030124020102402004124000002010240012400220410400002020102404012402000204001002010224"
    "02401024040000201020012400202410000002200120001000100120001001200010012000000010120000201020"
    "01200000011000200010201000110020201010202100",
    "00222020000220200220200020202020202000202020020000111010000022200200001110100000222002000011"
    "10100002022002000011101000020220020000111010000002202200001110100002022002000011101000002220"
    "02000011101300020020302002130011010030202020200010101013000002322020000001131100020032200000"
    "31201100002102042002300100311041000202023400200100114010303002202024000130101014000002224020"
    "30000311011400020023022400010011040130020020022300011401000100022202400010100411000402020202"
    "00001101400020120240020000114010001002224000201010101000002020202010101010300200322002000110"
    "13003100002202000201011301030002022002000001311000104022002023000013401001000034202002000014"
    "01013000002430202000013401000010002240230000013101140003002240202001010014013000004202030201"
    "01010143000000020232000113010100000230022000010110013000010230011003010200012001031020010010"
    "30102001002140014230001101404002000210140402101002400104000102101404002110104400002010104010"
    "42140002000140020110400210410102000010010102000020120020000210020012000210000001001220000012"
    "00021000001200021001002200001201000202020002",
    "00002202022022202200002022000200220020000000220020002000022200000011101000002220200000111010"
    "00002220200000111012000002220000011010010020220100200101100002000022200001001110000022003220"
    "10010100100002230022000011103010003022002321000001110003022000322000011110000002220023003001"
    "01034110000220202400031001011400020220303210004001041310020220003420000101032411000020220000"
    "03111140040320020200200100041110303202000014220000111004000202202040001001011020420000422000"
    "01100242110000002241000011100004022220000000101101002022200000001100133100022022000003110001"
    "10000203203220000111003100020200322000011110004300002002042300000110100040300220034200100010"
    "04310020000202400300101013004020020322000410111000400032022002004021010304310002220000210100"
    "40210033001200102002001003200000321010020200012130002020030000020012023000000302021103000202"
    "01020400030412002020040001220001440000044212200200014220000000102042010400022400014200004012"
    "02200004101220004001004202200040042002010201000201020000212200000010021000010002001001100020"
    "01000001000020010200000120010200000100010000020101210112020000011022",
)
UN = len(ORDER) - 2
RANK = {jg: k for k, jg in enumerate(jg for part in STREAM for jg in part)}


class _Group:
    def __init__(self, n):
        k = n // 2
        self.n = n
        self.side = (range(k), range(k, n))
        self.label = list(range(k)) + list(range(LT - k, LT))
        self.mates = [[b for b in self.side[c < k] if self.label[b] != self.label[c]]
                      for c in range(n)]
        self.plain = [[i for i in range(LT) if i != self.label[c]
                       and i not in [self.label[b] for b in self.mates[c]]] for c in range(n)]
        keys = [(i, c) for c in range(n) for i in range(LT)]
        keys += [("other", c) for c in range(n)]
        keys += [("both", a, b) for a in self.side[0] for b in self.mates[a]]
        self.slot = {key: i for i, key in enumerate(keys)}
        for a in self.side[0]:
            for b in self.mates[a]:
                self.slot["both", b, a] = self.slot["both", a, b]


GROUPS = [_Group(min(GW, FT - g * GW)) for g in range(NG)]
SLOTS = max(GROUPS[0].slot.values()) + 1


def _kind(j, g, ph):
    return 2 if RANK[j, g] < 1 else (RANK[j, g] + ph + (j == 3)) % 2


MATES = ((16, 0, 8), (None, 0, 8), (8, 0, None))


def _out_passes(groups, ph, first=False, last=False):
    passes = {}
    r0 = M * last
    for g in groups:
        grp = GROUPS[g]
        lab = grp.label
        n = 16 + 8 * _kind(3, g, ph)
        now = L if last else n

        def add(i, k, order, what, a, b, *to):
            to = tuple(x for x in to if not (first and x[0] > 0 or last and x[0] < 0))
            passes.setdefault((min(i, k), max(i, k), order, i), []).append((what, g, a, b, to))

        for a, b in zip(grp.side[ph], grp.side[1 - ph]):
            i, k = lab[a], lab[b]
            add(i, i, 0, "own", a, a, (0, i, r0, 0, now - r0, False),
                (2, i, n, now - r0, L - n, False))
            add(k, k, 0, "other", b, b, (0, k, r0, 0, L - r0, False),
                (1, k, L - n + r0, 0, n - r0, True), (-1, k, 0, n, L - n, True))
            if last:
                add(k, k, 0, "closing", b, b, (1, k, L - n, 0, n, False))
            for f in (a, b):
                for k in grp.plain[f]:
                    add(k, k, 0, "plain", f, f, (0, k, r0, 0, L - r0, False))
            for b in grp.mates[a]:
                k = lab[b]
                add(i, k, 1, "both", a, b, (0, i, r0, r0, now - r0, False),
                    (1, k, L - n, 0, n, False))
                add(min(i, k), max(i, k), 2, "cross", a, b,
                    *[(0, t, r0, 0, L - r0, False) for t in sorted((i, k))])
    return sorted(passes.items())


def _parts(ph):
    keys = [(part[0][1], x[-1]) for part in STREAM if part[0][0] == 3
            for _, passes in _out_passes([g for _, g in part], ph) for x in passes]
    if ph == 0:
        keys += [(None, (to,)) for i in range(LT)
                 for to in ((0, i, M, 0, SEG, False), (-1, i, 0, 0, 24, False))]
    return {key: n for n, key in enumerate(dict.fromkeys(keys))}


PARTS = _parts(0), _parts(1)


def _ds(i, n):
    return pl.ds(i * n if isinstance(i, int) else pl.multiple_of(i * n, n), n)


def _dot(a, b):
    return jnp.dot(a, b, preferred_element_type=F32)


def _inverse(x):
    r = pl.reciprocal(x, approx=True)
    return r * (2.0 - x * r)


def _rows(*parts):
    return parts[0] if len(parts) == 1 else lax.concatenate(parts, 0)


def _words(t):
    return pltpu.bitcast(t.astype(BF16), U32)


class _Sums(dict):
    def add(self, key, t, minus=False):
        if key in self:
            u, neg = self[key]
            t, minus = (t + u, neg) if neg == minus else (t - u if neg else u - t, False)
        self[key] = t, minus

    def add_rows(self, key, r0, t, minus=False):
        for r in range(0, t.shape[0], 8):
            self.add((*key, r0 + r), t[r:r + 8], minus)

    def take(self, key):
        t, neg = self.pop(key)
        return -t if neg else t


class _Plan:
    def __init__(self, zero, main):
        self.zero, self.never = zero, zero > 0
        self.tasks = [(k - 1e-6, 0, task) for k, task in enumerate(main)]
        self.latest = {}

    def spread(self, tasks, k0, k1=None):
        step = 0 if k1 is None else (k1 - k0) / len(tasks)
        self.tasks += [(k0 + n * step, step, task) for n, task in enumerate(tasks)]

    def run(self):
        for self.at, self.span, task in sorted(self.tasks, key=lambda x: x[0]):
            task(self)

    def result(self, t):
        self.latest.update({rows: (t, {}) for rows in range(8, t.shape[0] + 1, 8)})
        return t

    def paced(self, t, part=0.0):
        if t.shape[0] not in self.latest:
            return t
        now, cuts = self.latest[t.shape[0]]
        r = min(int((self.at % 1 + part * self.span) * now.shape[0]) // 8 * 8,
                now.shape[0] - t.shape[0])
        if (r, t.dtype) not in cuts:
            now = now[r:r + t.shape[0]]
            cuts[r, t.dtype] = now if t.dtype == F32 else pltpu.bitcast(now, t.dtype)
        return lax.select(self.never, cuts[r, t.dtype], t)


def _task(fn, *args):
    return lambda plan: fn(plan, *args)


def _kernel(ax_hbm, awqkv_hbm, awo_hbm, bx_hbm, mem_hbm, wq_hbm, wk_hbm, wv_hbm, wo_hbm,
            out_hbm,
            ax, awqkv, awo, tmp, aw, xw, qkv_s, oa_s, outa,
            bx, mem, raw, wt, l_tok, l_mem, ahead, y_s, qk_s, v_s, p_s, o_s, o_old, z_part, z_s,
            outb, sem_a, sem_x, sem_w, sem_b, sem_o):
    cp = pltpu.make_async_copy

    def rows_copy(src, dst, r0, r1, sem):
        return cp(src.at[pl.ds(r0, r1 - r0), :], dst.at[pl.ds(r0, r1 - r0), :], sem)

    c_wqkv = [cp(awqkv_hbm.at[:, pl.ds(j * D, D)], awqkv.at[j], sem_a.at[j]) for j in range(3)]
    c_awo = cp(awo_hbm, awo, sem_a.at[3])
    cuts = (0, 2, 3, 7, 11, NB)
    c_ax = [rows_copy(ax_hbm, ax, cuts[c] * TB, cuts[c + 1] * TB, sem_x.at[c]) for c in range(5)]
    c_mem = rows_copy(mem_hbm, mem, 0, M, sem_b.at[0])
    c_bx0 = rows_copy(bx_hbm, bx, 0, (4 + UN) * SEG, sem_b.at[1])
    c_bx1 = rows_copy(bx_hbm, bx, (4 + UN) * SEG, S, sem_b.at[2])
    c_outa = cp(outa, out_hbm.at[:, pl.ds(0, D)], sem_o.at[0])

    def chunk(j, g):
        return 3 * g + j if j < 3 else 3 * NG + g

    def c_w(c):
        j, g = (c % 3, c // 3) if c < 3 * NG else (3, c - 3 * NG)
        n = GROUPS[g].n * 128
        return cp((wq_hbm, wk_hbm, wv_hbm, wo_hbm)[j].at[pl.ds(g * GW * 128, n), :],
                  raw.at[c % RING, pl.ds(0, n), :], sem_w.at[c % 4])

    def c_outb(r0, n):
        return cp(outb.at[pl.ds(r0, n), :], out_hbm.at[pl.ds(r0, n), pl.ds(D, D)], sem_o.at[1])

    def start(copies, priority=1):
        for c in copies:
            c.start(priority=priority)

    def wait(copies):
        for c in copies:
            c.wait()

    def a_weights(j):
        def fill(plan, t):
            tmp[j % 2, t] = (awo[:, t * 128:(t + 1) * 128].astype(F32) if j == 3 else
                             awqkv[j, t * 128:(t + 1) * 128, :].astype(F32).T)

        def move(plan, t, d):
            aw[_ds(j * AD + d, AH // 2), t * 128:(t + 1) * 128] = _words(
                plan.paced(tmp[j % 2, t, pl.ds(d, AH, stride=AD), :]))

        return [task for t in range(LT)
                for task in [_task(fill, t)] + [_task(move, t, d) for d in range(AD)]]

    def a_input(i, b):
        xw[b] = _words(ax[_ds(i, TB), :])

    def a_proj(b, js=range(3), first_block=False):
        def tile(plan, c):
            x = pltpu.bitcast(xw[plan.zero + b], BF16)
            w = pltpu.bitcast(aw[c * 64:(c + 1) * 64, :], BF16)
            r = plan.result(lax.dot_general(x, w, NT, preferred_element_type=F32))
            qkv_s[b, c, HALO:HALO + TB, :] = r
            if c >= LT:
                qkv_s[b, c, 0:HALO, :] = (jnp.broadcast_to(r[0:1, :], (HALO, 128)) if first_block
                                          else qkv_s[1 - b, c, TB:TB + HALO, :])
        return [_task(tile, j * LT + t) for j in js for t in range(LT)]

    def a_attention(b, first_block=False, to=None):
        state = {}

        def window(j, r0, w):
            lo = HALO + r0 - ADIL * w
            return qkv_s[b, j * LT:(j + 1) * LT, lo:lo + 8, :]

        def logits(plan, r0):
            q = jnp.stack([plan.paced(qkv_s[b, t, HALO + r0:HALO + r0 + 8, :], t / LT)
                           for t in range(LT)])
            a = _rows(*[jnp.sum(q * window(1, r0, w), axis=0) for w in range(AW)])
            state[r0] = a + pltpu.roll(a, 2 * AH, 1)

        def fold(plan, r0):
            state[r0] = state[r0] + pltpu.roll(state[r0], AH, 1)

        def weigh(plan, r0):
            a = state[r0].reshape(AW, 8, 128)
            if first_block and r0 < HALO:
                w, pos = [lax.broadcasted_iota(jnp.int32, a.shape, axis) for axis in range(2)]
                a = jnp.where(pos + r0 >= ADIL * w, a, MASKED * AD ** 0.5)
            state[r0] = jnp.exp2((a - jnp.max(a, axis=0)) * (AD ** -0.5 * LOG2E))

        def mix(plan, r0):
            e = state.pop(r0)
            e = [plan.paced(e[w], w / AW) for w in range(AW)]
            o = functools.reduce(jnp.add, (e[w] * window(2, r0, w) for w in range(AW)))
            oa_s[to or b][0, :, r0:r0 + 8, :] = o * _inverse(functools.reduce(jnp.add, e))

        n = TB // 8
        return [_task(f, (k - lag) * 8) for k in range(n + 2)
                for lag, f in ((2, weigh), (0, logits), (1, fold), (2, mix)) if 0 <= k - lag < n]

    def a_out(i, b, depth=LT):
        sums = _Sums()

        def tile(plan, t, k0):
            o = lax.concatenate([oa_s[b][plan.zero, k] for k in range(k0, k0 + depth)], 1)
            n = 48 if depth > 1 and isinstance(i, int) else TB
            sums.add(t, _rows(*[_dot(o[r:r + n], pltpu.bitcast(aw[pl.ds(
                pl.multiple_of((plan.zero >> r // n + 3 * b) * 32 + 3 * D // 2 + k0 * 64, 32), depth * 64),
                t * 128:(t + 1) * 128], BF16)) for r in range(0, TB, n)]))
            if k0 + depth == LT:
                outa[_ds(i, TB), t * 128:(t + 1) * 128] = plan.result(sums.take(t)).astype(BF16)
        return [_task(tile, t, k0) for t in range(LT) for k0 in range(0, LT, depth)]

    def tiles_of(c, odd=None, zero=0):
        if isinstance(c, int) and c >= FULL:
            return wt[2 + c - FULL].at[zero]
        return wt[c % 2 if odd is None else odd].at[c // 2 + zero]

    def w_transpose(c, grp, odd=None):
        src, dst = raw.at[c % RING], tiles_of(c, odd)

        def two(plan, i, f):
            t = _words(src[f * 128:(f + 2) * 128, i * 128:(i + 1) * 128].T)
            for k in range(2):
                dst[grp.slot[i, f + k]] = t[:, k * 128:(k + 1) * 128]
        return [_task(two, i, f) for f in range(0, grp.n, 2) for i in range(LT)]

    def w_combine(c, grp, odd=None, transposed=True):
        w, own, other = tiles_of(c, odd, nil), {}, {}

        def edge(plan, r, a, b):
            def tile(i, f, part=0.0):
                if transposed:
                    t = plan.paced(w[grp.slot[i, f], _ds(r, 8)], part)
                else:
                    t = _words(raw[c % RING, _ds(8 * f + r, 16), i * 128:(i + 1) * 128])
                    t = plan.paced(t, part)
                    if i != grp.label[f]:
                        w[grp.slot[i, f], _ds(r, 8)] = t
                return pltpu.bitcast(t, BF16).astype(F32)

            for f in (a, b):
                if f not in own:
                    own[f] = other[f] = tile(grp.label[f], f)
            ta, tb = tile(grp.label[b], a), tile(grp.label[a], b, 0.5)
            w[grp.slot["both", a, b], _ds(r, 8)] = _words(ta + tb)
            own[a], other[a] = own[a] - ta, other[a] + tb
            own[b], other[b] = own[b] - tb, other[b] + ta
            for f, mate in ((a, b), (b, a)):
                if mate == grp.mates[f][-1]:
                    w[grp.slot[grp.label[f], f], _ds(r, 8)] = _words(own.pop(f))
                    w[grp.slot["other", f], _ds(r, 8)] = _words(other.pop(f))
                    for i in grp.plain[f] * (not transposed):
                        tile(i, f)

        return [_task(edge, r, a, b) for r in range(8) for a in grp.side[0] for b in grp.mates[a]]

    places = {}, {}

    def place(memory, *key):
        return places[memory].setdefault(key, len(places[memory]))

    def binade(tiles):
        top = jnp.max(functools.reduce(jnp.maximum, map(jnp.abs, tiles)), axis=1, keepdims=True)
        top = jnp.clip(jnp.broadcast_to(top, (8, 128)), 2.0 ** -60, 2.0 ** 60)
        return pltpu.bitcast(top, jnp.int32) & 0x7F800000

    def memory_operands(ph, known, i, t):
        known[i] = l_mem[ph][0, place(1, "plain", i)] = t
        for k, u in known.items():
            if k != i:
                l_mem[ph][0, place(1, "cross", min(i, k), max(i, k))] = t + u

    def memory_pair(plan, ph):
        cur = [l_mem[ph][0, place(1, "plain", i)] for i in range(LT)]
        shift = binade(cur) - pltpu.bitcast(
            l_tok[ph][plan.zero, place(0, "mate", 0), 8:16], jnp.int32)
        down, up = [pltpu.bitcast(x, F32) for x in (0x3F800000 + shift, 0x3F800000 - shift)]
        l_mem[ph][0, place(1, "down")], l_mem[ph][0, place(1, "up")] = down, up
        for k in range(LT):
            mate = l_tok[ph][plan.zero, place(0, "mate", k), 0:8]
            for kind in range(2):
                l_tok[1 - ph][0, place(0, "other", kind, k), 8:16] = mate - cur[k] * up
            mate = mate * down
            for i in range(LT):
                l_mem[ph][0, place(1, "both", i, k)] = cur[i] - mate if i == k else cur[i] + mate

    def token_operands(x, s, ph):
        def tokens(plan, ds, i):
            t = _words(x[_ds(max(s + ds, 0), SEG), i * 128:(i + 1) * 128])
            return pltpu.bitcast(plan.paced(t), BF16).astype(F32)

        def one(plan, i, kind):
            before, cur, after, later = [tokens(plan, ds, i) for ds in range(-1, 3)]
            third = (after[16:24], before[16:24], after[8:16])[kind]
            at = place(0, "other", kind, i)
            l_tok[ph][0, at, 0:8] = cur[0:8] - before[24:32]
            l_tok[ph][0, at, 16:32] = cur[16:32] - _rows(third, after[0:8])
            if kind < 2:
                l_tok[ph][0, place(0, "own", kind, i), 0:SEG] = _rows(later[:16 + 8 * kind],
                                                              cur[16 + 8 * kind:])
                return
            l_tok[ph][0, at, 8:16] = cur[8:16] - before[16:24]
            l_tok[ph][0, place(0, "plain", i), 0:SEG] = cur
            l_tok[ph][0, place(0, "mate", i), 0:8] = after[8:16]
            if s == 0:
                l_tok[ph][0, place(0, "next", i), 0:SEG] = after

        def two(plan, i, k):
            cur, after = tokens(plan, 0, i), tokens(plan, 1, k)
            if i < k:
                l_tok[ph][0, place(0, "cross", i, k), 0:SEG] = cur + tokens(plan, 0, k)
            fourth = cur[24:32] + after[0:8]
            l_tok[ph][0, place(0, "both", i, k), 0:SEG] = _rows(cur[16:24] + after[8:16], fourth,
                                                         cur[16:24] + after[16:24], fourth)

        def magnitude(plan):
            l_tok[ph][0, place(0, "mate", 0), 8:16] = pltpu.bitcast(
                binade([tokens(plan, 1, i)[8:16] for i in range(LT)]), F32)

        return [magnitude] + [task for i in range(LT) for task in
                              [_task(one, i, kind) for kind in range(3)]
                              + [_task(two, i, k) for k in range(LT) if k != i]]

    def segment(s, ph, operands, first=False, last=False):
        zero = nil if isinstance(s, int) else s >> 16
        zeros, uses = [zero >> k for k in range(3)], {}

        def again(*key):
            uses[key] = uses.get(key, 0) + 1
            return zeros[uses[key] % len(zeros)]

        def product(plan, parts, j, g, key):
            w = tiles_of(chunk(j, g))[GROUPS[g].slot[key]]
            return plan.result(_dot(_rows(*parts), pltpu.bitcast(w, BF16)))

        pieces = {}

        def project(j, g):
            grp, f0, kind = GROUPS[g], g * GW, _kind(j, g, ph)
            lab = grp.label
            late = 16 + 8 * (kind == 1)
            lo, end = 0 if first else late, SEG if last and j == 0 else L
            y, gift, kept = _Sums(), _Sums(), []
            left = {a: LT for a in grp.side[ph]}
            owed = {a: 1 + len(grp.mates[a]) for a in grp.side[ph]}

            def tok(r0, r1, *key):
                return [l_tok[ph][again(*key), place(0, *key), r0:r1]]

            def memory(*key):
                at = again(1, *key) if kind < 2 else 0
                return [l_mem[ph][at, place(1, *key)]] * (end == L)

            def keep(f, r0, t, minus=False):
                y_s[chunk(j, g)][0, len(kept), r0:end] = t
                pieces.setdefault((j, f0 + f), []).append((len(kept), r0, minus))
                kept.append(f)

            def add(a, t):
                y.add(a, t)
                left[a] -= 1
                if not left[a]:
                    keep(a, 0, y.take(a))

            def give(a, t):
                if last:
                    return
                gift.add(a, t)
                owed[a] -= 1
                if not owed[a]:
                    t = gift.take(a)
                    for r, mate in zip((16, 24, 32), MATES[kind]):
                        if mate is not None:
                            u = t[r - lo:r - lo + 8]
                            ahead[ph][0, j, f0 + a, 0, mate:mate + 8] = (
                                u if r < SEG else u * memory("up")[0])

            def own(plan, a):
                parts = tok(0, late if first else SEG, "own", kind % 2, lab[a]) * (not last)
                parts += tok(lo, SEG, "plain", lab[a]) if first or last else []
                t = product(plan, parts + memory("plain", lab[a]), j, g, (lab[a], a))
                old = [] if first else [ahead[ph][0, j, f0 + a, 1, 0:late]]
                if not last:
                    ahead[ph][0, j, f0 + a, 1, 0:late] = t[:late]
                    t = t[late:]
                add(a, _rows(*old, t))
                give(a, t)

            def opening(plan, b):
                n = 16 + 8 * (kind == 0)
                ahead[1 - ph][0, j, f0 + b, 1, 0:n] = product(
                    plan, tok(0, n, "next", lab[b]), j, g, (lab[b], b))

            def other(plan, b):
                k = lab[b]
                parts = tok(0, late, "plain", k) if first else []
                parts += tok(late - lo, late if last else SEG, "other", kind, k)
                parts += tok(late, SEG, "plain", k) if last else []
                parts += memory("plain", k) if last or kind == 2 else memory("both", k, k)
                at = 0 if first else zero
                got = [] if first else [ahead[1 - ph][at, j, f0 + b, 0, 0:late]]
                for r, mate in zip((16, 24, 32), MATES[kind] * (not last)):
                    if mate is not None:
                        u = ahead[1 - ph][at, j, f0 + b, 1, mate:mate + 8]
                        got.append(u if r < SEG else plan.paced(u) * memory("down")[0])
                t, got = product(plan, parts, j, g, ("other", b)), _rows(*got)
                r0, r1 = late - lo, late - lo + got.shape[0]
                t = _rows(*[t[:r0] for _ in range(r0 > 0)], t[r0:r1] + got,
                          *[t[r1:] for _ in range(r1 < end)])
                y.add(b, t)

            def both(plan, a, b):
                i, k = lab[a], lab[b]
                parts = tok(0, late, "plain", i) if first else []
                parts += tok(late, SEG, "plain", i) if last else tok(
                    *((0, 16) if kind == 2 else (late, SEG)), "both", i, k)
                parts += memory("plain", i) if last or kind == 2 else memory("both", i, k)
                t = product(plan, parts, j, g, ("both", a, b))
                give(a, t)
                if first:
                    y.add(b, t)
                elif b in y:
                    u = y.take(b)
                    keep(b, 0, _rows(u[:lo], u[lo:] + t))
                else:
                    keep(b, lo, t)

            def cross(plan, a, b):
                key = "cross", *sorted((lab[a], lab[b]))
                t = product(plan, tok(0, SEG, *key) + memory(*key), j, g, (lab[b], a))
                add(a, t)
                y.add(b, t, True)
                keep(b, 0, *y.pop(b))

            def plain(plan, i, f):
                t = product(plan, tok(0, SEG, "plain", i) + memory("plain", i), j, g, (i, f))
                (add if f in left else y.add)(f, t)

            passes = []
            others = list(grp.side[1 - ph])
            for a, b0 in zip(grp.side[ph], others[grp.n == GW:] + others):
                passes += [((), _task(opening, b0), 1, 16 + 8 * (kind == 0))] * first
                passes += [((lab[a],), _task(own, a), 0, end + late * (first - last)),
                           ((lab[b0],), _task(other, b0), 0, end)]
                passes += [((i,), _task(plain, i, f), 0, end)
                           for f in (a, b0) for i in grp.plain[f]]
                passes += [((lab[a],), _task(both, a, b), (2 - kind % 2) * (not first), end - lo)
                           for b in grp.mates[a]]
                passes += [((lab[a], lab[b]), _task(cross, a, b), 0, end) for b in grp.mates[a]]
            return passes

        n = SEG if last else L
        row, col = [lax.broadcasted_iota(jnp.int32, (L, 2 * n), axis) for axis in range(2)]
        head0 = col < n
        query = jnp.where(head0, col, col - n) + (L - n)
        visible = (query < M) | (row >= SEG) | (query >= row + M)
        scores = _Sums()

        def gather(j, f):
            sums, end = _Sums(), L if j else n

            def add_up(plan, part):
                todo = pieces[j, f]
                for k, (at, r0, minus) in enumerate(todo[part::2]):
                    u = y_s[chunk(j, f // GW)][zero, at, r0:end]
                    sums.add(r0, u if k else plan.paced(u), minus)
                if part < 2 - 1:
                    return
                t = sums.take(0)
                for r0 in list(sums):
                    t = _rows(t[:r0], t[r0:] + sums.take(r0))
                if j == 1:
                    qk_s[f][0, 1, 0:L] = pltpu.bitcast(t, U32)
                    return
                if j == 0 and not last:
                    t = _rows(t[SEG:], t[:SEG])
                pad = [jnp.zeros((8, 128), F32)] * (end % 16 // 8)
                if f % 3 == 1:
                    low = lax.broadcasted_iota(jnp.int32, t.shape, 1) < 64
                    t = _words(_rows(jnp.where(low, t, 0.0), jnp.where(low, 0.0, t)))
                else:
                    t = _words(_rows(*[t, *pad][::1 - f % 3]))
                (v_s if j else qk_s)[f][0, 0, 0:t.shape[0]] = t

            return [_task(add_up, part) for part in range(2)]

        def by_head(ref, f, rows, short=False):
            t = ref[f][zero, 0, 0:rows if f % 3 == 1 else pl.cdiv(rows, 16) * 8]
            if f % 3 == 2 or f % 3 == 0 and not short:
                t = _rows(*[t, jnp.zeros((rows - t.shape[0], 128), U32)][::1 - f % 3])
            return pltpu.bitcast(t, BF16)

        def score(plan, f):
            k = pltpu.bitcast(qk_s[f][zero, 1, 0:L], F32)
            scores.add(f // 3, lax.dot_general(k, by_head(qk_s, f, n), NT,
                                               preferred_element_type=F32))
            if f % 3 == 2:
                sc = jnp.where(visible, scores.take(f // 3), MASKED * DH ** 0.5)
                e = jnp.exp2((sc - jnp.max(sc, axis=0, keepdims=True)) * (DH ** -0.5 * LOG2E))
                p = e * _inverse(jnp.sum(e, axis=0, keepdims=True))
                p = _rows(jnp.where(head0, p, 0.0), jnp.where(head0, 0.0, p)).T
                p_s[f // 3][0, 0:3 * n, 0:2 * L] = _rows(p[:n], p[:n] + p[n:], p[n:])

        def mix(plan, f):
            v = by_head(v_s, f, L, True)
            o = _dot(p_s[f // 3][zero, _ds(f % 3, n), 0:v.shape[0]], v)
            if last:
                o = _rows(jnp.zeros((M, 128), F32), o)
            g = f // GW
            o_s[ph][g][0, f % GW] = o
            if not first and f % GW in GROUPS[g].side[1 - ph]:
                k = 16 + 8 * _kind(3, g, ph)
                o_old[1 - ph][0, f, 0:k] = o[:k] + o_s[1 - ph][g][zero, f % GW, L - k:]

        z = _Sums()

        def out_project(groups):
            def run(plan, part, left, what, g, a, b, to):
                k, r0, i = 16 + 8 * _kind(3, g, ph), L - n, to[0][1]

                def cur(f, r0, r1=L):
                    return o_s[ph][g][again(g, f), f, r0:r1]

                def joined(r0):
                    t = cur(b, r0, k)
                    if not first:
                        t = t + o_s[1 - ph][g][again(1, g, a), a, L - k + r0:]
                    return [t, cur(b, k)] if last else [t]

                if what == "own":
                    old = [] if first else [o_old[ph][zero, g * GW + a, 0:L - k]]
                    t = product(plan, joined(r0) + old, 3, g, (i, a))
                elif what == "closing":
                    t = product(plan, [o_old[1 - ph][0, g * GW + b, 0:k]], 3, g, (i, b))
                elif what == "both":
                    t = product(plan, joined(0), 3, g, (what, a, b))
                elif what == "cross":
                    t = product(plan, [cur(a, r0) - cur(b, r0)], 3, g, (GROUPS[g].label[b], a))
                else:
                    t = product(plan, [cur(b, r0)], 3, g, (what if what == "other" else i, b))
                part.add(to, t)
                left.remove(to)
                if to in left:
                    return
                t = part.take(to)
                for back, i, dst, src, rows, minus in to:
                    if first or last:
                        z.add_rows((back, i), dst, t[src:src + rows], minus)
                    elif back == 0:
                        z.add((0, i, 0), t[:M])
                if not first and not last:
                    r0 = M * all(x[0] % 2 == 0 for x in to)
                    z_part[ph][0, PARTS[ph][groups[0], to], r0:t.shape[0]] = t[r0:]

            tasks = [], []
            for (lo, hi, order, i), passes in _out_passes(groups, ph, first, last):
                part, left = _Sums(), [x[-1] for x in passes]
                tasks[order == 1].extend(
                    ((lo, hi) if order == 2 else (i,), _task(run, part, left, *x),
                     (order == 1) * (1 + _kind(3, x[1], ph)), max(t[3] + t[4] for t in x[-1]))
                    for x in passes)
            order = [((k // 4 + 0.5) / len(xs), short, k) for short, xs in enumerate(tasks)
                     for k in range(len(xs))]
            return [tasks[short][k] for _, short, k in sorted(order)]

        main, begin, done = [], {}, {}
        parts = FIRST if first else STREAM
        for part in parts:
            if part[0][0] == 3:
                new = out_project([g for _, g in part])
            else:
                new = [project(*jg) for jg in part]
                new = [x for k in range(0, len(new[0]), GW) for xs in new for x in xs[k:k + GW]]
            if part is parts[0] and not first:
                new.sort(key=lambda x: max(x[0]) == LT - 1)
            if part is parts[-1]:
                new.sort(key=lambda x: min(x[0]) == LT - 1)
            begin.update({jg: len(main) for jg in part})
            main += new
            done.update({jg: len(main) for jg in part})

        lag_s, lag_n, lag_v, lag_o = 36, 68, 34, 26
        ready, extra = {}, []
        for stage, js in ((score, (0, 1)), (mix, (2,))):
            at = -GW
            for f in range(FT):
                due = [begin[3, k // GW] if stage is mix else begin[3, k // 3 * 3 // GW] - lag_n
                       for k in range(f, FT)]
                step = min([GW] + [(x - lag_o - at) / k for k, x in enumerate(due, 1)])
                whole = max(done[j, f // GW] for j in js)
                at = max(at + max(step, 0.01), whole + lag_s if stage is score else
                         max(whole + lag_v, ready[f // 3] + lag_n))
                assert at < begin[3, f // GW] - 1
                if stage is score:
                    ready[f // 3] = at
                extra.append((at, stage, js, f, whole))
        queues = [[x for x in main if x[2] == q] for q in range(3)] + [extra[:FT], extra[FT:]]
        queues.append([((), task) for task in a_out(NB - 1, 2, 1) * first])
        main, extra = [], []
        for q in map(int, ORDER[0 if first else -1 if last else 2 - ph]):
            x = queues[q].pop(0)
            if q < 3:
                main.append(x)
            else:
                extra.append((len(main) - 1 + len(extra) * 1e-4, *x[1:]))
        plan = _Plan(zero, [x[1] for x in main])
        for at, stage, *rest in extra:
            if not rest:
                plan.spread([stage], at)
                continue
            js, f, whole = rest
            k0 = max(at - 38, whole - 1)
            plan.spread([t for j in js for t in gather(j, f)], k0, max(at - 28, k0))
            plan.spread([_task(stage, f)], at)

        if first:
            def arrive(plan, groups):
                wait([c_w(chunk(3, g)) for g in groups])
                start([c_w(chunk(3, g + 3)) for g in groups if g + 3 < NG])

            plan.spread([t for j in (1, 2) for t in w_transpose(FULL + j, GROUPS[-1])], 0)
            ends = 340, 640, 770, 880, begin[3, 4]
            plan.spread([t for j in range(3) for t in w_combine(FULL + j, GROUPS[-1])], 0, ends[0] - 8)
            for groups, k0, k1 in zip(((0, 1), (2,), (3,), (4,)), ends, ends[1:]):
                plan.spread([_task(arrive, groups)], k0)
                plan.spread([t for g in groups
                             for t in w_combine(chunk(3, g), GROUPS[g], None, False)], k0, k1 - 8)
        else:
            def resume(plan):
                for i in range(LT):
                    if not last:
                        z.add((0, i, 0), z_s[1 - ph][zero, 2, i, 0:M])
                        continue
                    for back in range(3):
                        z.add_rows((back, i), M, z_s[1 - ph][zero, (back - 1) % 3, i,
                                                            M:L if back else 24])

            plan.spread(settle(s - 1, 1 - ph), 30, 130)
            plan.spread([resume], begin[3, 0] - 1)
        if not last:
            k0 = 945 if first else 800
            plan.spread(operands, k0, k0 + 100)
            plan.spread([_task(memory_pair, ph)], 0)
            known = {}
            for i in range(LT):
                plan.spread([lambda _, i=i: memory_operands(1 - ph, known, i, z.take((0, i, 0)))],
                            max(k for k, (tiles, *_) in enumerate(main) if i in tiles))
        plan.run()
        for back in (2, 1, 0) * last:
            for i in range(LT):
                outb[_ds(s - back, SEG), i * 128:(i + 1) * 128] = _rows(
                    *[z.take((back, i, r)) for r in range(M, L, 8)]).astype(BF16)
        for (g, ((back, i, r0, _, rows, _), *_)), at in PARTS[ph].items():
            if g is None:
                z_part[ph][0, at, 0:rows] = _rows(
                    *[z.take((back, i, r)) for r in range(r0, r0 + rows, 8)]
                ) if first else jnp.zeros((rows, 128), F32)

    def settle(s, ph):
        found, sums = {}, _Sums()
        for (_, to), at in PARTS[ph].items():
            for back, i, dst, src, rows, minus in to:
                skip = M * (back == dst == 0)
                found.setdefault((i, back), []).append(
                    (at, dst + skip, src + skip, rows - skip, minus))

        def add(plan, some):
            for k, (at, dst, src, rows, minus) in enumerate(some):
                u = z_part[ph][plan.zero, at, src:src + rows]
                sums.add((dst, rows), u if k else plan.paced(u), minus)

        def finish(plan, i, back):
            t = _Sums()
            if back >= 0:
                t.add_rows((), M, z_s[1 - ph][plan.zero, (back - 1) % 3, i, M:L if back else 24])
            for dst, rows in list(sums):
                t.add_rows((), dst, *sums.pop((dst, rows)))
            r0 = min(t)[0]
            t = _rows(*[t.take(r) for r in sorted(t)])
            if back < 2:
                z_s[ph][0, back % 3, i, r0:r0 + t.shape[0]] = t
            else:
                seg = max(s - 2, 0) if isinstance(s, int) else jnp.maximum(s - 2, 0)
                outb[_ds(seg, SEG), i * 128:(i + 1) * 128] = t.astype(BF16)

        return [task for key, xs in sorted(found.items()) for task in
                [_task(add, xs[k:k + 4]) for k in range(0, len(xs), 4)] + [_task(finish, *key)]]

    def clear(k, carry):
        z_part[0][0, _ds(k, 4)] = jnp.zeros((4, L, 128), F32)
        return lax.shift_right_logical(k, 16)

    def with_weights(plan, first, groups):
        for b, grp in enumerate(groups):
            new, before = [k if isinstance(k, int) else jnp.where(k < 0, k + RING, k)
                           for k in (first + b, first + b - 1)]
            p0 = 8.0
            plan.spread(w_combine(before, GROUPS[0], b), p0 * b, p0 * (b + 1))
            plan.spread(w_transpose(new, grp, 1 - b), p0 * b, p0 * (b + 1))

    def a_step(it, carry):
        for k in range(FULL // 2):
            @pl.when(it == k)
            def _():
                wait([c_w(c) for c in (2 * k - 1, 2 * k) if c >= 0]
                     + {1: [c_ax[3]], 3: [c_ax[4]]}.get(k, []))
                start([c_w(2 * k + 2), c_w(2 * k + 3)])
                start({0: [c_ax[3]], 2: [c_ax[4]], 4: [c_mem, c_bx0]}.get(k, []), 0)
        plan = _Plan(nil, a_out(2 * it, 0) + a_out(2 * it + 1, 1) + a_proj(1) + a_proj(0))
        with_weights(plan, 2 * it - 1, [GROUPS[0]] * 2)
        plan.spread(a_attention(0), 15.5, 24.99)
        plan.spread(a_attention(1), 24.99, 38.5)
        plan.run()
        for b in range(2):
            a_input(jnp.minimum(2 * it + 6 - b, NB - 1), b)
        return carry

    def b_step(it, carry):
        @pl.when(it == 1)
        def _():
            c_bx1.wait()
        x = bx.at[pl.ds(pl.multiple_of(it * UN * SEG, UN * SEG), (4 + UN) * SEG)]
        for u in range(1, UN + 1):
            segment(it * UN + u, u % 2, token_operands(x, u + 1, 1 - u % 2))

        @pl.when(it > 1)
        def _():
            c_outb(pl.multiple_of((it - 2) * UN * SEG, UN * SEG), UN * SEG).start()
        return carry

    start([c_wqkv[0], c_ax[0], c_wqkv[1]])
    nil = lax.fori_loop(0, z_part[0].shape[1] // 4, clear, 0)
    for ref in (z_s[1], o_old[1]):
        ref[...] = jnp.zeros(ref.shape, F32)
    bx[S:, :] = jnp.zeros((2 * SEG, D), BF16)
    wait([c_wqkv[0]])
    start([c_wqkv[2]])
    _Plan(nil, a_weights(0)).run()
    wait([c_ax[0]])
    start([c_ax[1]])
    for b in range(2):
        a_input(b, b)
    _Plan(nil, a_proj(0, [0])).run()
    for j, copy in ((1, c_awo), (2, c_ax[2])):
        wait([c_wqkv[j]])
        start([copy])
        plan = _Plan(nil, a_proj(1, [j - 1]) + a_proj(0, [j], True))
        plan.spread(a_weights(j), 0, 2)
        plan.run()
    wait([c_ax[1], c_awo])
    start([c_w(0), c_w(1)])
    a_input(2, 0)
    plan = _Plan(nil, a_proj(1, [2]) + a_proj(0))
    plan.spread(a_attention(0, True), 0, 4.99)
    plan.spread(a_attention(1), 9, 18.5)
    plan.spread(a_weights(3), 9, 18.5)
    plan.run()
    wait([c_ax[2]])
    for b in range(2):
        a_input(4 - b, b)
    lax.fori_loop(0, FULL // 2, a_step, 0)
    wait([c_mem, c_bx0, c_w(FULL - 1), c_w(FULL), c_w(FULL + 1)])
    start([c_w(FULL + 2), c_w(FULL + 3), c_w(FULL + 4)])
    plan = _Plan(nil, a_out(NB - 4, 0) + a_proj(1) + a_out(NB - 3, 1) + a_out(NB - 2, 0))
    with_weights(plan, FULL - 1, [GROUPS[0], GROUPS[-1]])
    plan.spread(a_attention(0), 14, 21.0)
    plan.spread(a_attention(1, to=2), 21.0, 29)
    plan.spread(token_operands(bx, 0, 0), 16, 28)
    plan.run()
    wait([c_w(FULL + 2)])
    start([c_w(FULL + 5)])
    known = {}
    for i in range(LT):
        memory_operands(0, known, i, mem[0:M, i * 128:(i + 1) * 128].astype(F32))
    segment(0, 0, token_operands(bx, 1, 1), first=True)
    start([c_bx1, c_outa])
    steps = (NSEG - 2) // UN
    lax.fori_loop(0, steps, b_step, 0)
    c_outb((steps - 2) * UN * SEG, (2 * UN - 2) * SEG).start()
    for s in range(steps * UN + 1, NSEG - 1):
        segment(s, s % 2, token_operands(bx, s + 1, 1 - s % 2))
    segment(NSEG - 1, 1, None, last=True)
    c_outb((steps * UN - 2) * SEG, S - (steps * UN - 2) * SEG).start()
    wait([c_outa, c_outb(0, S)])


def pallas_concat_heads__sliding_local_dilated__memory_aug_recurrent_mem_tr__prompt_kernel(
    A_x, A_wqkv, A_wo, B_x, B_mem0, B_Wq, B_Wk, B_Wv, B_Wo, B_seg_len,
):
    assert B_seg_len == SEG
    assert A_x.shape == B_x.shape == (1, S, D) and B_mem0.shape == (1, M, D)
    assert B_Wq.shape == B_Wk.shape == B_Wv.shape == (D, H, DH) and B_Wo.shape == (H, DH, D)
    dma = pltpu.SemaphoreType.DMA

    def vmem(dtype, *shape):
        assert math.prod(shape) * jnp.dtype(dtype).itemsize % 16384 == 0, shape
        return pltpu.VMEM(shape, dtype)

    call = pl.pallas_call(
        _kernel,
        out_shape=jax.ShapeDtypeStruct((S, 2 * D), BF16),
        in_specs=[pl.BlockSpec(memory_space=pl.ANY)] * 9,
        out_specs=pl.BlockSpec(memory_space=pl.ANY),
        scratch_shapes=[
            vmem(BF16, S, D),
            vmem(BF16, 3, D, D),
            vmem(BF16, D, D),
            vmem(F32, 2, LT, D, 128),
            vmem(U32, 2 * D, D),
            vmem(U32, 2, TB // 2, D),
            vmem(F32, 2, 3 * LT, HALO + TB, 128),
            [vmem(F32, 1, LT, TB, 128)] * 3,
            vmem(BF16, S, D),
            vmem(BF16, S + 2 * SEG, D),
            vmem(BF16, 64, D),
            vmem(BF16, RING, GW * 128, D),
            [vmem(U32, n, SLOTS, 64, 128) for n in [FULL // 2] * 2 + [1] * 8],
            [vmem(F32, 1, 72, 40, 128)] * 2,
            [vmem(F32, 1, 44, M, 128)] * 2,
            [vmem(F32, 1, 3, FT, 2, 24, 128)] * 2,
            [vmem(F32, 1, 48, L, 128)] * (3 * NG),
            [vmem(U32, 1, 2, 48, 128)] * FT,
            [vmem(U32, 1, 1, 64, 128)] * FT,
            [vmem(F32, 1, 128, 128)] * (FT // 3),
            [[vmem(F32, 1, 12, L, 128)] * NG] * 2,
            [vmem(F32, 1, FT, 24, 128)] * 2,
            [vmem(F32, 1, pl.cdiv(len(PARTS[0]), 4) * 4, L, 128)] * 2,
            [vmem(F32, 1, 4, LT, L, 128)] * 2,
            vmem(BF16, S, D),
            dma((4,)), dma((5,)), dma((4,)), dma((3,)), dma((2,)),
        ],
        compiler_params=pltpu.CompilerParams(
            vmem_limit_bytes=126 * 1024 * 1024,
            flags={"XLA_TPU_EVENLY_DISTRIBUTE_CRITICAL_NODES": True}),
        name="sliding_and_memory_attention",
    )

    def by_feature(w):
        return w.transpose(1, 2, 0).reshape(H * DH, D)

    out = call(A_x.reshape(S, D), A_wqkv, A_wo, B_x.reshape(S, D), B_mem0.reshape(M, D),
               by_feature(B_Wq), by_feature(B_Wk), by_feature(B_Wv), B_Wo.reshape(H * DH, D))
    return out.reshape(1, S, 2 * D)
```

```python
import functools
import math

import jax
import jax.numpy as jnp
from jax import lax
from jax.experimental import pallas as pl
from jax.experimental.pallas import tpu as pltpu

F32, BF16, U32 = jnp.float32, jnp.bfloat16, jnp.uint32
NT = (((1,), (1,)), ((), ()))
MASKED = -1000000000.0
LOG2E = math.log2(math.e)

S, D = 2048, 640
LT = D // 128

AH, AD, AW, ADIL = 32, 20, 8, 2
HALO = 16
TB = 128
NB = S // TB

H, DH, M, SEG = 32, 192, 8, 32
L = M + SEG
FT = H * DH // 128
NSEG = S // SEG
GW = 2 * LT
NG = pl.cdiv(FT, GW)
FULL = 3 * (NG - 1)
RING = 8


def _stream(text):
    return [[("qkvo".index(w[0]), int(w[1])) for w in part.split("+")] for part in text.split(",")]


FIRST = _stream("v0,v1,q0,k0,q1,k1,q2,k2,v2,q3,k3,v3,q4,k4,v4,o0+o1+o2,o3,o4")
STREAM = _stream("q0,k0+v0,q1+k1,v1+q2,k2+v2,q3+k3,q4+k4,v3+v4,o0+o1+o2,o3+o4")
ORDER = (
    "10000000000010000001000000000000100000000001000000000001000000010000000000100000000000010000"
    "00010000000000000001000000100000000000000100000100000000000000010000000000100000000100000001"
    "00000000000100000000000100000000000010000001000000000001000000000001000000000103003000000000"
    "03010000000010030000001000000003000010030000000100003000000000103000001000030000031040000400"
    "00000100000000134000043000000000010400000103000430000001040000030000000001034000003014000000"
    "00000300100400000001030000030010404000000100000000001340000300004000000134000000001004000003"
    "00000010040030003104000000000003010040000000010300000100403000400000100430000000000010000004"
    "00001004000000014000000001004000000104000000000104000000000103000040000003000143000000000100"
    "30000000013000000000300001000000001000300000300100000000000301000000014004300000000010000000"
    "40104000000000100000400000010040000003000100301140042012055520135000010100321401002100553515"
    "00002000211013001020355551000000001032114100255501500020101001040200021551541500002010102400"
    "01120555140500001001004024020101250100010004100204120200000222200020200200020020020202200202"
    "0020000212000101010000000101011000010110000101000",
    "20200020200202202002002020220020202000020220200000222020000101101000000202202001011010000002"
    "22200000011110000020202200000111100000020220200001111000000022220000001110100002022020000011"
    "10103000202300122000001100102023002020001110130002022030032000011110000020202230003110100010"
    "00023020202010141001300300222402000101014300100202020240300101301014000202002402300101001140"
    "30000223024002001130011400002022023400010101010300200242020000101011400000222024000010114000"
    "10202020240001001104010000220240001201010140000202200200001110100300020202200001110030102003"
    "02002010320010001120300022200100310000103100220000200110401300002032402000001010341000000220"
    "40230000101041300000220202430001001140103000022230240030010104001002400220300001200114003000"
    "22023400200001101030002032020200013001101000020202320000020102030102030201020002020102300231"
    "00200200030124020102402004124000002010240012400220410400002020102404012402000204001002010224"
    "02401024040000201020012400202410000002200120001000100120001001200010012000000010120000201020"
    "01200000011000200010201000110020201010202100",
    "00222020000220200220200020202020202000202020020000111010000022200200001110100000222002000011"
    "10100002022002000011101000020220020000111010000002202200001110100002022002000011101000002220"
    "02000011101300020020302002130011010030202020200010101013000002322020000001131100020032200000"
    "31201100002102042002300100311041000202023400200100114010303002202024000130101014000002224020"
    "30000311011400020023022400010011040130020020022300011401000100022202400010100411000402020202"
    "00001101400020120240020000114010001002224000201010101000002020202010101010300200322002000110"
    "13003100002202000201011301030002022002000001311000104022002023000013401001000034202002000014"
    "01013000002430202000013401000010002240230000013101140003002240202001010014013000004202030201"
    "01010143000000020232000113010100000230022000010110013000010230011003010200012001031020010010"
    "30102001002140014230001101404002000210140402101002400104000102101404002110104400002010104010"
    "42140002000140020110400210410102000010010102000020120020000210020012000210000001001220000012"
    "00021000001200021001002200001201000202020002",
    "00002202022022202200002022000200220020000000220020002000022200000011101000002220200000111010"
    "00002220200000111012000002220000011010010020220100200101100002000022200001001110000022003220"
    "10010100100002230022000011103010003022002321000001110003022000322000011110000002220023003001"
    "01034110000220202400031001011400020220303210004001041310020220003420000101032411000020220000"
    "03111140040320020200200100041110303202000014220000111004000202202040001001011020420000422000"
    "01100242110000002241000011100004022220000000101101002022200000001100133100022022000003110001"
    "10000203203220000111003100020200322000011110004300002002042300000110100040300220034200100010"
    "04310020000202400300101013004020020322000410111000400032022002004021010304310002220000210100"
    "40210033001200102002001003200000321010020200012130002020030000020012023000000302021103000202"
    "01020400030412002020040001220001440000044212200200014220000000102042010400022400014200004012"
    "02200004101220004001004202200040042002010201000201020000212200000010021000010002001001100020"
    "01000001000020010200000120010200000100010000020101210112020000011022",
)
UN = len(ORDER) - 2
RANK = {jg: k for k, jg in enumerate(jg for part in STREAM for jg in part)}


class _Group:
    def __init__(self, n):
        k = n // 2
        self.n = n
        self.side = (range(k), range(k, n))
        self.label = list(range(k)) + list(range(LT - k, LT))
        self.mates = [[b for b in self.side[c < k] if self.label[b] != self.label[c]]
                      for c in range(n)]
        self.plain = [[i for i in range(LT) if i != self.label[c]
                       and i not in [self.label[b] for b in self.mates[c]]] for c in range(n)]
        keys = [(i, c) for c in range(n) for i in range(LT)]
        keys += [("other", c) for c in range(n)]
        keys += [("both", a, b) for a in self.side[0] for b in self.mates[a]]
        self.slot = {key: i for i, key in enumerate(keys)}
        for a in self.side[0]:
            for b in self.mates[a]:
                self.slot["both", b, a] = self.slot["both", a, b]


GROUPS = [_Group(min(GW, FT - g * GW)) for g in range(NG)]
SLOTS = max(GROUPS[0].slot.values()) + 1


def _kind(j, g, ph):
    return 2 if RANK[j, g] < 1 else (RANK[j, g] + ph + (j == 3)) % 2


MATES = ((16, 0, 8), (None, 0, 8), (8, 0, None))


def _out_passes(groups, ph, last=False):
    passes = {}
    r0 = M * last
    for g in groups:
        grp = GROUPS[g]
        lab = grp.label
        n = 16 + 8 * _kind(3, g, ph)
        now = L if last else n

        def add(i, k, order, what, a, b, *to):
            to = tuple(x for x in to if not (last and x[0] < 0))
            passes.setdefault((min(i, k), max(i, k), order, i), []).append((what, g, a, b, to))

        for a, b in zip(grp.side[ph], grp.side[1 - ph]):
            i, k = lab[a], lab[b]
            add(i, i, 0, "own", a, a, (0, i, r0, 0, now - r0, False),
                (2, i, n, now - r0, L - n, False))
            add(k, k, 0, "other", b, b, (0, k, r0, 0, L - r0, False),
                (1, k, L - n + r0, 0, n - r0, True), (-1, k, 0, n, L - n, True))
            if last:
                add(k, k, 0, "closing", b, b, (1, k, L - n, 0, n, False))
            for f in (a, b):
                for k in grp.plain[f]:
                    add(k, k, 0, "plain", f, f, (0, k, r0, 0, L - r0, False))
            for b in grp.mates[a]:
                k = lab[b]
                add(i, k, 1, "both", a, b, (0, i, r0, r0, now - r0, False),
                    (1, k, L - n, 0, n, False))
                add(min(i, k), max(i, k), 2, "cross", a, b,
                    *[(0, t, r0, 0, L - r0, False) for t in sorted((i, k))])
    return sorted(passes.items())


def _parts(ph):
    keys = [(part[0][1], x[-1]) for part in STREAM if part[0][0] == 3
            for _, passes in _out_passes([g for _, g in part], ph) for x in passes]
    return {key: n for n, key in enumerate(dict.fromkeys(keys))}


PARTS = _parts(0), _parts(1)


def _ds(i, n):
    return pl.ds(i * n if isinstance(i, int) else pl.multiple_of(i * n, n), n)


def _dot(a, b):
    return jnp.dot(a, b, preferred_element_type=F32)


def _inverse(x):
    r = pl.reciprocal(x, approx=True)
    return r * (2.0 - x * r)


def _rows(*parts):
    return parts[0] if len(parts) == 1 else lax.concatenate(parts, 0)


def _words(t):
    return pltpu.bitcast(t.astype(BF16), U32)


class _Sums(dict):
    def add(self, key, t, minus=False):
        if key in self:
            u, neg = self[key]
            t, minus = (t + u, neg) if neg == minus else (t - u if neg else u - t, False)
        self[key] = t, minus

    def add_rows(self, key, r0, t, minus=False):
        for r in range(0, t.shape[0], 8):
            self.add((*key, r0 + r), t[r:r + 8], minus)

    def take(self, key):
        t, neg = self.pop(key)
        return -t if neg else t


class _Plan:
    def __init__(self, zero, main):
        self.zero, self.never = zero, zero > 0
        self.tasks = [(k - 1e-6, 0, task) for k, task in enumerate(main)]
        self.latest = {}

    def spread(self, tasks, k0, k1=None):
        step = 0 if k1 is None else (k1 - k0) / len(tasks)
        self.tasks += [(k0 + n * step, step, task) for n, task in enumerate(tasks)]

    def run(self):
        for self.at, self.span, task in sorted(self.tasks, key=lambda x: x[0]):
            task(self)

    def result(self, t):
        self.latest.update({rows: (t, {}) for rows in range(8, t.shape[0] + 1, 8)})
        return t

    def paced(self, t, part=0.0):
        if t.shape[0] not in self.latest:
            return t
        now, cuts = self.latest[t.shape[0]]
        r = min(int((self.at % 1 + part * self.span) * now.shape[0]) // 8 * 8,
                now.shape[0] - t.shape[0])
        if (r, t.dtype) not in cuts:
            now = now[r:r + t.shape[0]]
            cuts[r, t.dtype] = now if t.dtype == F32 else pltpu.bitcast(now, t.dtype)
        return lax.select(self.never, cuts[r, t.dtype], t)


def _task(fn, *args):
    return lambda plan: fn(plan, *args)


def _kernel(ax_hbm, awqkv_hbm, awo_hbm, bx_hbm, mem_hbm, wq_hbm, wk_hbm, wv_hbm, wo_hbm,
            out_hbm,
            ax, awqkv, awo, tmp, aw, xw, qkv_s, oa_s, outa,
            bx, mem, raw, wt, l_tok, l_mem, ahead, y_s, qk_s, v_s, p_s, o_s, o_old, z_part, z_s,
            outb, sem_a, sem_x, sem_w, sem_b, sem_o):
    cp = pltpu.make_async_copy

    def rows_copy(src, dst, r0, r1, sem):
        return cp(src.at[pl.ds(r0, r1 - r0), :], dst.at[pl.ds(r0, r1 - r0), :], sem)

    c_wqkv = [cp(awqkv_hbm.at[:, pl.ds(j * D, D)], awqkv.at[j], sem_a.at[j]) for j in range(3)]
    c_awo = cp(awo_hbm, awo, sem_a.at[3])
    cuts = (0, 2, 3, 7, 11, NB)
    c_ax = [rows_copy(ax_hbm, ax, cuts[c] * TB, cuts[c + 1] * TB, sem_x.at[c]) for c in range(5)]
    c_mem = rows_copy(mem_hbm, mem, 0, M, sem_b.at[0])
    c_bx0 = rows_copy(bx_hbm, bx, 0, (4 + UN) * SEG, sem_b.at[1])
    c_bx1 = rows_copy(bx_hbm, bx, (4 + UN) * SEG, S, sem_b.at[2])
    c_outa = cp(outa, out_hbm.at[:, pl.ds(0, D)], sem_o.at[0])

    def chunk(j, g):
        return 3 * g + j if j < 3 else 3 * NG + g

    def c_w(c):
        j, g = (c % 3, c // 3) if c < 3 * NG else (3, c - 3 * NG)
        n = GROUPS[g].n * 128
        return cp((wq_hbm, wk_hbm, wv_hbm, wo_hbm)[j].at[pl.ds(g * GW * 128, n), :],
                  raw.at[c % RING, pl.ds(0, n), :], sem_w.at[c % 4])

    def c_outb(r0, n):
        return cp(outb.at[pl.ds(r0, n), :], out_hbm.at[pl.ds(r0, n), pl.ds(D, D)], sem_o.at[1])

    def start(copies, priority=1):
        for c in copies:
            c.start(priority=priority)

    def wait(copies):
        for c in copies:
            c.wait()

    def a_weights(j):
        def fill(plan, t):
            tmp[j % 2, t] = (awo[:, t * 128:(t + 1) * 128].astype(F32) if j == 3 else
                             awqkv[j, t * 128:(t + 1) * 128, :].astype(F32).T)

        def move(plan, t, d):
            aw[_ds(j * AD + d, AH // 2), t * 128:(t + 1) * 128] = _words(
                plan.paced(tmp[j % 2, t, pl.ds(d, AH, stride=AD), :]))

        return [task for t in range(LT)
                for task in [_task(fill, t)] + [_task(move, t, d) for d in range(AD)]]

    def a_input(i, b):
        xw[b] = _words(ax[_ds(i, TB), :])

    def a_proj(b, js=range(3), first_block=False):
        def tile(plan, c):
            x = pltpu.bitcast(xw[plan.zero + b], BF16)
            w = pltpu.bitcast(aw[c * 64:(c + 1) * 64, :], BF16)
            r = plan.result(lax.dot_general(x, w, NT, preferred_element_type=F32))
            qkv_s[b, c, HALO:HALO + TB, :] = r
            if c >= LT:
                qkv_s[b, c, 0:HALO, :] = (jnp.broadcast_to(r[0:1, :], (HALO, 128)) if first_block
                                          else qkv_s[1 - b, c, TB:TB + HALO, :])
        return [_task(tile, j * LT + t) for j in js for t in range(LT)]

    def a_attention(b, first_block=False, to=None):
        state = {}

        def window(j, r0, w):
            lo = HALO + r0 - ADIL * w
            return qkv_s[b, j * LT:(j + 1) * LT, lo:lo + 8, :]

        def logits(plan, r0):
            q = jnp.stack([plan.paced(qkv_s[b, t, HALO + r0:HALO + r0 + 8, :], t / LT)
                           for t in range(LT)])
            a = _rows(*[jnp.sum(q * window(1, r0, w), axis=0) for w in range(AW)])
            state[r0] = a + pltpu.roll(a, 2 * AH, 1)

        def fold(plan, r0):
            state[r0] = state[r0] + pltpu.roll(state[r0], AH, 1)

        def weigh(plan, r0):
            a = state[r0].reshape(AW, 8, 128)
            if first_block and r0 < HALO:
                w, pos = [lax.broadcasted_iota(jnp.int32, a.shape, axis) for axis in range(2)]
                a = jnp.where(pos + r0 >= ADIL * w, a, MASKED * AD ** 0.5)
            state[r0] = jnp.exp2((a - jnp.max(a, axis=0)) * (AD ** -0.5 * LOG2E))

        def mix(plan, r0):
            e = state.pop(r0)
            e = [plan.paced(e[w], w / AW) for w in range(AW)]
            o = functools.reduce(jnp.add, (e[w] * window(2, r0, w) for w in range(AW)))
            oa_s[to or b][0, :, r0:r0 + 8, :] = o * _inverse(functools.reduce(jnp.add, e))

        n = TB // 8
        return [_task(f, (k - lag) * 8) for k in range(n + 2)
                for lag, f in ((2, weigh), (0, logits), (1, fold), (2, mix)) if 0 <= k - lag < n]

    def a_out(i, b, depth=LT):
        sums = _Sums()

        def tile(plan, t, k0):
            o = lax.concatenate([oa_s[b][plan.zero, k] for k in range(k0, k0 + depth)], 1)
            n = 48 if depth > 1 and isinstance(i, int) else TB
            sums.add(t, _rows(*[_dot(o[r:r + n], pltpu.bitcast(aw[pl.ds(
                pl.multiple_of((plan.zero >> r // n + 3 * b) * 32 + 3 * D // 2 + k0 * 64, 32), depth * 64),
                t * 128:(t + 1) * 128], BF16)) for r in range(0, TB, n)]))
            if k0 + depth == LT:
                outa[_ds(i, TB), t * 128:(t + 1) * 128] = plan.result(sums.take(t)).astype(BF16)
        return [_task(tile, t, k0) for t in range(LT) for k0 in range(0, LT, depth)]

    def tiles_of(c, odd=None, zero=0):
        if isinstance(c, int) and c >= FULL:
            return wt[2 + c - FULL].at[zero]
        return wt[c % 2 if odd is None else odd].at[c // 2 + zero]

    def w_transpose(c, grp, odd=None):
        src, dst = raw.at[c % RING], tiles_of(c, odd)

        def two(plan, i, f):
            t = _words(src[f * 128:(f + 2) * 128, i * 128:(i + 1) * 128].T)
            for k in range(2):
                dst[grp.slot[i, f + k]] = t[:, k * 128:(k + 1) * 128]
        return [_task(two, i, f) for f in range(0, grp.n, 2) for i in range(LT)]

    def w_combine(c, grp, odd=None, transposed=True):
        w, own, other = tiles_of(c, odd, nil), {}, {}

        def edge(plan, r, a, b):
            def tile(i, f, part=0.0):
                if transposed:
                    t = plan.paced(w[grp.slot[i, f], _ds(r, 8)], part)
                else:
                    t = _words(raw[c % RING, _ds(8 * f + r, 16), i * 128:(i + 1) * 128])
                    t = plan.paced(t, part)
                    if i != grp.label[f]:
                        w[grp.slot[i, f], _ds(r, 8)] = t
                return pltpu.bitcast(t, BF16).astype(F32)

            for f in (a, b):
                if f not in own:
                    own[f] = other[f] = tile(grp.label[f], f)
            ta, tb = tile(grp.label[b], a), tile(grp.label[a], b, 0.5)
            w[grp.slot["both", a, b], _ds(r, 8)] = _words(ta + tb)
            own[a], other[a] = own[a] - ta, other[a] + tb
            own[b], other[b] = own[b] - tb, other[b] + ta
            for f, mate in ((a, b), (b, a)):
                if mate == grp.mates[f][-1]:
                    w[grp.slot[grp.label[f], f], _ds(r, 8)] = _words(own.pop(f))
                    w[grp.slot["other", f], _ds(r, 8)] = _words(other.pop(f))
                    for i in grp.plain[f] * (not transposed):
                        tile(i, f)

        return [_task(edge, r, a, b) for r in range(8) for a in grp.side[0] for b in grp.mates[a]]

    places = {}, {}

    def place(memory, *key):
        return places[memory].setdefault(key, len(places[memory]))

    def binade(tiles):
        top = jnp.max(functools.reduce(jnp.maximum, map(jnp.abs, tiles)), axis=1, keepdims=True)
        top = jnp.clip(jnp.broadcast_to(top, (8, 128)), 2.0 ** -60, 2.0 ** 60)
        return pltpu.bitcast(top, jnp.int32) & 0x7F800000

    def memory_operands(ph, known, i, t):
        known[i] = l_mem[ph][0, place(1, "plain", i)] = t
        for k, u in known.items():
            if k != i:
                l_mem[ph][0, place(1, "cross", min(i, k), max(i, k))] = t + u

    def memory_pair(plan, ph):
        cur = [l_mem[ph][0, place(1, "plain", i)] for i in range(LT)]
        shift = binade(cur) - pltpu.bitcast(
            l_tok[ph][plan.zero, place(0, "mate", 0), 8:16], jnp.int32)
        down, up = [pltpu.bitcast(x, F32) for x in (0x3F800000 + shift, 0x3F800000 - shift)]
        l_mem[ph][0, place(1, "down")], l_mem[ph][0, place(1, "up")] = down, up
        for k in range(LT):
            mate = l_tok[ph][plan.zero, place(0, "mate", k), 0:8]
            for kind in range(2):
                l_tok[1 - ph][0, place(0, "other", kind, k), 8:16] = mate - cur[k] * up
            mate = mate * down
            for i in range(LT):
                l_mem[ph][0, place(1, "both", i, k)] = cur[i] - mate if i == k else cur[i] + mate

    def token_operands(x, s, ph):
        def tokens(plan, ds, i):
            t = _words(x[_ds(max(s + ds, 0), SEG), i * 128:(i + 1) * 128])
            return pltpu.bitcast(plan.paced(t), BF16).astype(F32)

        def one(plan, i, kind):
            before, cur, after, later = [tokens(plan, ds, i) for ds in range(-1, 3)]
            third = (after[16:24], before[16:24], after[8:16])[kind]
            at = place(0, "other", kind, i)
            l_tok[ph][0, at, 0:8] = cur[0:8] - before[24:32]
            l_tok[ph][0, at, 16:32] = cur[16:32] - _rows(third, after[0:8])
            if kind < 2:
                l_tok[ph][0, place(0, "own", kind, i), 0:SEG] = _rows(later[:16 + 8 * kind],
                                                              cur[16 + 8 * kind:])
                return
            l_tok[ph][0, at, 8:16] = cur[8:16] - before[16:24]
            l_tok[ph][0, place(0, "plain", i), 0:SEG] = cur
            l_tok[ph][0, place(0, "mate", i), 0:8] = after[8:16]
            if s == 0:
                l_tok[ph][0, place(0, "next", i), 0:SEG] = after

        def two(plan, i, k):
            cur, after = tokens(plan, 0, i), tokens(plan, 1, k)
            if i < k:
                l_tok[ph][0, place(0, "cross", i, k), 0:SEG] = cur + tokens(plan, 0, k)
            fourth = cur[24:32] + after[0:8]
            l_tok[ph][0, place(0, "both", i, k), 0:SEG] = _rows(cur[16:24] + after[8:16], fourth,
                                                         cur[16:24] + after[16:24], fourth)

        def magnitude(plan):
            l_tok[ph][0, place(0, "mate", 0), 8:16] = pltpu.bitcast(
                binade([tokens(plan, 1, i)[8:16] for i in range(LT)]), F32)

        return [magnitude] + [task for i in range(LT) for task in
                              [_task(one, i, kind) for kind in range(3)]
                              + [_task(two, i, k) for k in range(LT) if k != i]]

    def segment(s, ph, operands, first=False, last=False):
        zero = nil if isinstance(s, int) else s >> 16
        zeros, uses = [zero >> k for k in range(3)], {}

        def again(*key):
            uses[key] = uses.get(key, 0) + 1
            return zeros[uses[key] % len(zeros)]

        def product(plan, parts, j, g, key):
            w = tiles_of(chunk(j, g))[GROUPS[g].slot[key]]
            return plan.result(_dot(_rows(*parts), pltpu.bitcast(w, BF16)))

        pieces = {}

        def project(j, g):
            grp, f0, kind = GROUPS[g], g * GW, _kind(j, g, ph)
            lab = grp.label
            late = 16 + 8 * (kind == 1)
            lo, end = 0 if first else late, SEG if last and j == 0 else L
            y, gift, kept = _Sums(), _Sums(), []
            left = {a: LT for a in grp.side[ph]}
            owed = {a: 1 + len(grp.mates[a]) for a in grp.side[ph]}

            def tok(r0, r1, *key):
                return [l_tok[ph][again(*key), place(0, *key), r0:r1]]

            def memory(*key):
                at = again(1, *key) if kind < 2 else 0
                return [l_mem[ph][at, place(1, *key)]] * (end == L)

            def keep(f, r0, t, minus=False):
                y_s[chunk(j, g)][0, len(kept), r0:end] = t
                pieces.setdefault((j, f0 + f), []).append((len(kept), r0, minus))
                kept.append(f)

            def add(a, t):
                y.add(a, t)
                left[a] -= 1
                if not left[a]:
                    keep(a, 0, y.take(a))

            def give(a, t):
                if last:
                    return
                gift.add(a, t)
                owed[a] -= 1
                if not owed[a]:
                    t = gift.take(a)
                    for r, mate in zip((16, 24, 32), MATES[kind]):
                        if mate is not None:
                            u = t[r - lo:r - lo + 8]
                            ahead[ph][0, j, f0 + a, 0, mate:mate + 8] = (
                                u if r < SEG else u * memory("up")[0])

            def own(plan, a):
                parts = tok(0, late if first else SEG, "own", kind % 2, lab[a]) * (not last)
                parts += tok(lo, SEG, "plain", lab[a]) if first or last else []
                t = product(plan, parts + memory("plain", lab[a]), j, g, (lab[a], a))
                old = [] if first else [ahead[ph][0, j, f0 + a, 1, 0:late]]
                if not last:
                    ahead[ph][0, j, f0 + a, 1, 0:late] = t[:late]
                    t = t[late:]
                add(a, _rows(*old, t))
                give(a, t)

            def opening(plan, b):
                n = 16 + 8 * (kind == 0)
                ahead[1 - ph][0, j, f0 + b, 1, 0:n] = product(
                    plan, tok(0, n, "next", lab[b]), j, g, (lab[b], b))

            def other(plan, b):
                k = lab[b]
                parts = tok(0, late, "plain", k) if first else []
                parts += tok(late - lo, late if last else SEG, "other", kind, k)
                parts += tok(late, SEG, "plain", k) if last else []
                parts += memory("plain", k) if last or kind == 2 else memory("both", k, k)
                at = 0 if first else zero
                got = [] if first else [ahead[1 - ph][at, j, f0 + b, 0, 0:late]]
                for r, mate in zip((16, 24, 32), MATES[kind] * (not last)):
                    if mate is not None:
                        u = ahead[1 - ph][at, j, f0 + b, 1, mate:mate + 8]
                        got.append(u if r < SEG else plan.paced(u) * memory("down")[0])
                t, got = product(plan, parts, j, g, ("other", b)), _rows(*got)
                r0, r1 = late - lo, late - lo + got.shape[0]
                t = _rows(*[t[:r0] for _ in range(r0 > 0)], t[r0:r1] + got,
                          *[t[r1:] for _ in range(r1 < end)])
                y.add(b, t)

            def both(plan, a, b):
                i, k = lab[a], lab[b]
                parts = tok(0, late, "plain", i) if first else []
                parts += tok(late, SEG, "plain", i) if last else tok(
                    *((0, 16) if kind == 2 else (late, SEG)), "both", i, k)
                parts += memory("plain", i) if last or kind == 2 else memory("both", i, k)
                t = product(plan, parts, j, g, ("both", a, b))
                give(a, t)
                if first:
                    y.add(b, t)
                elif b in y:
                    u = y.take(b)
                    keep(b, 0, _rows(u[:lo], u[lo:] + t))
                else:
                    keep(b, lo, t)

            def cross(plan, a, b):
                key = "cross", *sorted((lab[a], lab[b]))
                t = product(plan, tok(0, SEG, *key) + memory(*key), j, g, (lab[b], a))
                add(a, t)
                y.add(b, t, True)
                keep(b, 0, *y.pop(b))

            def plain(plan, i, f):
                t = product(plan, tok(0, SEG, "plain", i) + memory("plain", i), j, g, (i, f))
                (add if f in left else y.add)(f, t)

            passes = []
            others = list(grp.side[1 - ph])
            for a, b0 in zip(grp.side[ph], others[grp.n == GW:] + others):
                passes += [((), _task(opening, b0), 1, 16 + 8 * (kind == 0))] * first
                passes += [((lab[a],), _task(own, a), 0, end + late * (first - last)),
                           ((lab[b0],), _task(other, b0), 0, end)]
                passes += [((i,), _task(plain, i, f), 0, end)
                           for f in (a, b0) for i in grp.plain[f]]
                passes += [((lab[a],), _task(both, a, b), (2 - kind % 2) * (not first), end - lo)
                           for b in grp.mates[a]]
                passes += [((lab[a], lab[b]), _task(cross, a, b), 0, end) for b in grp.mates[a]]
            return passes

        n = SEG if last else L
        row, col = [lax.broadcasted_iota(jnp.int32, (L, 2 * n), axis) for axis in range(2)]
        head0 = col < n
        query = jnp.where(head0, col, col - n) + (L - n)
        visible = (query < M) | (row >= SEG) | (query >= row + M)
        scores = _Sums()

        def gather(j, f):
            sums, end = _Sums(), L if j else n

            def add_up(plan, part):
                todo = pieces[j, f]
                for k, (at, r0, minus) in enumerate(todo[part::2]):
                    u = y_s[chunk(j, f // GW)][zero, at, r0:end]
                    sums.add(r0, u if k else plan.paced(u), minus)
                if part < 2 - 1:
                    return
                t = sums.take(0)
                for r0 in list(sums):
                    t = _rows(t[:r0], t[r0:] + sums.take(r0))
                if j == 1:
                    qk_s[f][0, 1, 0:L] = pltpu.bitcast(t, U32)
                    return
                if j == 0 and not last:
                    t = _rows(t[SEG:], t[:SEG])
                pad = [jnp.zeros((8, 128), F32)] * (end % 16 // 8)
                if f % 3 == 1:
                    low = lax.broadcasted_iota(jnp.int32, t.shape, 1) < 64
                    t = _words(_rows(jnp.where(low, t, 0.0), jnp.where(low, 0.0, t)))
                else:
                    t = _words(_rows(*[t, *pad][::1 - f % 3]))
                (v_s if j else qk_s)[f][0, 0, 0:t.shape[0]] = t

            return [_task(add_up, part) for part in range(2)]

        def by_head(ref, f, rows, short=False):
            t = ref[f][zero, 0, 0:rows if f % 3 == 1 else pl.cdiv(rows, 16) * 8]
            if f % 3 == 2 or f % 3 == 0 and not short:
                t = _rows(*[t, jnp.zeros((rows - t.shape[0], 128), U32)][::1 - f % 3])
            return pltpu.bitcast(t, BF16)

        def score(plan, f):
            k = pltpu.bitcast(qk_s[f][zero, 1, 0:L], F32)
            scores.add(f // 3, lax.dot_general(k, by_head(qk_s, f, n), NT,
                                               preferred_element_type=F32))
            if f % 3 == 2:
                sc = jnp.where(visible, scores.take(f // 3), MASKED * DH ** 0.5)
                e = jnp.exp2((sc - jnp.max(sc, axis=0, keepdims=True)) * (DH ** -0.5 * LOG2E))
                p = e * _inverse(jnp.sum(e, axis=0, keepdims=True))
                p = _rows(jnp.where(head0, p, 0.0), jnp.where(head0, 0.0, p)).T
                p_s[f // 3][0, 0:3 * n, 0:2 * L] = _rows(p[:n], p[:n] + p[n:], p[n:])

        def mix(plan, f):
            v = by_head(v_s, f, L, True)
            o = _dot(p_s[f // 3][zero, _ds(f % 3, n), 0:v.shape[0]], v)
            if last:
                o = _rows(jnp.zeros((M, 128), F32), o)
            g = f // GW
            o_s[ph][g][0, f % GW] = o
            if not first and f % GW in GROUPS[g].side[1 - ph]:
                k = 16 + 8 * _kind(3, g, ph)
                o_old[1 - ph][0, f, 0:k] = o[:k] + o_s[1 - ph][g][zero, f % GW, L - k:]

        z, written = _Sums(), set()

        def out_project(groups):
            def run(plan, part, left, what, g, a, b, to):
                k, r0, i = 16 + 8 * _kind(3, g, ph), L - n, to[0][1]

                def cur(f, r0, r1=L):
                    return o_s[ph][g][again(g, f), f, r0:r1]

                def joined(r0):
                    t = cur(b, r0, k)
                    if not first:
                        t = t + o_s[1 - ph][g][again(1, g, a), a, L - k + r0:]
                    return [t, cur(b, k)] if last else [t]

                if what == "own":
                    old = [] if first else [o_old[ph][zero, g * GW + a, 0:L - k]]
                    t = product(plan, joined(r0) + old, 3, g, (i, a))
                elif what == "closing":
                    t = product(plan, [o_old[1 - ph][0, g * GW + b, 0:k]], 3, g, (i, b))
                elif what == "both":
                    t = product(plan, joined(0), 3, g, (what, a, b))
                elif what == "cross":
                    t = product(plan, [cur(a, r0) - cur(b, r0)], 3, g, (GROUPS[g].label[b], a))
                else:
                    t = product(plan, [cur(b, r0)], 3, g, (what if what == "other" else i, b))
                part.add(to, t)
                left.remove(to)
                if to in left:
                    return
                t = part.take(to)
                for back, i, dst, src, rows, minus in to:
                    if last:
                        z.add_rows((back, i), dst, t[src:src + rows], minus)
                    elif back == 0:
                        z.add((0, i, 0), t[:M])
                if not last:
                    r0 = M * all(x[0] % 2 == 0 for x in to)
                    at = PARTS[ph][[x[0][1] for x in STREAM if (3, g) in x][0], to]
                    rows = slice(r0, t.shape[0])
                    z_part[ph][0, at, rows] = (t[r0:] + z_part[ph][0, at, rows] if at in written
                                               else t[r0:])
                    written.add(at)

            tasks = [], []
            for (lo, hi, order, i), passes in _out_passes(groups, ph, last):
                part, left = _Sums(), [x[-1] for x in passes]
                tasks[order == 1].extend(
                    ((lo, hi) if order == 2 else (i,), _task(run, part, left, *x),
                     (order == 1) * (1 + _kind(3, x[1], ph)), max(t[3] + t[4] for t in x[-1] if not (first and t[0] > 0)))
                    for x in passes)
            order = [((k // 4 + 0.5) / len(xs), short, k) for short, xs in enumerate(tasks)
                     for k in range(len(xs))]
            return [tasks[short][k] for _, short, k in sorted(order)]

        main, begin, done = [], {}, {}
        parts = FIRST if first else STREAM
        for part in parts:
            if part[0][0] == 3:
                new = out_project([g for _, g in part])
            else:
                new = [project(*jg) for jg in part]
                new = [x for k in range(0, len(new[0]), GW) for xs in new for x in xs[k:k + GW]]
            if part is parts[0] and not first:
                new.sort(key=lambda x: max(x[0]) == LT - 1)
            if part is parts[-1]:
                new.sort(key=lambda x: min(x[0]) == LT - 1)
            begin.update({jg: len(main) for jg in part})
            main += new
            done.update({jg: len(main) for jg in part})

        lag_s, lag_n, lag_v, lag_o = 36, 68, 34, 26
        ready, extra = {}, []
        for stage, js in ((score, (0, 1)), (mix, (2,))):
            at = -GW
            for f in range(FT):
                due = [begin[3, k // GW] if stage is mix else begin[3, k // 3 * 3 // GW] - lag_n
                       for k in range(f, FT)]
                step = min([GW] + [(x - lag_o - at) / k for k, x in enumerate(due, 1)])
                whole = max(done[j, f // GW] for j in js)
                at = max(at + max(step, 0.01), whole + lag_s if stage is score else
                         max(whole + lag_v, ready[f // 3] + lag_n))
                assert at < begin[3, f // GW] - 1
                if stage is score:
                    ready[f // 3] = at
                extra.append((at, stage, js, f, whole))
        queues = [[x for x in main if x[2] == q] for q in range(3)] + [extra[:FT], extra[FT:]]
        queues.append([((), task) for task in a_out(NB - 1, 2, 1) * first])
        main, extra = [], []
        for q in map(int, ORDER[0 if first else -1 if last else 2 - ph]):
            x = queues[q].pop(0)
            if q < 3:
                main.append(x)
            else:
                extra.append((len(main) - 1 + len(extra) * 1e-4, *x[1:]))
        plan = _Plan(zero, [x[1] for x in main])
        for at, stage, *rest in extra:
            if not rest:
                plan.spread([stage], at)
                continue
            js, f, whole = rest
            k0 = max(at - 38, whole - 1)
            plan.spread([t for j in js for t in gather(j, f)], k0, max(at - 28, k0))
            plan.spread([_task(stage, f)], at)

        if first:
            def arrive(plan, groups):
                wait([c_w(chunk(3, g)) for g in groups])
                start([c_w(chunk(3, g + 3)) for g in groups if g + 3 < NG])

            plan.spread([t for j in (1, 2) for t in w_transpose(FULL + j, GROUPS[-1])], 0)
            ends = 340, 640, 770, 880, begin[3, 4]
            plan.spread([t for j in range(3) for t in w_combine(FULL + j, GROUPS[-1])], 0, ends[0] - 8)
            for groups, k0, k1 in zip(((0, 1), (2,), (3,), (4,)), ends, ends[1:]):
                plan.spread([_task(arrive, groups)], k0)
                plan.spread([t for g in groups
                             for t in w_combine(chunk(3, g), GROUPS[g], None, False)], k0, k1 - 8)
        else:
            def resume(plan):
                for i in range(LT):
                    if not last:
                        z.add((0, i, 0), z_s[1 - ph][zero, 2, i, 0:M])
                        continue
                    for back in range(3):
                        z.add_rows((back, i), M, z_s[1 - ph][zero, (back - 1) % 3, i,
                                                            M:L if back else 24])

            plan.spread(settle(s - 1, 1 - ph), 30, 130)
            plan.spread([resume], begin[3, 0] - 1)
        if not last:
            k0 = 945 if first else 800
            plan.spread(operands, k0, k0 + 100)
            plan.spread([_task(memory_pair, ph)], 0)
            known = {}
            for i in range(LT):
                plan.spread([lambda _, i=i: memory_operands(1 - ph, known, i, z.take((0, i, 0)))],
                            max(k for k, (tiles, *_) in enumerate(main) if i in tiles))
        plan.run()
        for back in (2, 1, 0) * last:
            for i in range(LT):
                outb[_ds(s - back, SEG), i * 128:(i + 1) * 128] = _rows(
                    *[z.take((back, i, r)) for r in range(M, L, 8)]).astype(BF16)

    def settle(s, ph):
        found, sums = {}, _Sums()
        for (_, to), at in PARTS[ph].items():
            for back, i, dst, src, rows, minus in to:
                skip = M * (back == dst == 0)
                found.setdefault((i, back), []).append(
                    (at, dst + skip, src + skip, rows - skip, minus))

        def add(plan, some):
            for k, (at, dst, src, rows, minus) in enumerate(some):
                u = z_part[ph][plan.zero, at, src:src + rows]
                sums.add((dst, rows), u if k else plan.paced(u), minus)

        def finish(plan, i, back):
            t = _Sums()
            if back >= 0:
                t.add_rows((), M, z_s[1 - ph][plan.zero, (back - 1) % 3, i, M:L if back else 24])
            for dst, rows in list(sums):
                t.add_rows((), dst, *sums.pop((dst, rows)))
            r0 = min(t)[0]
            t = _rows(*[t.take(r) for r in sorted(t)])
            if back < 2:
                z_s[ph][0, back % 3, i, r0:r0 + t.shape[0]] = t
            else:
                seg = max(s - 2, 0) if isinstance(s, int) else jnp.maximum(s - 2, 0)
                outb[_ds(seg, SEG), i * 128:(i + 1) * 128] = t.astype(BF16)

        return [task for key, xs in sorted(found.items()) for task in
                [_task(add, xs[k:k + 4]) for k in range(0, len(xs), 4)] + [_task(finish, *key)]]

    def clear(k, carry):
        z_part[0][0, _ds(k, 4)] = jnp.zeros((4, L, 128), F32)
        return lax.shift_right_logical(k, 16)

    def with_weights(plan, first, groups):
        for b, grp in enumerate(groups):
            new, before = [k if isinstance(k, int) else jnp.where(k < 0, k + RING, k)
                           for k in (first + b, first + b - 1)]
            p0 = 8.0
            plan.spread(w_combine(before, GROUPS[0], b), p0 * b, p0 * (b + 1))
            plan.spread(w_transpose(new, grp, 1 - b), p0 * b, p0 * (b + 1))

    def a_step(it, carry):
        for k in range(FULL // 2):
            @pl.when(it == k)
            def _():
                wait([c_w(c) for c in (2 * k - 1, 2 * k) if c >= 0]
                     + {1: [c_ax[3]], 3: [c_ax[4]]}.get(k, []))
                start([c_w(2 * k + 2), c_w(2 * k + 3)])
                start({0: [c_ax[3]], 2: [c_ax[4]], 4: [c_mem, c_bx0]}.get(k, []), 0)
        plan = _Plan(nil, a_out(2 * it, 0) + a_out(2 * it + 1, 1) + a_proj(1) + a_proj(0))
        with_weights(plan, 2 * it - 1, [GROUPS[0]] * 2)
        plan.spread(a_attention(0), 15.5, 24.99)
        plan.spread(a_attention(1), 24.99, 38.5)
        plan.run()
        for b in range(2):
            a_input(jnp.minimum(2 * it + 6 - b, NB - 1), b)
        return carry

    def b_step(it, carry):
        @pl.when(it == 1)
        def _():
            c_bx1.wait()
        x = bx.at[pl.ds(pl.multiple_of(it * UN * SEG, UN * SEG), (4 + UN) * SEG)]
        for u in range(1, UN + 1):
            segment(it * UN + u, u % 2, token_operands(x, u + 1, 1 - u % 2))

        @pl.when(it > 1)
        def _():
            c_outb(pl.multiple_of((it - 2) * UN * SEG, UN * SEG), UN * SEG).start()
        return carry

    start([c_wqkv[0], c_ax[0], c_wqkv[1]])
    nil = lax.fori_loop(0, z_part[0].shape[1] // 4, clear, 0)
    for ref in (z_s[1], o_old[1]):
        ref[...] = jnp.zeros(ref.shape, F32)
    bx[S:, :] = jnp.zeros((2 * SEG, D), BF16)
    wait([c_wqkv[0]])
    start([c_wqkv[2]])
    _Plan(nil, a_weights(0)).run()
    wait([c_ax[0]])
    start([c_ax[1]])
    for b in range(2):
        a_input(b, b)
    _Plan(nil, a_proj(0, [0])).run()
    for j, copy in ((1, c_awo), (2, c_ax[2])):
        wait([c_wqkv[j]])
        start([copy])
        plan = _Plan(nil, a_proj(1, [j - 1]) + a_proj(0, [j], True))
        plan.spread(a_weights(j), 0, 2)
        plan.run()
    wait([c_ax[1], c_awo])
    start([c_w(0), c_w(1)])
    a_input(2, 0)
    plan = _Plan(nil, a_proj(1, [2]) + a_proj(0))
    plan.spread(a_attention(0, True), 0, 4.99)
    plan.spread(a_attention(1), 9, 18.5)
    plan.spread(a_weights(3), 9, 18.5)
    plan.run()
    wait([c_ax[2]])
    for b in range(2):
        a_input(4 - b, b)
    lax.fori_loop(0, FULL // 2, a_step, 0)
    wait([c_mem, c_bx0, c_w(FULL - 1), c_w(FULL), c_w(FULL + 1)])
    start([c_w(FULL + 2), c_w(FULL + 3), c_w(FULL + 4)])
    plan = _Plan(nil, a_out(NB - 4, 0) + a_proj(1) + a_out(NB - 3, 1) + a_out(NB - 2, 0))
    with_weights(plan, FULL - 1, [GROUPS[0], GROUPS[-1]])
    plan.spread(a_attention(0), 14, 21.0)
    plan.spread(a_attention(1, to=2), 21.0, 29)
    plan.spread(token_operands(bx, 0, 0), 16, 28)
    plan.run()
    wait([c_w(FULL + 2)])
    start([c_w(FULL + 5)])
    known = {}
    for i in range(LT):
        memory_operands(0, known, i, mem[0:M, i * 128:(i + 1) * 128].astype(F32))
    segment(0, 0, token_operands(bx, 1, 1), first=True)
    start([c_bx1, c_outa])
    steps = (NSEG - 2) // UN
    lax.fori_loop(0, steps, b_step, 0)
    c_outb((steps - 2) * UN * SEG, (2 * UN - 2) * SEG).start()
    for s in range(steps * UN + 1, NSEG - 1):
        segment(s, s % 2, token_operands(bx, s + 1, 1 - s % 2))
    segment(NSEG - 1, 1, None, last=True)
    c_outb((steps * UN - 2) * SEG, S - (steps * UN - 2) * SEG).start()
    wait([c_outa, c_outb(0, S)])


def pallas_concat_heads__sliding_local_dilated__memory_aug_recurrent_mem_tr__prompt_kernel(
    A_x, A_wqkv, A_wo, B_x, B_mem0, B_Wq, B_Wk, B_Wv, B_Wo, B_seg_len,
):
    assert B_seg_len == SEG
    assert A_x.shape == B_x.shape == (1, S, D) and B_mem0.shape == (1, M, D)
    assert B_Wq.shape == B_Wk.shape == B_Wv.shape == (D, H, DH) and B_Wo.shape == (H, DH, D)
    dma = pltpu.SemaphoreType.DMA

    def vmem(dtype, *shape):
        assert math.prod(shape) * jnp.dtype(dtype).itemsize % 16384 == 0, shape
        return pltpu.VMEM(shape, dtype)

    call = pl.pallas_call(
        _kernel,
        out_shape=jax.ShapeDtypeStruct((S, 2 * D), BF16),
        in_specs=[pl.BlockSpec(memory_space=pl.ANY)] * 9,
        out_specs=pl.BlockSpec(memory_space=pl.ANY),
        scratch_shapes=[
            vmem(BF16, S, D),
            vmem(BF16, 3, D, D),
            vmem(BF16, D, D),
            vmem(F32, 2, LT, D, 128),
            vmem(U32, 2 * D, D),
            vmem(U32, 2, TB // 2, D),
            vmem(F32, 2, 3 * LT, HALO + TB, 128),
            [vmem(F32, 1, LT, TB, 128)] * 3,
            vmem(BF16, S, D),
            vmem(BF16, S + 2 * SEG, D),
            vmem(BF16, 64, D),
            vmem(BF16, RING, GW * 128, D),
            [vmem(U32, n, SLOTS, 64, 128) for n in [FULL // 2] * 2 + [1] * 8],
            [vmem(F32, 1, 72, 40, 128)] * 2,
            [vmem(F32, 1, 44, M, 128)] * 2,
            [vmem(F32, 1, 3, FT, 2, 24, 128)] * 2,
            [vmem(F32, 1, 48, L, 128)] * (3 * NG),
            [vmem(U32, 1, 2, 48, 128)] * FT,
            [vmem(U32, 1, 1, 64, 128)] * FT,
            [vmem(F32, 1, 128, 128)] * (FT // 3),
            [[vmem(F32, 1, 12, L, 128)] * NG] * 2,
            [vmem(F32, 1, FT, 24, 128)] * 2,
            [vmem(F32, 1, pl.cdiv(max(map(len, PARTS)), 4) * 4, L, 128)] * 2,
            [vmem(F32, 1, 4, LT, L, 128)] * 2,
            vmem(BF16, S, D),
            dma((4,)), dma((5,)), dma((4,)), dma((3,)), dma((2,)),
        ],
        compiler_params=pltpu.CompilerParams(
            vmem_limit_bytes=126 * 1024 * 1024,
            flags={"XLA_TPU_EVENLY_DISTRIBUTE_CRITICAL_NODES": True}),
        name="sliding_and_memory_attention",
    )

    def by_feature(w):
        return w.transpose(1, 2, 0).reshape(H * DH, D)

    out = call(A_x.reshape(S, D), A_wqkv, A_wo, B_x.reshape(S, D), B_mem0.reshape(M, D),
               by_feature(B_Wq), by_feature(B_Wk), by_feature(B_Wv), B_Wo.reshape(H * DH, D))
    return out.reshape(1, S, 2 * D)
```

```python
import functools
import math

import jax
import jax.numpy as jnp
from jax import lax
from jax.experimental import pallas as pl
from jax.experimental.pallas import tpu as pltpu

F32, BF16, U32 = jnp.float32, jnp.bfloat16, jnp.uint32
NT = (((1,), (1,)), ((), ()))
MASKED = -1000000000.0
LOG2E = math.log2(math.e)

S, D = 2048, 640
LT = D // 128

AH, AD, AW, ADIL = 32, 20, 8, 2
HALO = 16
TB = 128
NB = S // TB

H, DH, M, SEG = 32, 192, 8, 32
L = M + SEG
FT = H * DH // 128
NSEG = S // SEG
GW = 2 * LT
NG = pl.cdiv(FT, GW)
FULL = 3 * (NG - 1)
RING = 8


def _stream(text):
    return [[("qkvo".index(w[0]), int(w[1])) for w in part.split("+")] for part in text.split(",")]


FIRST = _stream("v0,v1,q0,k0,q1,k1,q2,k2,v2,q3,k3,v3,q4,k4,v4,o0+o1+o2,o3,o4")
STREAM = _stream("q0,k0+v0,q1+k1,v1+q2,k2+v2,q3+k3,q4+k4,v3+v4,o0+o1+o2,o3+o4")
ORDER = (
    "10000000000010000001000000000000100000000001000000000001000000010000000000100000000000010000"
    "00010000000000000001000000100000000000000100000100000000000000010000000000100000000100000001"
    "00000000000100000000000100000000000010000001000000000001000000000001000000000103003000000000"
    "03010000000010030000001000000003000010030000000100003000000000103000001000030000031040000400"
    "00000100000000134000043000000000010400000103000430000001040000030000000001034000003014000000"
    "00000300100400000001030000030010404000000100000000001340000300004000000134000000001004000003"
    "00000010040030003104000000000003010040000000010300000100403000400000100430000000000010000004"
    "00001004000000014000000001004000000104000000000104000000000103000040000003000143000000000100"
    "30000000013000000000300001000000001000300000300100000000000301000000014004300000000010000000"
    "40104000000000100000400000010040000003000100301140042012055520135000010100321401002100553515"
    "00002000211013001020355551000000001032114100255501500020101001040200021551541500002010102400"
    "01120555140500001001004024020101250100010004100204120200000222200020200200020020020202200202"
    "0020000212000101010000000101011000010110000101000",
    "20200020200202202002002020220020202000020220200000222020000101101000000202202001011010000002"
    "22200000011110000020202200000111100000020220200001111000000022220000001110100002022020000011"
    "10103000202300122000001100102023002020001110130002022030032000011110000020202230003110100010"
    "00023020202010141001300300222402000101014300100202020240300101301014000202002402300101001140"
    "30000223024002001130011400002022023400010101010300200242020000101011400000222024000010114000"
    "10202020240001001104010000220240001201010140000202200200001110100300020202200001110030102003"
    "02002010320010001120300022200100310000103100220000200110401300002032402000001010341000000220"
    "40230000101041300000220202430001001140103000022230240030010104001002400220300001200114003000"
    "22023400200001101030002032020200013001101000020202320000020102030102030201020002020102300231"
    "00200200030124020102402004124000002010240012400220410400002020102404012402000204001002010224"
    "02401024040000201020012400202410000002200120001000100120001001200010012000000010120000201020"
    "01200000011000200010201000110020201010202100",
    "00222020000220200220200020202020202000202020020000111010000022200200001110100000222002000011"
    "10100002022002000011101000020220020000111010000002202200001110100002022002000011101000002220"
    "02000011101300020020302002130011010030202020200010101013000002322020000001131100020032200000"
    "31201100002102042002300100311041000202023400200100114010303002202024000130101014000002224020"
    "30000311011400020023022400010011040130020020022300011401000100022202400010100411000402020202"
    "00001101400020120240020000114010001002224000201010101000002020202010101010300200322002000110"
    "13003100002202000201011301030002022002000001311000104022002023000013401001000034202002000014"
    "01013000002430202000013401000010002240230000013101140003002240202001010014013000004202030201"
    "01010143000000020232000113010100000230022000010110013000010230011003010200012001031020010010"
    "30102001002140014230001101404002000210140402101002400104000102101404002110104400002010104010"
    "42140002000140020110400210410102000010010102000020120020000210020012000210000001001220000012"
    "00021000001200021001002200001201000202020002",
    "00002202022022202200002022000200220020000000220020002000022200000011101000002220200000111010"
    "00002220200000111012000002220000011010010020220100200101100002000022200001001110000022003220"
    "10010100100002230022000011103010003022002321000001110003022000322000011110000002220023003001"
    "01034110000220202400031001011400020220303210004001041310020220003420000101032411000020220000"
    "03111140040320020200200100041110303202000014220000111004000202202040001001011020420000422000"
    "01100242110000002241000011100004022220000000101101002022200000001100133100022022000003110001"
    "10000203203220000111003100020200322000011110004300002002042300000110100040300220034200100010"
    "04310020000202400300101013004020020322000410111000400032022002004021010304310002220000210100"
    "40210033001200102002001003200000321010020200012130002020030000020012023000000302021103000202"
    "01020400030412002020040001220001440000044212200200014220000000102042010400022400014200004012"
    "02200004101220004001004202200040042002010201000201020000212200000010021000010002001001100020"
    "01000001000020010200000120010200000100010000020101210112020000011022",
)
RANK = {jg: k for k, jg in enumerate(jg for part in STREAM for jg in part)}


class _Group:
    def __init__(self, n):
        k = n // 2
        self.n = n
        self.side = (range(k), range(k, n))
        self.label = list(range(k)) + list(range(LT - k, LT))
        self.mates = [[b for b in self.side[c < k] if self.label[b] != self.label[c]]
                      for c in range(n)]
        self.plain = [[i for i in range(LT) if i != self.label[c]
                       and i not in [self.label[b] for b in self.mates[c]]] for c in range(n)]
        keys = [(i, c) for c in range(n) for i in range(LT)]
        keys += [("other", c) for c in range(n)]
        keys += [("both", a, b) for a in self.side[0] for b in self.mates[a]]
        self.slot = {key: i for i, key in enumerate(keys)}
        for a in self.side[0]:
            for b in self.mates[a]:
                self.slot["both", b, a] = self.slot["both", a, b]


GROUPS = [_Group(min(GW, FT - g * GW)) for g in range(NG)]
SLOTS = max(GROUPS[0].slot.values()) + 1


def _kind(j, g, ph):
    return (RANK[j, g] + ph + (j == 3)) % 2 if RANK[j, g] else 2


MATES = ((16, 0, 8), (None, 0, 8), (8, 0, None))


def _out_passes(groups, ph, last=False):
    passes = {}
    r0 = M * last
    for g in groups:
        grp = GROUPS[g]
        lab = grp.label
        n = 16 + 8 * _kind(3, g, ph)
        now = L if last else n

        def add(i, k, order, what, a, b, *to):
            to = tuple(x for x in to if not (last and x[0] < 0))
            passes.setdefault((min(i, k), max(i, k), order, i), []).append((what, g, a, b, to))

        for a, b in zip(grp.side[ph], grp.side[1 - ph]):
            i, k = lab[a], lab[b]
            add(i, i, 0, "own", a, a, (0, i, r0, 0, now - r0, False),
                (2, i, n, now - r0, L - n, False))
            add(k, k, 0, "other", b, b, (0, k, r0, 0, L - r0, False),
                (1, k, L - n + r0, 0, n - r0, True), (-1, k, 0, n, L - n, True))
            if last:
                add(k, k, 0, "closing", b, b, (1, k, L - n, 0, n, False))
            for f in (a, b):
                for k in grp.plain[f]:
                    add(k, k, 0, "plain", f, f, (0, k, r0, 0, L - r0, False))
            for b in grp.mates[a]:
                k = lab[b]
                add(i, k, 1, "both", a, b, (0, i, r0, r0, now - r0, False),
                    (1, k, L - n, 0, n, False))
                add(min(i, k), max(i, k), 2, "cross", a, b,
                    *[(0, t, r0, 0, L - r0, False) for t in sorted((i, k))])
    return sorted(passes.items())


def _parts(ph):
    keys = [(part[0][1], x[-1]) for part in STREAM if part[0][0] == 3
            for _, passes in _out_passes([g for _, g in part], ph) for x in passes]
    return {key: n for n, key in enumerate(dict.fromkeys(keys))}


PARTS = _parts(0), _parts(1)


def _ds(i, n):
    return pl.ds(i * n if isinstance(i, int) else pl.multiple_of(i * n, n), n)


def _dot(a, b):
    return jnp.dot(a, b, preferred_element_type=F32)


def _inverse(x):
    r = pl.reciprocal(x, approx=True)
    return r * (2.0 - x * r)


def _rows(*parts):
    return parts[0] if len(parts) == 1 else lax.concatenate(parts, 0)


def _words(t):
    return pltpu.bitcast(t.astype(BF16), U32)


class _Sums(dict):
    def add(self, key, t, minus=False):
        if key in self:
            u, neg = self[key]
            t, minus = (t + u, neg) if neg == minus else (t - u if neg else u - t, False)
        self[key] = t, minus

    def add_rows(self, key, r0, t, minus=False):
        for r in range(0, t.shape[0], 8):
            self.add((*key, r0 + r), t[r:r + 8], minus)

    def take(self, key):
        t, neg = self.pop(key)
        return -t if neg else t


class _Plan:
    def __init__(self, zero, main):
        self.zero, self.never = zero, zero > 0
        self.tasks = [(k - 1e-6, 0, task) for k, task in enumerate(main)]
        self.latest = {}

    def spread(self, tasks, k0, k1=None):
        step = 0 if k1 is None else (k1 - k0) / len(tasks)
        self.tasks += [(k0 + n * step, step, task) for n, task in enumerate(tasks)]

    def run(self):
        for self.at, self.span, task in sorted(self.tasks, key=lambda x: x[0]):
            task(self)

    def result(self, t):
        self.latest.update({rows: (t, {}) for rows in range(8, t.shape[0] + 1, 8)})
        return t

    def paced(self, t, part=0.0):
        if t.shape[0] not in self.latest:
            return t
        now, cuts = self.latest[t.shape[0]]
        r = min(int((self.at % 1 + part * self.span) * now.shape[0]) // 8 * 8,
                now.shape[0] - t.shape[0])
        if (r, t.dtype) not in cuts:
            now = now[r:r + t.shape[0]]
            cuts[r, t.dtype] = now if t.dtype == F32 else pltpu.bitcast(now, t.dtype)
        return lax.select(self.never, cuts[r, t.dtype], t)


def _task(fn, *args):
    return lambda plan: fn(plan, *args)


def _kernel(ax_hbm, awqkv_hbm, awo_hbm, bx_hbm, mem_hbm, wq_hbm, wk_hbm, wv_hbm, wo_hbm,
            out_hbm,
            ax, awqkv, awo, tmp, aw, xw, qkv_s, oa_s, outa,
            bx, mem, raw, wt, l_tok, l_mem, ahead, y_s, qk_s, v_s, p_s, o_s, o_old, z_part, z_s,
            outb, sem_a, sem_x, sem_w, sem_b, sem_o):
    cp = pltpu.make_async_copy

    def rows_copy(src, dst, r0, r1, sem):
        return cp(src.at[pl.ds(r0, r1 - r0), :], dst.at[pl.ds(r0, r1 - r0), :], sem)

    c_wqkv = [cp(awqkv_hbm.at[:, pl.ds(j * D, D)], awqkv.at[j], sem_a.at[j]) for j in range(3)]
    c_awo = cp(awo_hbm, awo, sem_a.at[3])
    cuts = (0, 2, 3, 7, 11, NB)
    c_ax = [rows_copy(ax_hbm, ax, cuts[c] * TB, cuts[c + 1] * TB, sem_x.at[c]) for c in range(5)]
    c_mem = rows_copy(mem_hbm, mem, 0, M, sem_b.at[0])
    c_bx0 = rows_copy(bx_hbm, bx, 0, 6 * SEG, sem_b.at[1])
    c_bx1 = rows_copy(bx_hbm, bx, 6 * SEG, S, sem_b.at[2])
    c_outa = cp(outa, out_hbm.at[:, pl.ds(0, D)], sem_o.at[0])

    def chunk(j, g):
        return 3 * g + j if j < 3 else 3 * NG + g

    def c_w(c):
        j, g = (c % 3, c // 3) if c < 3 * NG else (3, c - 3 * NG)
        n = GROUPS[g].n * 128
        return cp((wq_hbm, wk_hbm, wv_hbm, wo_hbm)[j].at[pl.ds(g * GW * 128, n), :],
                  raw.at[c % RING, pl.ds(0, n), :], sem_w.at[c % 4])

    def c_outb(r0, n):
        return cp(outb.at[pl.ds(r0, n), :], out_hbm.at[pl.ds(r0, n), pl.ds(D, D)], sem_o.at[1])

    def start(copies, priority=1):
        for c in copies:
            c.start(priority=priority)

    def wait(copies):
        for c in copies:
            c.wait()

    def a_weights(j):
        def fill(plan, t):
            tmp[j % 2, t] = (awo[:, t * 128:(t + 1) * 128].astype(F32) if j == 3 else
                             awqkv[j, t * 128:(t + 1) * 128, :].astype(F32).T)

        def move(plan, t, d):
            aw[_ds(j * AD + d, AH // 2), t * 128:(t + 1) * 128] = _words(
                plan.paced(tmp[j % 2, t, pl.ds(d, AH, stride=AD), :]))

        return [task for t in range(LT)
                for task in [_task(fill, t)] + [_task(move, t, d) for d in range(AD)]]

    def a_input(i, b):
        xw[b] = _words(ax[_ds(i, TB), :])

    def a_proj(b, js=range(3), first_block=False):
        def tile(plan, c):
            x = pltpu.bitcast(xw[plan.zero + b], BF16)
            w = pltpu.bitcast(aw[c * 64:(c + 1) * 64, :], BF16)
            r = plan.result(lax.dot_general(x, w, NT, preferred_element_type=F32))
            qkv_s[b, c, HALO:HALO + TB, :] = r
            if c >= LT:
                qkv_s[b, c, 0:HALO, :] = (jnp.broadcast_to(r[0:1, :], (HALO, 128)) if first_block
                                          else qkv_s[1 - b, c, TB:TB + HALO, :])
        return [_task(tile, j * LT + t) for j in js for t in range(LT)]

    def a_attention(b, first_block=False, to=None):
        state = {}

        def window(j, r0, w):
            lo = HALO + r0 - ADIL * w
            return qkv_s[b, j * LT:(j + 1) * LT, lo:lo + 8, :]

        def logits(plan, r0):
            q = _rows(*[plan.paced(qkv_s[b, t, HALO + r0:HALO + r0 + 8, :], t / LT)
                        for t in range(LT)]).reshape(LT, 8, 128)
            a = _rows(*[jnp.sum(q * window(1, r0, w), axis=0) for w in range(AW)])
            state[r0] = a + pltpu.roll(a, 2 * AH, 1)

        def fold(plan, r0):
            state[r0] = state[r0] + pltpu.roll(state[r0], AH, 1)

        def weigh(plan, r0):
            a = state[r0].reshape(AW, 8, 128)
            if first_block and r0 < HALO:
                w, pos = [lax.broadcasted_iota(jnp.int32, a.shape, axis) for axis in range(2)]
                a = jnp.where(pos + r0 >= ADIL * w, a, MASKED * AD ** 0.5)
            state[r0] = jnp.exp2((a - jnp.max(a, axis=0)) * (AD ** -0.5 * LOG2E))

        def mix(plan, r0):
            e = state.pop(r0)
            e = [plan.paced(e[w], w / AW) for w in range(AW)]
            o = functools.reduce(jnp.add, (e[w] * window(2, r0, w) for w in range(AW)))
            oa_s[to or b][0, :, r0:r0 + 8, :] = o * _inverse(functools.reduce(jnp.add, e))

        n = TB // 8
        return [_task(f, (k - lag) * 8) for k in range(n + 2)
                for lag, f in ((2, weigh), (0, logits), (1, fold), (2, mix)) if 0 <= k - lag < n]

    def a_out(i, b, rows=TB, depth=LT):
        sums = _Sums()

        def tile(plan, t, k0):
            def weights(r):
                at = (plan.zero >> r // rows + 3 * b) * 32 + 3 * D // 2 + k0 * 64
                return aw[pl.ds(pl.multiple_of(at, 32), depth * 64), t * 128:(t + 1) * 128]

            o = lax.concatenate([oa_s[b][plan.zero, k] for k in range(k0, k0 + depth)], 1)
            sums.add(t, _rows(*[_dot(o[r:r + rows], pltpu.bitcast(weights(r), BF16))
                                for r in range(0, TB, rows)]))
            if k0 + depth == LT:
                outa[_ds(i, TB), t * 128:(t + 1) * 128] = plan.result(sums.take(t)).astype(BF16)
        return [_task(tile, t, k0) for t in range(LT) for k0 in range(0, LT, depth)]

    def tiles_of(c, odd=None, zero=0):
        if isinstance(c, int) and c >= FULL:
            return wt[2 + c - FULL].at[zero]
        return wt[c % 2 if odd is None else odd].at[c // 2 + zero]

    def w_transpose(c, grp, odd=None):
        src, dst = raw.at[c % RING], tiles_of(c, odd)

        def two(plan, i, f):
            t = _words(src[f * 128:(f + 2) * 128, i * 128:(i + 1) * 128].T)
            for k in range(2):
                dst[grp.slot[i, f + k]] = t[:, k * 128:(k + 1) * 128]
        return [_task(two, i, f) for f in range(0, grp.n, 2) for i in range(LT)]

    def w_combine(c, grp, odd=None, transposed=True):
        w, own, other = tiles_of(c, odd, nil), {}, {}

        def edge(plan, r, a, b):
            def tile(i, f, part=0.0):
                if transposed:
                    t = plan.paced(w[grp.slot[i, f], _ds(r, 8)], part)
                else:
                    t = _words(raw[c % RING, _ds(8 * f + r, 16), i * 128:(i + 1) * 128])
                    t = plan.paced(t, part)
                    if i != grp.label[f]:
                        w[grp.slot[i, f], _ds(r, 8)] = t
                return pltpu.bitcast(t, BF16).astype(F32)

            for f in (a, b):
                if f not in own:
                    own[f] = other[f] = tile(grp.label[f], f)
            ta, tb = tile(grp.label[b], a), tile(grp.label[a], b, 0.5)
            w[grp.slot["both", a, b], _ds(r, 8)] = _words(ta + tb)
            own[a], other[a] = own[a] - ta, other[a] + tb
            own[b], other[b] = own[b] - tb, other[b] + ta
            for f, mate in ((a, b), (b, a)):
                if mate == grp.mates[f][-1]:
                    w[grp.slot[grp.label[f], f], _ds(r, 8)] = _words(own.pop(f))
                    w[grp.slot["other", f], _ds(r, 8)] = _words(other.pop(f))
                    for i in grp.plain[f] * (not transposed):
                        tile(i, f)

        return [_task(edge, r, a, b) for r in range(8) for a in grp.side[0] for b in grp.mates[a]]

    places = {}, {}

    def place(memory, *key):
        return places[memory].setdefault(key, len(places[memory]))

    def binade(tiles):
        top = jnp.max(functools.reduce(jnp.maximum, map(jnp.abs, tiles)), axis=1, keepdims=True)
        top = jnp.clip(jnp.broadcast_to(top, (8, 128)), 2.0 ** -60, 2.0 ** 60)
        return pltpu.bitcast(top, jnp.int32) & 0x7F800000

    def memory_operands(ph, known, i, t):
        known[i] = l_mem[ph][0, place(1, "plain", i)] = t
        for k, u in known.items():
            if k != i:
                l_mem[ph][0, place(1, "cross", min(i, k), max(i, k))] = t + u

    def memory_pair(plan, ph):
        cur = [l_mem[ph][0, place(1, "plain", i)] for i in range(LT)]
        shift = binade(cur) - pltpu.bitcast(
            l_tok[ph][plan.zero, place(0, "mate", 0), 8:16], jnp.int32)
        down, up = [pltpu.bitcast(x, F32) for x in (0x3F800000 + shift, 0x3F800000 - shift)]
        l_mem[ph][0, place(1, "down")], l_mem[ph][0, place(1, "up")] = down, up
        for k in range(LT):
            mate = l_tok[ph][plan.zero, place(0, "mate", k), 0:8]
            for kind in range(2):
                l_tok[1 - ph][0, place(0, "other", kind, k), 8:16] = mate - cur[k] * up
            mate = mate * down
            for i in range(LT):
                l_mem[ph][0, place(1, "both", i, k)] = cur[i] - mate if i == k else cur[i] + mate

    def token_operands(x, s, ph):
        def tokens(plan, ds, i):
            t = _words(x[_ds(max(s + ds, 0), SEG), i * 128:(i + 1) * 128])
            return pltpu.bitcast(plan.paced(t), BF16).astype(F32)

        def one(plan, i, kind):
            before, cur, after, later = [tokens(plan, ds, i) for ds in range(-1, 3)]
            third = (after[16:24], before[16:24], after[8:16])[kind]
            at = place(0, "other", kind, i)
            l_tok[ph][0, at, 0:8] = cur[0:8] - before[24:32]
            l_tok[ph][0, at, 16:32] = cur[16:32] - _rows(third, after[0:8])
            if kind < 2:
                l_tok[ph][0, place(0, "own", kind, i), 0:SEG] = _rows(
                    later[:16 + 8 * kind], cur[16 + 8 * kind:])
                return
            l_tok[ph][0, at, 8:16] = cur[8:16] - before[16:24]
            l_tok[ph][0, place(0, "plain", i), 0:SEG] = cur
            l_tok[ph][0, place(0, "mate", i), 0:8] = after[8:16]
            if s == 0:
                l_tok[ph][0, place(0, "next", i), 0:SEG] = after

        def two(plan, i, k):
            cur, after = tokens(plan, 0, i), tokens(plan, 1, k)
            if i < k:
                l_tok[ph][0, place(0, "cross", i, k), 0:SEG] = cur + tokens(plan, 0, k)
            fourth = cur[24:32] + after[0:8]
            l_tok[ph][0, place(0, "both", i, k), 0:SEG] = _rows(
                cur[16:24] + after[8:16], fourth, cur[16:24] + after[16:24], fourth)

        def magnitude(plan):
            l_tok[ph][0, place(0, "mate", 0), 8:16] = pltpu.bitcast(
                binade([tokens(plan, 1, i)[8:16] for i in range(LT)]), F32)

        return [magnitude] + [task for i in range(LT) for task in
                              [_task(one, i, kind) for kind in range(3)]
                              + [_task(two, i, k) for k in range(LT) if k != i]]

    def segment(s, ph, operands, first=False, last=False):
        zero = nil if isinstance(s, int) else s >> 16
        zeros, uses = [zero >> k for k in range(3)], {}

        def again(*key):
            uses[key] = uses.get(key, 0) + 1
            return zeros[uses[key] % len(zeros)]

        def product(plan, parts, j, g, key):
            w = tiles_of(chunk(j, g))[GROUPS[g].slot[key]]
            return plan.result(_dot(_rows(*parts), pltpu.bitcast(w, BF16)))

        unsaved = {}
        pieces = {}

        def project(j, g):
            grp, f0, kind = GROUPS[g], g * GW, _kind(j, g, ph)
            lab = grp.label
            late = 16 + 8 * (kind == 1)
            lo, end = 0 if first else late, SEG if last and j == 0 else L
            y, gift, kept = unsaved.setdefault((j, g), _Sums()), _Sums(), []
            left = {a: LT for a in grp.side[ph]}
            owed = {a: 1 + len(grp.mates[a]) for a in grp.side[ph]}

            def tok(r0, r1, *key):
                return [l_tok[ph][again(*key), place(0, *key), r0:r1]]

            def memory(*key):
                at = again(1, *key) if kind < 2 else 0
                return [l_mem[ph][at, place(1, *key)]] * (end == L)

            def keep(f, r0, t, minus=False):
                y_s[chunk(j, g)][0, len(kept), r0:end] = t
                pieces.setdefault((j, f0 + f), []).append((len(kept), r0, minus))
                kept.append(f)

            def add(a, t):
                y.add(a, t)
                left[a] -= 1
                if not left[a]:
                    keep(a, 0, y.take(a))

            def give(a, t):
                if last:
                    return
                gift.add(a, t)
                owed[a] -= 1
                if not owed[a]:
                    t = gift.take(a)
                    for r, mate in zip((16, 24, 32), MATES[kind]):
                        if mate is not None:
                            u = t[r - lo:r - lo + 8]
                            ahead[ph][0, j, f0 + a, 0, mate:mate + 8] = (
                                u if r < SEG else u * memory("up")[0])

            def own(plan, a):
                parts = tok(0, late if first else SEG, "own", kind % 2, lab[a]) * (not last)
                parts += tok(lo, SEG, "plain", lab[a]) if first or last else []
                t = product(plan, parts + memory("plain", lab[a]), j, g, (lab[a], a))
                old = [] if first else [ahead[ph][0, j, f0 + a, 1, 0:late]]
                if not last:
                    ahead[ph][0, j, f0 + a, 1, 0:late] = t[:late]
                    t = t[late:]
                add(a, _rows(*old, t))
                give(a, t)

            def opening(plan, b):
                n = 16 + 8 * (kind == 0)
                ahead[1 - ph][0, j, f0 + b, 1, 0:n] = product(
                    plan, tok(0, n, "next", lab[b]), j, g, (lab[b], b))

            def other(plan, b):
                k = lab[b]
                parts = tok(0, late, "plain", k) if first else []
                parts += tok(late - lo, late if last else SEG, "other", kind, k)
                parts += tok(late, SEG, "plain", k) if last else []
                parts += memory("plain", k) if last or kind == 2 else memory("both", k, k)
                at = 0 if first else zero
                got = [] if first else [ahead[1 - ph][at, j, f0 + b, 0, 0:late]]
                for r, mate in zip((16, 24, 32), MATES[kind] * (not last)):
                    if mate is not None:
                        u = ahead[1 - ph][at, j, f0 + b, 1, mate:mate + 8]
                        got.append(u if r < SEG else plan.paced(u) * memory("down")[0])
                t, got = product(plan, parts, j, g, ("other", b)), _rows(*got)
                r0, r1 = late - lo, late - lo + got.shape[0]
                y.add(b, _rows(*[t[:r0] for _ in range(r0 > 0)], t[r0:r1] + got,
                               *[t[r1:] for _ in range(r1 < end)]))

            def both(plan, a, b):
                i, k = lab[a], lab[b]
                parts = tok(0, late, "plain", i) if first else []
                parts += tok(late, SEG, "plain", i) if last else tok(
                    *((0, 16) if kind == 2 else (late, SEG)), "both", i, k)
                parts += memory("plain", i) if last or kind == 2 else memory("both", i, k)
                t = product(plan, parts, j, g, ("both", a, b))
                give(a, t)
                if first:
                    y.add(b, t)
                elif b in y:
                    u = y.take(b)
                    keep(b, 0, _rows(u[:lo], u[lo:] + t))
                else:
                    keep(b, lo, t)

            def cross(plan, a, b):
                key = "cross", *sorted((lab[a], lab[b]))
                t = product(plan, tok(0, SEG, *key) + memory(*key), j, g, (lab[b], a))
                add(a, t)
                y.add(b, t, True)
                keep(b, 0, *y.pop(b))

            def plain(plan, i, f):
                t = product(plan, tok(0, SEG, "plain", i) + memory("plain", i), j, g, (i, f))
                (add if f in left else y.add)(f, t)

            passes = []
            others = list(grp.side[1 - ph])
            for a, b0 in zip(grp.side[ph], others[grp.n == GW:] + others):
                passes += [((), _task(opening, b0), 1)] * first
                passes += [((lab[a],), _task(own, a), 0), ((lab[b0],), _task(other, b0), 0)]
                passes += [((i,), _task(plain, i, f), 0) for f in (a, b0) for i in grp.plain[f]]
                passes += [((lab[a],), _task(both, a, b), 0 if first else 2 - kind % 2)
                           for b in grp.mates[a]]
                passes += [((lab[a], lab[b]), _task(cross, a, b), 0) for b in grp.mates[a]]
            return passes

        n = SEG if last else L
        row, col = [lax.broadcasted_iota(jnp.int32, (L, 2 * n), axis) for axis in range(2)]
        head0 = col < n
        query = jnp.where(head0, col, col - n) + (L - n)
        visible = (query < M) | (row >= SEG) | (query >= row + M)
        scores = _Sums()

        def gather(j, f):
            sums, end = _Sums(), L if j else n

            def add_up(plan, part):
                assert not unsaved[j, f // GW]
                for k, (at, r0, minus) in enumerate(pieces[j, f][part::2]):
                    u = y_s[chunk(j, f // GW)][zero, at, r0:end]
                    sums.add(r0, u if k else plan.paced(u), minus)
                if part == 0:
                    return
                t = sums.take(0)
                for r0 in list(sums):
                    t = _rows(t[:r0], t[r0:] + sums.take(r0))
                if j == 1:
                    qk_s[f][0, 1, 0:L] = pltpu.bitcast(t, U32)
                    return
                if j == 0 and not last:
                    t = _rows(t[SEG:], t[:SEG])
                pad = [jnp.zeros((8, 128), F32)] * (end % 16 // 8)
                if f % 3 == 1:
                    low = lax.broadcasted_iota(jnp.int32, t.shape, 1) < 64
                    t = _words(_rows(jnp.where(low, t, 0.0), jnp.where(low, 0.0, t)))
                else:
                    t = _words(_rows(*[t, *pad][::1 - f % 3]))
                (v_s if j else qk_s)[f][0, 0, 0:t.shape[0]] = t

            return [_task(add_up, part) for part in range(2)]

        def by_head(ref, f, rows, short=False):
            t = ref[f][zero, 0, 0:rows if f % 3 == 1 else pl.cdiv(rows, 16) * 8]
            if f % 3 == 2 or f % 3 == 0 and not short:
                t = _rows(*[t, jnp.zeros((rows - t.shape[0], 128), U32)][::1 - f % 3])
            return pltpu.bitcast(t, BF16)

        def score(plan, f):
            k = pltpu.bitcast(qk_s[f][zero, 1, 0:L], F32)
            scores.add(f // 3, lax.dot_general(k, by_head(qk_s, f, n), NT,
                                               preferred_element_type=F32))
            if f % 3 == 2:
                sc = jnp.where(visible, scores.take(f // 3), MASKED * DH ** 0.5)
                e = jnp.exp2((sc - jnp.max(sc, axis=0, keepdims=True)) * (DH ** -0.5 * LOG2E))
                p = e * _inverse(jnp.sum(e, axis=0, keepdims=True))
                p = _rows(jnp.where(head0, p, 0.0), jnp.where(head0, 0.0, p)).T
                p_s[f // 3][0, 0:3 * n, 0:2 * L] = _rows(p[:n], p[:n] + p[n:], p[n:])

        def mix(plan, f):
            v = by_head(v_s, f, L, True)
            o = _dot(p_s[f // 3][zero, _ds(f % 3, n), 0:v.shape[0]], v)
            if last:
                o = _rows(jnp.zeros((M, 128), F32), o)
            g = f // GW
            o_s[ph][g][0, f % GW] = o
            if not first and f % GW in GROUPS[g].side[1 - ph]:
                k = 16 + 8 * _kind(3, g, ph)
                o_old[1 - ph][0, f, 0:k] = o[:k] + o_s[1 - ph][g][zero, f % GW, L - k:]

        z, written = _Sums(), set()

        def out_project(groups):
            def run(plan, part, left, what, g, a, b, to):
                k, r0, i = 16 + 8 * _kind(3, g, ph), L - n, to[0][1]

                def cur(f, r0, r1=L):
                    return o_s[ph][g][again(g, f), f, r0:r1]

                def joined(r0):
                    t = cur(b, r0, k)
                    if not first:
                        t = t + o_s[1 - ph][g][again(1, g, a), a, L - k + r0:]
                    return [t, cur(b, k)] if last else [t]

                if what == "own":
                    old = [] if first else [o_old[ph][zero, g * GW + a, 0:L - k]]
                    t = product(plan, joined(r0) + old, 3, g, (i, a))
                elif what == "closing":
                    t = product(plan, [o_old[1 - ph][0, g * GW + b, 0:k]], 3, g, (i, b))
                elif what == "both":
                    t = product(plan, joined(0), 3, g, (what, a, b))
                elif what == "cross":
                    t = product(plan, [cur(a, r0) - cur(b, r0)], 3, g, (GROUPS[g].label[b], a))
                else:
                    t = product(plan, [cur(b, r0)], 3, g, (what if what == "other" else i, b))
                part.add(to, t)
                left.remove(to)
                if to in left:
                    return
                t = part.take(to)
                for back, i, dst, src, rows, minus in to:
                    if last:
                        z.add_rows((back, i), dst, t[src:src + rows], minus)
                    elif back == 0:
                        z.add((0, i, 0), t[:M])
                if not last:
                    r0 = M * all(x[0] % 2 == 0 for x in to)
                    at = PARTS[ph][[x[0][1] for x in STREAM if (3, g) in x][0], to]
                    rows = slice(r0, t.shape[0])
                    z_part[ph][0, at, rows] = (t[r0:] + z_part[ph][0, at, rows] if at in written
                                               else t[r0:])
                    written.add(at)

            tasks = [], []
            for (lo, hi, order, i), passes in _out_passes(groups, ph, last):
                part, left = _Sums(), [x[-1] for x in passes]
                tasks[order == 1].extend(
                    ((lo, hi) if order == 2 else (i,), _task(run, part, left, *x),
                     (order == 1) * (1 + _kind(3, x[1], ph))) for x in passes)
            order = [((k // 4 + 0.5) / len(xs), short, k) for short, xs in enumerate(tasks)
                     for k in range(len(xs))]
            return [tasks[short][k] for _, short, k in sorted(order)]

        main, begin, done = [], {}, {}
        parts = FIRST if first else STREAM
        for part in parts:
            if part[0][0] == 3:
                new = out_project([g for _, g in part])
            else:
                new = [project(*jg) for jg in part]
                new = [x for k in range(0, len(new[0]), GW) for xs in new for x in xs[k:k + GW]]
            if part is parts[0] and not first:
                new.sort(key=lambda x: max(x[0]) == LT - 1)
            if part is parts[-1]:
                new.sort(key=lambda x: min(x[0]) == LT - 1)
            begin.update({jg: len(main) for jg in part})
            main += new
            done.update({jg: len(main) for jg in part})

        queues = [[x for x in main if x[2] == q] for q in range(3)]
        queues += [[(_task(stage, f), js, f) for f in range(FT)]
                   for stage, js in ((score, (0, 1)), (mix, (2,)))]
        queues += [[(task, (), 0) for task in a_out(NB - 1, 2, depth=1) * first]]
        main, extra = [], []
        for q in map(int, ORDER[0 if first else 3 if last else 2 - ph]):
            if q < 3:
                main.append(queues[q].pop(0))
            else:
                extra.append((len(main) - 1 + len(extra) * 1e-4, *queues[q].pop(0)))
        assert not any(queues)
        plan = _Plan(zero, [x[1] for x in main])
        for at, task, js, f in extra:
            if js:
                k0 = max(at - 38, *[done[j, f // GW] - 1 for j in js])
                assert k0 < at < begin[3, f // GW] - 1
                plan.spread([t for j in js for t in gather(j, f)], k0, max(at - 28, k0))
            plan.spread([task], at)

        if first:
            def arrive(plan, groups):
                wait([c_w(chunk(3, g)) for g in groups])
                start([c_w(chunk(3, g + 3)) for g in groups if g + 3 < NG])

            plan.spread([t for j in (1, 2) for t in w_transpose(FULL + j, GROUPS[-1])], 0)
            ends = 340, 640, 770, 880, begin[3, 4]
            plan.spread([t for j in range(3) for t in w_combine(FULL + j, GROUPS[-1])],
                        0, ends[0] - 8)
            for groups, k0, k1 in zip(((0, 1), (2,), (3,), (4,)), ends, ends[1:]):
                plan.spread([_task(arrive, groups)], k0)
                plan.spread([t for g in groups
                             for t in w_combine(chunk(3, g), GROUPS[g], None, False)], k0, k1 - 8)
        else:
            def resume(plan):
                for i in range(LT):
                    if not last:
                        z.add((0, i, 0), z_s[1 - ph][zero, 2, i, 0:M])
                        continue
                    for back in range(3):
                        z.add_rows((back, i), M, z_s[1 - ph][zero, (back - 1) % 3, i,
                                                            M:L if back else 24])

            plan.spread(settle(s - 1, 1 - ph), 30, 130)
            plan.spread([resume], begin[3, 0] - 1)
        if not last:
            k0 = 945 if first else 800
            plan.spread(operands, k0, k0 + 100)
            plan.spread([_task(memory_pair, ph)], 0)
            known = {}
            for i in range(LT):
                plan.spread([lambda _, i=i: memory_operands(1 - ph, known, i, z.take((0, i, 0)))],
                            max(k for k, (tiles, *_) in enumerate(main) if i in tiles))
        plan.run()
        for back in (2, 1, 0) * last:
            for i in range(LT):
                outb[_ds(s - back, SEG), i * 128:(i + 1) * 128] = _rows(
                    *[z.take((back, i, r)) for r in range(M, L, 8)]).astype(BF16)

    def settle(s, ph):
        found, sums = {}, _Sums()
        for (_, to), at in PARTS[ph].items():
            for back, i, dst, src, rows, minus in to:
                skip = M * (back == dst == 0)
                found.setdefault((i, back), []).append(
                    (at, dst + skip, src + skip, rows - skip, minus))

        def add(plan, some):
            for k, (at, dst, src, rows, minus) in enumerate(some):
                u = z_part[ph][plan.zero, at, src:src + rows]
                sums.add((dst, rows), u if k else plan.paced(u), minus)

        def finish(plan, i, back):
            t = _Sums()
            if back >= 0:
                t.add_rows((), M, z_s[1 - ph][plan.zero, (back - 1) % 3, i, M:L if back else 24])
            for dst, rows in list(sums):
                t.add_rows((), dst, *sums.pop((dst, rows)))
            r0 = min(t)[0]
            t = _rows(*[t.take(r) for r in sorted(t)])
            if back < 2:
                z_s[ph][0, back % 3, i, r0:r0 + t.shape[0]] = t
            else:
                seg = max(s - 2, 0) if isinstance(s, int) else jnp.maximum(s - 2, 0)
                outb[_ds(seg, SEG), i * 128:(i + 1) * 128] = t.astype(BF16)

        return [task for key, xs in sorted(found.items()) for task in
                [_task(add, xs[k:k + 4]) for k in range(0, len(xs), 4)] + [_task(finish, *key)]]

    def clear(k, carry):
        z_part[0][0, _ds(k, 4)] = jnp.zeros((4, L, 128), F32)
        return lax.shift_right_logical(k, 16)

    def with_weights(plan, first, groups):
        for b, grp in enumerate(groups):
            new, before = [k if isinstance(k, int) else jnp.where(k < 0, k + RING, k)
                           for k in (first + b, first + b - 1)]
            plan.spread(w_combine(before, GROUPS[0], b), 8 * b, 8 * b + 8)
            plan.spread(w_transpose(new, grp, 1 - b), 8 * b, 8 * b + 8)

    def a_step(it, carry):
        for k in range(FULL // 2):
            @pl.when(it == k)
            def _():
                wait([c_w(c) for c in (2 * k - 1, 2 * k) if c >= 0]
                     + {1: [c_ax[3]], 3: [c_ax[4]]}.get(k, []))
                start([c_w(2 * k + 2), c_w(2 * k + 3)])
                start({0: [c_ax[3]], 2: [c_ax[4]], 4: [c_mem, c_bx0]}.get(k, []), 0)
        plan = _Plan(nil, a_out(2 * it, 0) + a_out(2 * it + 1, 1) + a_proj(1) + a_proj(0))
        with_weights(plan, 2 * it - 1, [GROUPS[0]] * 2)
        plan.spread(a_attention(0), 15.5, 24.99)
        plan.spread(a_attention(1), 24.99, 38.5)
        plan.run()
        for b in range(2):
            a_input(jnp.minimum(2 * it + 6 - b, NB - 1), b)
        return carry

    def b_step(it, carry):
        @pl.when(it == 1)
        def _():
            c_bx1.wait()
        x = bx.at[pl.ds(pl.multiple_of(2 * it * SEG, 2 * SEG), 6 * SEG)]
        for u in (1, 2):
            segment(2 * it + u, u % 2, token_operands(x, u + 1, 1 - u % 2))

        @pl.when(it > 1)
        def _():
            c_outb(pl.multiple_of((it - 2) * 2 * SEG, 2 * SEG), 2 * SEG).start()
        return carry

    start([c_wqkv[0], c_ax[0], c_wqkv[1]])
    nil = lax.fori_loop(0, z_part[0].shape[1] // 4, clear, 0)
    for ref in (z_s[1], o_old[1]):
        ref[...] = jnp.zeros(ref.shape, F32)
    bx[S:, :] = jnp.zeros((2 * SEG, D), BF16)
    wait([c_wqkv[0]])
    start([c_wqkv[2]])
    _Plan(nil, a_weights(0)).run()
    wait([c_ax[0]])
    start([c_ax[1]])
    for b in range(2):
        a_input(b, b)
    _Plan(nil, a_proj(0, [0])).run()
    for j, copy in ((1, c_awo), (2, c_ax[2])):
        wait([c_wqkv[j]])
        start([copy])
        plan = _Plan(nil, a_proj(1, [j - 1]) + a_proj(0, [j], True))
        plan.spread(a_weights(j), 0, 2)
        plan.run()
    wait([c_ax[1], c_awo])
    start([c_w(0), c_w(1)])
    a_input(2, 0)
    plan = _Plan(nil, a_proj(1, [2]) + a_proj(0))
    plan.spread(a_attention(0, True), 0, 4.99)
    plan.spread(a_attention(1), 9, 18.5)
    plan.spread(a_weights(3), 9, 18.5)
    plan.run()
    wait([c_ax[2]])
    for b in range(2):
        a_input(4 - b, b)
    lax.fori_loop(0, FULL // 2, a_step, 0)
    wait([c_mem, c_bx0, c_w(FULL - 1), c_w(FULL), c_w(FULL + 1)])
    start([c_w(FULL + 2), c_w(FULL + 3), c_w(FULL + 4)])
    plan = _Plan(nil, a_out(NB - 4, 0, 48) + a_proj(1) + a_out(NB - 3, 1, 48)
                 + a_out(NB - 2, 0, 48))
    with_weights(plan, FULL - 1, [GROUPS[0], GROUPS[-1]])
    plan.spread(a_attention(0), 14, 21.0)
    plan.spread(a_attention(1, to=2), 21.0, 29)
    plan.spread(token_operands(bx, 0, 0), 16, 28)
    plan.run()
    wait([c_w(FULL + 2)])
    start([c_w(FULL + 5)])
    known = {}
    for i in range(LT):
        memory_operands(0, known, i, mem[0:M, i * 128:(i + 1) * 128].astype(F32))
    segment(0, 0, token_operands(bx, 1, 1), first=True)
    start([c_bx1, c_outa])
    lax.fori_loop(0, NSEG // 2 - 1, b_step, 0)
    c_outb(S - 6 * SEG, 2 * SEG).start()
    segment(NSEG - 1, 1, None, last=True)
    c_outb(S - 4 * SEG, 4 * SEG).start()
    wait([c_outa, c_outb(0, S)])


def pallas_concat_heads__sliding_local_dilated__memory_aug_recurrent_mem_tr__prompt_kernel(
    A_x, A_wqkv, A_wo, B_x, B_mem0, B_Wq, B_Wk, B_Wv, B_Wo, B_seg_len,
):
    assert B_seg_len == SEG
    assert A_x.shape == B_x.shape == (1, S, D) and B_mem0.shape == (1, M, D)
    assert B_Wq.shape == B_Wk.shape == B_Wv.shape == (D, H, DH) and B_Wo.shape == (H, DH, D)
    dma = pltpu.SemaphoreType.DMA

    def vmem(dtype, *shape):
        assert math.prod(shape) * jnp.dtype(dtype).itemsize % 16384 == 0, shape
        return pltpu.VMEM(shape, dtype)

    call = pl.pallas_call(
        _kernel,
        out_shape=jax.ShapeDtypeStruct((S, 2 * D), BF16),
        in_specs=[pl.BlockSpec(memory_space=pl.ANY)] * 9,
        out_specs=pl.BlockSpec(memory_space=pl.ANY),
        scratch_shapes=[
            vmem(BF16, S, D),
            vmem(BF16, 3, D, D),
            vmem(BF16, D, D),
            vmem(F32, 2, LT, D, 128),
            vmem(U32, 2 * D, D),
            vmem(U32, 2, TB // 2, D),
            vmem(F32, 2, 3 * LT, HALO + TB, 128),
            [vmem(F32, 1, LT, TB, 128)] * 3,
            vmem(BF16, S, D),
            vmem(BF16, S + 2 * SEG, D),
            vmem(BF16, 64, D),
            vmem(BF16, RING, GW * 128, D),
            [vmem(U32, n, SLOTS, 64, 128) for n in [FULL // 2] * 2 + [1] * 8],
            [vmem(F32, 1, 72, 40, 128)] * 2,
            [vmem(F32, 1, 44, M, 128)] * 2,
            [vmem(F32, 1, 3, FT, 2, 24, 128)] * 2,
            [vmem(F32, 1, 48, L, 128)] * (3 * NG),
            [vmem(U32, 1, 2, 48, 128)] * FT,
            [vmem(U32, 1, 1, 64, 128)] * FT,
            [vmem(F32, 1, 128, 128)] * (FT // 3),
            [[vmem(F32, 1, 12, L, 128)] * NG] * 2,
            [vmem(F32, 1, FT, 24, 128)] * 2,
            [vmem(F32, 1, pl.cdiv(max(map(len, PARTS)), 4) * 4, L, 128)] * 2,
            [vmem(F32, 1, 4, LT, L, 128)] * 2,
            vmem(BF16, S, D),
            dma((4,)), dma((5,)), dma((4,)), dma((3,)), dma((2,)),
        ],
        compiler_params=pltpu.CompilerParams(
            vmem_limit_bytes=126 * 1024 * 1024,
            flags={"XLA_TPU_EVENLY_DISTRIBUTE_CRITICAL_NODES": True}),
        name="sliding_and_memory_attention",
    )

    def by_feature(w):
        return w.transpose(1, 2, 0).reshape(H * DH, D)

    out = call(A_x.reshape(S, D), A_wqkv, A_wo, B_x.reshape(S, D), B_mem0.reshape(M, D),
               by_feature(B_Wq), by_feature(B_Wk), by_feature(B_Wv), B_Wo.reshape(H * DH, D))
    return out.reshape(1, S, 2 * D)
```
